```python
import jax
import jax.numpy as jnp

def _softmax(x, axis=-1):
    return jax.nn.softmax(x, axis=axis)

def _gelu(x):
    return jax.nn.gelu(x, approximate=True)

def _silu(x):
    return jax.nn.silu(x)

def _sigmoid(x):
    return jax.nn.sigmoid(x)

def _layernorm(x, axis=-1, eps=1e-05):
    m = jnp.mean(x, axis=axis, keepdims=True)
    v = jnp.var(x, axis=axis, keepdims=True)
    return (x - m) / jnp.sqrt(v + eps)

def _scatter_add(tgt, idx, src, axis=0):
    return tgt.at[idx].add(src)

def _segment_sum(src, seg, n):
    return jax.ops.segment_sum(src, seg, n)

class _Rng:

    def __init__(self, key):
        self._k = key

    def _next(self):
        self._k, sub = jax.random.split(self._k)
        return sub

    def normal(self, shape):
        return jax.random.normal(self._next(), shape, dtype=jnp.bfloat16)

    def randint(self, lo, hi, shape):
        return jax.random.randint(self._next(), shape, lo, hi, dtype=jnp.int32)

    def uniform(self, shape, lo=0.0, hi=1.0):
        return jax.random.uniform(self._next(), shape, jnp.bfloat16, lo, hi)

    def permutation(self, n):
        return jax.random.permutation(self._next(), n)
kernel_name = 'adaLN_cond__memory_aug_recurrent_mem_tr__mixer_s_mlp__prompt'

def setup_inputs():
    _rng = _Rng(jax.random.key(int.from_bytes(__import__("os").urandom(4), "little")))
    _w = lambda a: (lambda t: t.astype(jnp.bfloat16) if jnp.issubdtype(t.dtype, jnp.floating) else t)(jnp.asarray(a))

    def _A_setup():
        B, S, Dm = (1, 2048, 1024)
        H, Dh = (32, 128)
        M, seg = (8, 32)
        seg = min(seg, S)
        S = S // seg * seg
        return {'x': _w((lambda *s: _rng.normal(s) * 0.05)(B, S, Dm)), 'mem0': _w((lambda *s: _rng.normal(s) * 0.05)(B, M, Dm)), 'Wq': _w((lambda *s: _rng.normal(s) * 0.05)(Dm, H, Dh) * Dm ** (-0.5)), 'Wk': _w((lambda *s: _rng.normal(s) * 0.05)(Dm, H, Dh) * Dm ** (-0.5)), 'Wv': _w((lambda *s: _rng.normal(s) * 0.05)(Dm, H, Dh) * Dm ** (-0.5)), 'Wo': _w((lambda *s: _rng.normal(s) * 0.05)(H, Dh, Dm) * (H * Dh) ** (-0.5)), 'seg_len': seg}
    _A_in = _A_setup()

    def _B_setup():
        B, S, D, F = (1, 2048, 1024, 3584)
        return {'x': _w((lambda *s: _rng.normal(s) * 0.05)(B, S, D)), 'w1': _w((lambda *s: _rng.normal(s) * 0.05)(D, D) * D ** (-0.5)), 'w2': _w((lambda *s: _rng.normal(s) * 0.05)(D, D) * D ** (-0.5)), 'w3': _w((lambda *s: _rng.normal(s) * 0.05)(D, F) * D ** (-0.5)), 'w4': _w((lambda *s: _rng.normal(s) * 0.05)(F, D) * F ** (-0.5))}
    _B_in = _B_setup()
    return {'A_x': _A_in['x'], 'A_mem0': _A_in['mem0'], 'A_Wq': _A_in['Wq'], 'A_Wk': _A_in['Wk'], 'A_Wv': _A_in['Wv'], 'A_Wo': _A_in['Wo'], 'A_seg_len': _A_in['seg_len'], 'B_x': _B_in['x'], 'B_w1': _B_in['w1'], 'B_w2': _B_in['w2'], 'B_w3': _B_in['w3'], 'B_w4': _B_in['w4'], 'c': _w((lambda *s: _rng.normal(s) * 0.05)(1, 1024)), 'w_mod': _w((lambda *s: _rng.normal(s) * 0.05)(1024, 6 * 1024) * 1024 ** (-0.5))}

def reference(A_x, A_mem0, A_Wq, A_Wk, A_Wv, A_Wo, A_seg_len, B_x, B_w1, B_w2, B_w3, B_w4, c, w_mod):

    def _A_ref(x, mem0, Wq, Wk, Wv, Wo, seg_len):
        B, S, Dm = x.shape
        H, Dh = (Wq.shape[1], Wq.shape[2])
        M = mem0.shape[1]
        scale = Dh ** (-0.5)
        n_seg = S // seg_len
        L = M + seg_len
        idx = jnp.arange(L)
        mask = (idx[:, None] < M) | (idx[:, None] >= idx[None, :])
        mem = mem0
        outs = []
        for s in range(n_seg):
            xs = x[:, s * seg_len:(s + 1) * seg_len, :].copy()
            h = jnp.concatenate([mem, xs], axis=1)
            q = jnp.einsum('btd,dhe->bhte', h, Wq)
            k = jnp.einsum('btd,dhe->bhte', h, Wk)
            v = jnp.einsum('btd,dhe->bhte', h, Wv)
            scores = jnp.einsum('bhqe,bhke->bhqk', q, k) * scale
            scores = jnp.where(mask[None, None], scores, -1000000000.0)
            p = _softmax(scores, axis=-1)
            o = jnp.einsum('bhqk,bhke->bhqe', p, v)
            o = jnp.einsum('bhte,hed->btd', o, Wo)
            mem = o[:, :M, :].copy()
            outs.append(o[:, M:, :])
        return jnp.concatenate(outs, axis=1)

    def _B_ref(x, w1, w2, w3, w4):
        B, S, D = x.shape
        h = _gelu(_layernorm(x, axis=-1) @ w1)
        c = D // 4
        g0 = jnp.pad(h[:, :, 0 * c:1 * c], ((0, 0), (1, 0), (0, 0)))[:, :S, :]
        g1 = jnp.pad(h[:, :, 1 * c:2 * c], ((0, 0), (0, 1), (0, 0)))[:, 1:, :]
        g2 = jnp.pad(h[:, :, 2 * c:3 * c], ((0, 0), (2, 0), (0, 0)))[:, :S, :]
        g3 = jnp.pad(h[:, :, 3 * c:], ((0, 0), (0, 2), (0, 0)))[:, 2:, :]
        hs = jnp.concatenate([g0, g1, g2, g3], axis=-1) @ w2
        x1 = x + hs
        h2 = _gelu(_layernorm(x1, axis=-1) @ w3) @ w4
        return x1 + h2
    x = A_x
    mod = (_silu(c) @ w_mod).reshape(c.shape[0], 6, 1, -1)
    sa, ca, ga, sb, cb, gb = (mod[:, 0].copy(), mod[:, 1].copy(), mod[:, 2].copy(), mod[:, 3].copy(), mod[:, 4].copy(), mod[:, 5].copy())
    h = _layernorm(x, axis=-1) * (1 + ca) + sa
    x = x + ga * _A_ref(h, A_mem0, A_Wq, A_Wk, A_Wv, A_Wo, A_seg_len)
    h = _layernorm(x, axis=-1) * (1 + cb) + sb
    x = x + gb * _B_ref(h, B_w1, B_w2, B_w3, B_w4)
    return x
```

```python
import functools

import jax
import jax.numpy as jnp
import numpy as np
from jax import lax
import jax.experimental.pallas as pl
import jax.experimental.pallas.tpu as pltpu

F32 = jnp.float32
BF16 = jnp.bfloat16
U32 = jnp.uint32

_NN = (((1,), (0,)), ((), ()))
_NT = (((1,), (1,)), ((), ()))


def _dot(a, b, dims=_NN):
    return lax.dot_general(a, b, dims, preferred_element_type=F32)


def _ln(x):
    m = jnp.mean(x, axis=-1, keepdims=True)
    d = x - m
    v = jnp.mean(d * d, axis=-1, keepdims=True)
    return d * lax.rsqrt(v + 1e-5)


def _gelu(x):
    k0 = float(np.sqrt(2.0 / np.pi))
    k1 = float(np.sqrt(2.0 / np.pi) * 0.044715)
    hx = 0.5 * x
    return hx + hx * jnp.tanh(x * (k0 + k1 * (x * x)))


def _split_pair(raw):
    lo = pltpu.bitcast(raw << 16, F32).astype(BF16)
    hi = pltpu.bitcast(raw & np.uint32(0xFFFF0000), F32).astype(BF16)
    return pltpu.bitcast(lo, U32), pltpu.bitcast(hi, U32)


def _pair_weight(lo, hi):
    return pltpu.bitcast(jnp.concatenate([lo, hi], axis=1), BF16)


def _kernel(x_hbm, mem_hbm, wq_hbm, wk_hbm, wv_hbm, wo_hbm, w1_hbm, w2_hbm,
            w3_hbm, w4_hbm, c_hbm, wm_hbm, out_hbm,
            wq_s, wk_s, wv_s, wo_s, w1_s, w2_s, w3_s, w4_s, wm_s,
            x_s, h_s, hb_s, kr_s, vr_s, c_s, m0_s, mem_s, kvl_s, o_s, mod_s,
            hh_s, r_s, n_s, t_s, y_s,
            sq, sk, sv, so, sm, sb, sx, sy,
            *, S, D, H, DH, M, SEG, RB):
    HP = H // 2
    NSEG = S // SEG
    L = M + SEG
    KVR = SEG - M
    LOOK = S - NSEG * KVR
    RING = kr_s.shape[1]
    ROFF = RING - LOOK
    D2 = D // 2
    scale = float(DH) ** -0.5

    wq_w = wq_hbm.bitcast(U32)
    wk_w = wk_hbm.bitcast(U32)
    wv_w = wv_hbm.bitcast(U32)
    wo_w = wo_hbm.bitcast(U32)
    wm_w = wm_hbm.bitcast(U32)

    def cp_q(p):
        return pltpu.make_async_copy(wq_w.at[:, p], wq_s.at[p], sq.at[p])

    def cp_k(p):
        return pltpu.make_async_copy(wk_w.at[:, p], wk_s.at[p], sk.at[p])

    def cp_v(p):
        return pltpu.make_async_copy(wv_w.at[:, p], wv_s.at[p], sv.at[p])

    def cp_o(p):
        return pltpu.make_async_copy(
            wo_w.at[pl.ds(p * DH, DH)], wo_s.at[p], so.at[p])

    def cp_m(j):
        return pltpu.make_async_copy(
            wm_w.at[:, pl.ds(j * D, D)], wm_s.at[j], sm.at[j])

    cp_c = pltpu.make_async_copy(c_hbm, c_s, sx.at[0])
    cp_m0 = pltpu.make_async_copy(mem_hbm, m0_s, sx.at[1])
    cp_x0 = pltpu.make_async_copy(
        x_hbm.at[pl.ds(0, LOOK)], x_s.at[pl.ds(0, LOOK)], sx.at[2])
    cp_x1 = pltpu.make_async_copy(
        x_hbm.at[pl.ds(LOOK, S - LOOK)], x_s.at[pl.ds(LOOK, S - LOOK)], sx.at[3])
    cp_b = [pltpu.make_async_copy(src.bitcast(U32), dst, sb.at[i])
            for i, (src, dst) in enumerate(
                [(w1_hbm, w1_s), (w2_hbm, w2_s), (w3_hbm, w3_s), (w4_hbm, w4_s)])]

    cp_c.start()
    cp_x0.start()
    cp_m(0).start()
    cp_m(1).start()
    cp_m0.start()
    for p in range(HP):
        cp_k(p).start()

    cp_c.wait()
    cf = c_s[...].astype(F32)
    sc = jnp.broadcast_to(cf * jax.nn.sigmoid(cf), (8, D))

    def mod_vec(j):
        cp_m(j).wait()
        mod_s[j] = _dot(sc, pltpu.bitcast(wm_s[j], BF16))

    cp_x0.wait()
    PB = 128

    @pl.loop(0, LOOK // PB)
    def _(i):
        r = pl.ds(pl.multiple_of(i * PB, PB), PB)
        h_s[r, :] = _ln(x_s[r, :].astype(F32))

    mod_vec(0)
    mod_vec(1)

    @pl.loop(0, LOOK // PB)
    def _(i):
        r = pl.ds(pl.multiple_of(i * PB, PB), PB)
        h = h_s[r, :] * (1.0 + mod_s[1, 0:1, :]) + mod_s[0, 0:1, :]
        h_s[r, :] = h
        hb_s[r, :] = h.astype(BF16)

    def bulk(w_s, ring, p):
        lo, hi = _split_pair(w_s[p])
        y = _dot(hb_s[...], _pair_weight(lo, hi))
        w_s[p, pl.ds(0, D2), :] = lo
        w_s[p, pl.ds(D2, D2), :] = hi
        ring[p, pl.ds(ROFF, LOOK), :] = y.astype(BF16)

    @pl.loop(0, HP)
    def _(p):
        cp_v(p).start()
        cp_q(p).start()
        cp_k(p).wait()
        bulk(wk_s, kr_s, p)

    cp_x1.start()
    cp_x1.wait()
    XB = (S - LOOK) // HP

    @pl.loop(0, HP)
    def _(p):
        cp_o(p).start()
        cp_v(p).wait()
        cp_q(p).wait()
        bulk(wv_s, vr_s, p)
        lo, hi = _split_pair(wq_s[p])
        wq_s[p, pl.ds(0, D2), :] = lo
        wq_s[p, pl.ds(D2, D2), :] = hi
        r = pl.ds(pl.multiple_of(LOOK + p * XB, XB // 3), XB)
        h_s[r, :] = (_ln(x_s[r, :].astype(F32)) * (1.0 + mod_s[1, 0:1, :])
                     + mod_s[0, 0:1, :])

    for j in range(2, 6):
        cp_m(j).start()
    for cp in cp_b:
        cp.start()
    cp_m0.wait()
    mem_s[...] = m0_s[...].astype(F32)
    for p in range(HP):
        cp_o(p).wait()

    KP = 128
    row = lax.broadcasted_iota(jnp.int32, (L, KP), 0)
    col = lax.broadcasted_iota(jnp.int32, (L, KP), 1)
    visible = (col < L) & ((row < M) | (col >= SEG) | (row - M >= col))
    fill = jnp.where(col < L, -1e9, -jnp.inf).astype(F32)

    def wpair(w_s, p):
        return _pair_weight(w_s[p, pl.ds(0, D2), :], w_s[p, pl.ds(D2, D2), :])

    @pl.loop(0, NSEG)
    def _(s):
        seg = pl.ds(pl.multiple_of(s * SEG, SEG), SEG)
        ahead = pl.ds(pl.multiple_of(LOOK + s * KVR, 8), KVR)
        wr = pl.ds(pl.multiple_of(lax.rem(s * KVR, RING), 8), KVR)
        rd = pl.ds(pl.multiple_of(lax.rem(s * SEG + ROFF, RING), SEG), SEG)
        kvl_s[...] = jnp.concatenate([mem_s[...], h_s[ahead, :]], axis=0).astype(BF16)
        zpad = jnp.zeros((KP - L, 2 * DH), F32)

        def keys(w_s, ring, p):
            y = _dot(kvl_s[...], wpair(w_s, p))
            ring[p, wr, :] = y[M:].astype(BF16)
            tail = jnp.concatenate([y[:M], zpad], axis=0).astype(BF16)
            return jnp.concatenate([ring[p, rd, :], tail], axis=0)

        def project(p):
            k = keys(wk_s, kr_s, p)
            lhs = jnp.concatenate([mem_s[...], h_s[seg, :]], axis=0)
            q = _dot(lhs, wpair(wq_s, p))
            return q, k

        def scores(qk):
            q, k = qk
            out = []
            for i in range(2):
                c = slice(i * DH, (i + 1) * DH)
                z = jnp.where(visible, _dot(q[:, c], k[:, c], _NT) * scale, fill)
                e = jnp.exp(z - jnp.max(z, axis=-1, keepdims=True))
                out.append((e, 1.0 / jnp.sum(e, axis=-1, keepdims=True)))
            return out

        def mix(p, es, v):
            for i, (e, inv) in enumerate(es):
                c = slice(i * DH, (i + 1) * DH)
                o_s[p, :, c] = _dot(e, v[:, c]) * inv

        def out_proj(p0, p1):
            lhs = jnp.concatenate([o_s[p] for p in range(p0, p1)], axis=1)
            w = jnp.concatenate([wo_s[p] for p in range(p0, p1)], axis=0)
            return _dot(lhs, pltpu.bitcast(w, BF16))

        qk, es, vs = {}, {}, {}
        acc = None
        for t in range(HP + 2):
            if t < HP:
                qk[t] = project(t)
            elif t == HP:
                acc = out_proj(0, HP // 4)
            else:
                acc = acc + out_proj(HP // 4, HP // 2)
            if 1 <= t <= HP:
                es[t - 1] = scores(qk.pop(t - 1))
                vs[t - 1] = keys(wv_s, vr_s, t - 1)
            if t >= 2:
                mix(t - 2, es.pop(t - 2), vs.pop(t - 2))
        acc = acc + out_proj(HP // 2, HP)
        mem_s[...] = acc[:M]
        h_s[seg, :] = acc[M:]

    for j in range(2, 6):
        mod_vec(j)
    for cp in cp_b:
        cp.wait()
    NB = S // RB
    CT = D // 128
    G = CT // 4
    for j in range(CT):
        hh_s[j, pl.ds(0, 8), :] = jnp.zeros((8, 128), F32)
        hh_s[j, pl.ds(8 + S, 8), :] = jnp.zeros((8, 128), F32)

    def rows(i):
        return pl.ds(pl.multiple_of(i * RB, RB), RB)

    def prep(i):
        r = rows(i)
        x1 = x_s[r, :].astype(F32) + mod_s[2, 0:1, :] * h_s[r, :]
        h_s[r, :] = x1
        hb = _ln(x1) * (1.0 + mod_s[4, 0:1, :]) + mod_s[3, 0:1, :]
        r_s[r, :] = hb
        return _ln(hb).astype(BF16)

    def token_fc(i, n):
        g = _gelu(_dot(n, pltpu.bitcast(w1_s[...], BF16)))
        for j in range(CT):
            hh_s[j, pl.ds(pl.multiple_of(8 + i * RB, 8), RB), :] = (
                g[:, j * 128:(j + 1) * 128])

    n_s[0] = prep(0)

    @pl.loop(0, NB - 1)
    def _(i):
        token_fc(i, n_s[i % 2])
        n_s[(i + 1) % 2] = prep(i + 1)

    token_fc(NB - 1, n_s[(NB - 1) % 2])

    def token_mix(i):
        r = rows(i)
        shifted = jnp.concatenate(
            [hh_s[j, pl.ds(8 + i * RB + (-1, 1, -2, 2)[j // G], RB), :]
             for j in range(CT)], axis=1)
        x2 = r_s[r, :] + _dot(shifted, pltpu.bitcast(w2_s[...], BF16))
        return x2, _ln(x2).astype(BF16)

    def cp_y(i):
        return pltpu.make_async_copy(y_s.at[i % 2], out_hbm.at[rows(i)], sy.at[i % 2])

    def channel_mlp(i, n):
        r = rows(i)
        t_s[...] = _gelu(_dot(n, pltpu.bitcast(w3_s[...], BF16))).astype(BF16)
        h2 = _dot(t_s[...], pltpu.bitcast(w4_s[...], BF16))
        y = h_s[r, :] + mod_s[5, 0:1, :] * (r_s[r, :] + h2)
        y_s[i % 2] = y.astype(y_s.dtype)

    x2, n = token_mix(0)
    r_s[rows(0), :] = x2
    n_s[0] = n

    @pl.loop(0, NB - 1)
    def _(i):
        @pl.when(i >= 2)
        def _():
            cp_y(i - 2).wait()

        x2, n = token_mix(i + 1)
        channel_mlp(i, n_s[i % 2])
        r_s[rows(i + 1), :] = x2
        n_s[(i + 1) % 2] = n
        cp_y(i).start()

    cp_y(NB - 3).wait()
    channel_mlp(NB - 1, n_s[(NB - 1) % 2])
    cp_y(NB - 1).start()
    cp_y(NB - 2).wait()
    cp_y(NB - 1).wait()


@functools.partial(jax.jit, static_argnames=("A_seg_len",))
def pallas_adaLN_cond__memory_aug_recurrent_mem_tr__mixer_s_mlp__prompt_kernel(
    A_x, A_mem0, A_Wq, A_Wk, A_Wv, A_Wo, A_seg_len, B_x, B_w1, B_w2, B_w3, B_w4,
    c, w_mod,
):
    del B_x
    _, S, D = A_x.shape
    _, H, DH = A_Wq.shape
    M = A_mem0.shape[1]
    SEG = int(A_seg_len)
    FF = B_w3.shape[1]
    HP = H // 2
    RB = 256
    LOOK = S - (S // SEG) * (SEG - M)
    RING = LOOK + 64
    vm = pltpu.VMEM
    dma = pltpu.SemaphoreType.DMA
    scratch = [
        vm((HP, D, DH), U32), vm((HP, D, DH), U32), vm((HP, D, DH), U32),
        vm((HP, DH, D), U32),
        vm((D // 2, D), U32), vm((D // 2, D), U32),
        vm((D // 2, FF), U32), vm((FF // 2, D), U32),
        vm((6, D // 2, D), U32),
        vm((S, D), A_x.dtype), vm((S, D), F32), vm((LOOK, D), BF16),
        vm((HP, RING, 2 * DH), BF16), vm((HP, RING, 2 * DH), BF16),
        vm((1, D), c.dtype), vm((M, D), A_mem0.dtype), vm((M, D), F32),
        vm((SEG, D), BF16), vm((HP, M + SEG, 2 * DH), F32), vm((6, 8, D), F32),
        vm((D // 128, S + 16, 128), F32), vm((S, D), F32), vm((2, RB, D), BF16),
        vm((RB, FF), BF16), vm((2, RB, D), A_x.dtype),
        dma((HP,)), dma((HP,)), dma((HP,)), dma((HP,)), dma((6,)), dma((4,)),
        dma((4,)), dma((2,)),
    ]
    out = pl.pallas_call(
        functools.partial(_kernel, S=S, D=D, H=H, DH=DH, M=M, SEG=SEG, RB=RB),
        out_shape=jax.ShapeDtypeStruct((S, D), A_x.dtype),
        in_specs=[pl.BlockSpec(memory_space=pl.ANY)] * 12,
        out_specs=pl.BlockSpec(memory_space=pl.ANY),
        scratch_shapes=scratch,
        compiler_params=pltpu.CompilerParams(vmem_limit_bytes=120 * 1024 * 1024),
    )(A_x.reshape(S, D), A_mem0.reshape(M, D), A_Wq, A_Wk, A_Wv,
      A_Wo.reshape(H * DH, D), B_w1, B_w2, B_w3, B_w4, c, w_mod)
    return out.reshape(A_x.shape)
```

```python
import functools

import jax
import jax.numpy as jnp
import numpy as np
from jax import lax
import jax.experimental.pallas as pl
import jax.experimental.pallas.tpu as pltpu

F32 = jnp.float32
BF16 = jnp.bfloat16
U32 = jnp.uint32

_NN = (((1,), (0,)), ((), ()))
_NT = (((1,), (1,)), ((), ()))


def _dot(a, b, dims=_NN):
    return lax.dot_general(a, b, dims, preferred_element_type=F32)


def _ln(x):
    m = jnp.mean(x, axis=-1, keepdims=True)
    d = x - m
    v = jnp.mean(d * d, axis=-1, keepdims=True)
    return d * lax.rsqrt(v + 1e-5)


def _gelu(x):
    k0 = float(np.sqrt(2.0 / np.pi))
    k1 = float(np.sqrt(2.0 / np.pi) * 0.044715)
    hx = 0.5 * x
    return hx + hx * jnp.tanh(x * (k0 + k1 * (x * x)))


def _split_pair(ref, p):
    half = ref.shape[1] // 2
    even = ref[p, pl.ds(0, half, stride=2), :]
    odd = ref[p, pl.ds(1, half, stride=2), :]
    lo = (even & np.uint32(0xFFFF)) | (odd << 16)
    hi = (even >> 16) | (odd & np.uint32(0xFFFF0000))
    return lo, hi


def _pair_weight(lo, hi):
    return pltpu.bitcast(jnp.concatenate([lo, hi], axis=1), BF16)


def _kernel(x_hbm, mem_hbm, wq_hbm, wk_hbm, wv_hbm, wo_hbm, w1_hbm, w2_hbm,
            w3_hbm, w4_hbm, c_hbm, wm_hbm, out_hbm,
            wq_s, wkv_s, wo_s, w1_s, w2_s, w3_s, w4_s, wm_s,
            x_s, h_s, hb_s, ring_s, c_s, m0_s, mem_s, kvl_s, o_s, mod_s,
            hh_s, r_s, n_s, t_s, y_s,
            sq, skv, so, sm, sb, sx, sy,
            *, S, D, H, DH, M, SEG, RB):
    HP = H // 2
    NSEG = S // SEG
    L = M + SEG
    KVR = SEG - M
    LOOK = S - NSEG * KVR
    RING = ring_s.shape[1]
    ROFF = RING - LOOK
    D2 = D // 2
    X0 = LOOK + 32
    scale = float(DH) ** -0.5

    wq_w = wq_hbm.bitcast(U32)
    wk_w = wk_hbm.bitcast(U32)
    wv_w = wv_hbm.bitcast(U32)
    wo_w = wo_hbm.bitcast(U32)
    wm_w = wm_hbm.bitcast(U32)

    def cp_q(p):
        return pltpu.make_async_copy(wq_w.at[:, p], wq_s.at[p], sq.at[p])

    def cp_k(p):
        return pltpu.make_async_copy(wk_w.at[:, p], wkv_s.at[p], skv.at[p])

    def cp_v(p):
        return pltpu.make_async_copy(wv_w.at[:, p], wkv_s.at[HP + p], skv.at[HP + p])

    def cp_o(p):
        return pltpu.make_async_copy(
            wo_w.at[pl.ds(p * DH, DH)], wo_s.at[p], so.at[p])

    def cp_m(j):
        return pltpu.make_async_copy(
            wm_w.at[:, pl.ds(j * D, D)], wm_s.at[j], sm.at[j])

    cp_c = pltpu.make_async_copy(c_hbm, c_s, sx.at[0])
    cp_m0 = pltpu.make_async_copy(mem_hbm, m0_s, sx.at[1])
    cp_x0 = pltpu.make_async_copy(
        x_hbm.at[pl.ds(0, X0)], x_s.at[pl.ds(0, X0)], sx.at[2])
    cp_x1 = pltpu.make_async_copy(
        x_hbm.at[pl.ds(X0, S - X0)], x_s.at[pl.ds(X0, S - X0)], sx.at[3])
    cp_b = [pltpu.make_async_copy(src.bitcast(U32), dst, sb.at[i])
            for i, (src, dst) in enumerate(
                [(w1_hbm, w1_s), (w2_hbm, w2_s), (w3_hbm, w3_s), (w4_hbm, w4_s)])]

    cp_c.start()
    cp_x0.start()
    cp_m(1).start()
    cp_m(0).start()
    cp_m0.start()
    for p in range(HP):
        cp_k(p).start()
    for p in range(HP):
        cp_v(p).start()
        cp_q(p).start()
    cp_x1.start()
    for p in range(HP):
        cp_o(p).start()

    cp_c.wait()
    cf = c_s[...].astype(F32)
    sc = jnp.broadcast_to(cf * jax.nn.sigmoid(cf), (8, D))

    def mod_vec(j, add=0.0):
        cp_m(j).wait()
        mod_s[j] = _dot(sc, pltpu.bitcast(wm_s[j], BF16)) + add

    cp_x0.wait()

    @pl.loop(0, X0 // 32)
    def _(i):
        r = pl.ds(pl.multiple_of(i * 32, 32), 32)
        h_s[r, :] = _ln(x_s[r, :].astype(F32))

    mod_vec(1, 1.0)
    mod_vec(0)
    for i in range(X0 // 16):
        r = pl.ds(i * 16, 16)
        h = h_s[r, :] * mod_s[1, 0:1, :] + mod_s[0, 0:1, :]
        h_s[r, :] = h
        if i < LOOK // 16:
            hb_s[pl.ds(i * 8, 8), :] = pltpu.bitcast(h.astype(BF16), U32)

    @pl.loop(0, HP)
    def _(i):
        second = i >= HP // 2
        pq = jnp.where(second, 2 * (i - HP // 2), HP)

        @pl.when(jnp.logical_not(second))
        def _():
            cp_k(2 * i).wait()
            cp_k(2 * i + 1).wait()

        @pl.when(second)
        def _():
            for u in range(2):
                cp_v(pq + u).wait()
                cp_q(pq + u).wait()

        ws = [_split_pair(wkv_s, 2 * i + u) for u in range(2)]
        for u, (lo, hi) in enumerate(ws):
            p = 2 * i + u
            for j, w in enumerate((lo, hi)):
                y = _dot(pltpu.bitcast(hb_s[...], BF16), pltpu.bitcast(w, BF16))
                wkv_s[p, pl.ds(j * D2, D2), :] = w
                ring_s[p, pl.ds(ROFF, LOOK), pl.ds(j * DH, DH)] = y.astype(BF16)
            lo, hi = _split_pair(wq_s, pq + u)
            wq_s[pq + u, pl.ds(0, D2), :] = lo
            wq_s[pq + u, pl.ds(D2, D2), :] = hi

    for j in range(2, 6):
        cp_m(j).start()
    for cp in cp_b:
        cp.start()
    cp_m0.wait()
    mem_s[...] = m0_s[...].astype(F32)
    cp_x1.wait()
    for p in range(HP):
        cp_o(p).wait()

    KP = 128
    row = lax.broadcasted_iota(jnp.int32, (L, KP), 0)
    col = lax.broadcasted_iota(jnp.int32, (L, KP), 1)
    visible = (col < L) & ((row < M) | (col >= SEG) | (row - M >= col))
    fill = jnp.where(col < L, -1e9, -jnp.inf).astype(F32)

    def wpair(w_s, p):
        return _pair_weight(w_s[p, pl.ds(0, D2), :], w_s[p, pl.ds(D2, D2), :])

    @pl.loop(0, NSEG)
    def _(s):
        seg = pl.ds(pl.multiple_of(s * SEG, SEG), SEG)
        ahead = pl.ds(pl.multiple_of(LOOK + s * KVR, 8), KVR)
        nxt = pl.ds(pl.multiple_of(
            jnp.minimum(LOOK + (s + 1) * KVR, S - KVR), 8), KVR)
        wr = pl.ds(pl.multiple_of(lax.rem(s * KVR, RING), 8), KVR)
        rd = pl.ds(pl.multiple_of(lax.rem(s * SEG + ROFF, RING), SEG), SEG)
        kvl_s[...] = pltpu.bitcast(
            jnp.concatenate([mem_s[...], h_s[ahead, :]], axis=0).astype(BF16), U32)
        zpad = jnp.zeros((KP - L, 2 * DH), F32)

        def keys(p):
            y = _dot(pltpu.bitcast(kvl_s[...], BF16), wpair(wkv_s, p))
            ring_s[p, wr, :] = y[M:].astype(BF16)
            tail = jnp.concatenate([y[:M], zpad], axis=0).astype(BF16)
            return jnp.concatenate([ring_s[p, rd, :], tail], axis=0)

        def project(p):
            k = keys(p)
            lhs = jnp.concatenate([mem_s[...], h_s[seg, :]], axis=0)
            q = _dot(lhs, wpair(wq_s, p))
            return q, k

        def scores(qk):
            q, k = qk
            out = []
            for i in range(2):
                c = slice(i * DH, (i + 1) * DH)
                z = jnp.where(visible, _dot(q[:, c], k[:, c], _NT) * scale, fill)
                e = jnp.exp(z - jnp.max(z, axis=-1, keepdims=True))
                out.append((e, 1.0 / jnp.sum(e, axis=-1, keepdims=True)))
            return out

        def mix(p, es, v):
            for i, (e, inv) in enumerate(es):
                c = slice(i * DH, (i + 1) * DH)
                o_s[p, :, c] = _dot(e, v[:, c]) * inv

        def out_proj(p0, p1):
            lhs = jnp.concatenate([o_s[p] for p in range(p0, p1)], axis=1)
            w = jnp.concatenate([wo_s[p] for p in range(p0, p1)], axis=0)
            return _dot(lhs, pltpu.bitcast(w, BF16))

        qk, es, vs = {}, {}, {}
        acc = None
        for t in range(HP + 2):
            if t < HP:
                qk[t] = project(t)
            elif t == HP:
                h_s[nxt, :] = (_ln(x_s[nxt, :].astype(F32)) * mod_s[1, 0:1, :]
                               + mod_s[0, 0:1, :])
                acc = out_proj(0, HP // 8)
            else:
                acc = acc + out_proj(HP // 8, HP // 4)
            if 1 <= t <= HP:
                es[t - 1] = scores(qk.pop(t - 1))
                vs[t - 1] = keys(HP + t - 1)
            if t >= 2:
                mix(t - 2, es.pop(t - 2), vs.pop(t - 2))
        acc = acc + out_proj(HP // 4, HP)
        mem_s[...] = acc[:M]
        h_s[seg, :] = acc[M:]

    mod_vec(2)
    mod_vec(3)
    mod_vec(4, 1.0)
    mod_vec(5)
    for cp in cp_b:
        cp.wait()
    NB = S // RB
    CT = D // 128
    G = CT // 4
    FT = w3_s.shape[1] // 128
    SUB = RB // CT
    for j in range(CT):
        hh_s[j, pl.ds(0, 8), :] = jnp.zeros((8, 128), F32)
        hh_s[j, pl.ds(8 + S, 8), :] = jnp.zeros((8, 128), F32)

    def rows(i, off=0, n=RB):
        return pl.ds(pl.multiple_of(i * RB + off, n), n)

    def col(j, n=1):
        return pl.ds(j * 128, n * 128)

    def put_n(slot, j, v):
        n_s[slot][pl.ds(j * SUB // 2, SUB // 2), :] = pltpu.bitcast(v.astype(BF16), U32)

    def prep(i, j, slot):
        r = rows(i, j * SUB, SUB)
        x1 = x_s[r, :].astype(F32) + mod_s[2, 0:1, :] * h_s[r, :]
        hb = _ln(x1) * mod_s[4, 0:1, :] + mod_s[3, 0:1, :]
        r_s[r, :] = hb
        put_n(slot, j, _ln(hb))

    for j in range(CT):
        prep(0, j, 0)

    @pl.loop(0, NB // 2)
    def _(ii):
        for u in range(2):
            i = 2 * ii + u
            for j in range(CT):
                g = _gelu(_dot(pltpu.bitcast(n_s[u][...], BF16),
                               pltpu.bitcast(w1_s[:, col(j)], BF16)))
                hh_s[j, pl.ds(pl.multiple_of(8 + i * RB, 8), RB), :] = g
                prep(jnp.minimum(i + 1, NB - 1), j, 1 - u)

    @pl.loop(0, NB // 2)
    def _(ii):
        for u in range(2):
            i = 2 * ii + u
            for j in range(CT):
                shifted = jnp.concatenate(
                    [hh_s[k, pl.ds(8 + i * RB + (-1, 1, -2, 2)[k // G], RB), :]
                     for k in range(CT)], axis=1)
                r_s[rows(i), col(j)] += _dot(
                    shifted, pltpu.bitcast(w2_s[:, col(j)], BF16))

    def cp_y(i):
        return pltpu.make_async_copy(y_s.at[i % 2], out_hbm.at[rows(i)], sy.at[i % 2])

    for j in range(CT):
        put_n(0, j, _ln(r_s[rows(0, j * SUB, SUB), :]))

    @pl.loop(0, NB)
    def _(i):
        @pl.when(i >= 2)
        def _():
            cp_y(i - 2).wait()

        for f in range(FT):
            g = _gelu(_dot(pltpu.bitcast(n_s[0][...], BF16),
                           pltpu.bitcast(w3_s[:, col(f)], BF16)))
            t_s[:, col(f)] = pltpu.bitcast(g.astype(BF16), U32)
        r = rows(i)
        for j in range(CT):
            h2 = _dot(pltpu.bitcast(t_s[...], BF16),
                      pltpu.bitcast(w4_s[:, col(j)], BF16))
            x1 = x_s[r, col(j)].astype(F32) + mod_s[2, 0:1, col(j)] * h_s[r, col(j)]
            y = x1 + mod_s[5, 0:1, col(j)] * (r_s[r, col(j)] + h2)
            y_s[i % 2, :, col(j)] = y.astype(y_s.dtype)
            if j < CT // 2:
                for jj in (2 * j, 2 * j + 1):
                    put_n(0, jj, _ln(
                        r_s[rows(jnp.minimum(i + 1, NB - 1), jj * SUB, SUB), :]))
        cp_y(i).start()

    cp_y(NB - 2).wait()
    cp_y(NB - 1).wait()


@functools.partial(jax.jit, static_argnames=("A_seg_len",))
def pallas_adaLN_cond__memory_aug_recurrent_mem_tr__mixer_s_mlp__prompt_kernel(
    A_x, A_mem0, A_Wq, A_Wk, A_Wv, A_Wo, A_seg_len, B_x, B_w1, B_w2, B_w3, B_w4,
    c, w_mod,
):
    del B_x
    _, S, D = A_x.shape
    _, H, DH = A_Wq.shape
    M = A_mem0.shape[1]
    SEG = int(A_seg_len)
    FF = B_w3.shape[1]
    HP = H // 2
    RB = 256
    LOOK = S - (S // SEG) * (SEG - M)
    RING = LOOK + 64
    vm = pltpu.VMEM
    dma = pltpu.SemaphoreType.DMA
    scratch = [
        vm((HP + 2, D, DH), U32), vm((2 * HP, D, DH), U32), vm((HP, DH, D), U32),
        vm((D // 2, D), U32), vm((D // 2, D), U32),
        vm((D // 2, FF), U32), vm((FF // 2, D), U32),
        vm((6, D // 2, D), U32),
        vm((S, D), A_x.dtype), vm((S, D), F32), vm((LOOK // 2, D), U32),
        vm((2 * HP, RING, 2 * DH), BF16),
        vm((1, D), c.dtype), vm((M, D), A_mem0.dtype), vm((M, D), F32),
        vm((SEG // 2, D), U32), vm((HP, M + SEG, 2 * DH), F32), vm((6, 8, D), F32),
        vm((D // 128, S + 16, 128), F32), vm((S, D), F32),
        [vm((RB // 2, D), U32), vm((RB // 2, D), U32)],
        vm((RB // 2, FF), U32), vm((2, RB, D), A_x.dtype),
        dma((HP,)), dma((2 * HP,)), dma((HP,)), dma((6,)), dma((4,)),
        dma((4,)), dma((2,)),
    ]
    out = pl.pallas_call(
        functools.partial(_kernel, S=S, D=D, H=H, DH=DH, M=M, SEG=SEG, RB=RB),
        out_shape=jax.ShapeDtypeStruct((S, D), A_x.dtype),
        in_specs=[pl.BlockSpec(memory_space=pl.ANY)] * 12,
        out_specs=pl.BlockSpec(memory_space=pl.ANY),
        scratch_shapes=scratch,
        compiler_params=pltpu.CompilerParams(vmem_limit_bytes=120 * 1024 * 1024),
    )(A_x.reshape(S, D), A_mem0.reshape(M, D), A_Wq, A_Wk, A_Wv,
      A_Wo.reshape(H * DH, D), B_w1, B_w2, B_w3, B_w4, c, w_mod)
    return out.reshape(A_x.shape)
```

```python
import functools

import jax
import jax.numpy as jnp
import numpy as np
from jax import lax
import jax.experimental.pallas as pl
import jax.experimental.pallas.tpu as pltpu

F32 = jnp.float32
BF16 = jnp.bfloat16
U32 = jnp.uint32

_NN = (((1,), (0,)), ((), ()))
_NT = (((1,), (1,)), ((), ()))


def _dot(a, b, dims=_NN):
    return lax.dot_general(a, b, dims, preferred_element_type=F32)


def _ln(x):
    m = jnp.mean(x, axis=-1, keepdims=True)
    d = x - m
    v = jnp.mean(d * d, axis=-1, keepdims=True)
    return d * lax.rsqrt(v + 1e-5)


def _gelu(x):
    k0 = float(np.sqrt(2.0 / np.pi))
    k1 = float(np.sqrt(2.0 / np.pi) * 0.044715)
    hx = 0.5 * x
    return hx + hx * jnp.tanh(x * (k0 + k1 * (x * x)))


_CH = 64


def _repack(ref, p, lo_c, hi_c):
    for c in range(lo_c, hi_c):
        even = ref[p, pl.ds(c * _CH, _CH // 2, stride=2), :]
        odd = ref[p, pl.ds(c * _CH + 1, _CH // 2, stride=2), :]
        ref[p, pl.ds(c * _CH, _CH // 2), :] = (even & np.uint32(0xFFFF)) | (odd << 16)
        ref[p, pl.ds(c * _CH + _CH // 2, _CH // 2), :] = (
            (even >> 16) | (odd & np.uint32(0xFFFF0000)))


def _head_words(ref, p, j):
    return jnp.concatenate(
        [ref[p, pl.ds(c * _CH + j * (_CH // 2), _CH // 2), :]
         for c in range(ref.shape[1] // _CH)], axis=0)


def _kernel(x_hbm, mem_hbm, wq_hbm, wk_hbm, wv_hbm, wo_hbm, w1_hbm, w2_hbm,
            w3_hbm, w4_hbm, c_hbm, wm_hbm, out_hbm,
            wq_s, wkv_s, wo_s, w1_s, w2_s, w3_s, w4_s, wm_s,
            x_s, h_s, hb_s, ring_s, c_s, m0_s, ql_s, kvl_s, o_s, acc_s, mod_s,
            hh_s, r_s, nb_s, n_s, t_s, y_s,
            sq, skv, so, sm, sb, sx, sy,
            *, S, D, H, DH, M, SEG, RB):
    HP = H // 2
    NSEG = S // SEG
    L = M + SEG
    KVR = SEG - M
    LOOK = S - NSEG * KVR
    RING = ring_s.shape[1]
    ROFF = RING - LOOK
    D2 = D // 2
    X0 = LOOK + 32
    scale = float(DH) ** -0.5

    wq_w = wq_hbm.bitcast(U32)
    wk_w = wk_hbm.bitcast(U32)
    wv_w = wv_hbm.bitcast(U32)
    wo_w = wo_hbm.bitcast(U32)
    wm_w = wm_hbm.bitcast(U32)

    def cp_q(p):
        return pltpu.make_async_copy(wq_w.at[:, p], wq_s.at[p], sq.at[p])

    def cp_k(p):
        return pltpu.make_async_copy(wk_w.at[:, p], wkv_s.at[p], skv.at[p])

    def cp_v(p):
        return pltpu.make_async_copy(wv_w.at[:, p], wkv_s.at[HP + p], skv.at[HP + p])

    def cp_o(p):
        return pltpu.make_async_copy(
            wo_w.at[pl.ds(p * DH, DH)], wo_s.at[p], so.at[p])

    def cp_m(j):
        return pltpu.make_async_copy(
            wm_w.at[:, pl.ds(j * D, D)], wm_s.at[j], sm.at[j])

    cp_c = pltpu.make_async_copy(c_hbm, c_s, sx.at[0])
    cp_m0 = pltpu.make_async_copy(mem_hbm, m0_s, sx.at[1])
    cp_x0 = pltpu.make_async_copy(
        x_hbm.at[pl.ds(0, X0)], x_s.at[pl.ds(0, X0)], sx.at[2])
    cp_x1 = pltpu.make_async_copy(
        x_hbm.at[pl.ds(X0, S - X0)], x_s.at[pl.ds(X0, S - X0)], sx.at[3])
    cp_b = [pltpu.make_async_copy(src.bitcast(U32), dst, sb.at[i])
            for i, (src, dst) in enumerate(
                [(w1_hbm, w1_s), (w2_hbm, w2_s), (w3_hbm, w3_s), (w4_hbm, w4_s)])]

    cp_c.start()
    cp_x0.start()
    cp_m(1).start()
    cp_m(0).start()
    cp_m0.start()
    for p in range(HP):
        cp_k(p).start()
    for p in range(HP):
        cp_v(p).start()
        cp_q(p).start()
    cp_x1.start()
    for p in range(HP):
        cp_o(p).start()

    cp_c.wait()
    cf = c_s[...].astype(F32)
    sc = jnp.broadcast_to(cf * jax.nn.sigmoid(cf), (8, D))

    def mod_vec(j, add=0.0):
        cp_m(j).wait()
        mod_s[j] = _dot(sc, pltpu.bitcast(wm_s[j], BF16)) + add

    def mod(j, n, c=slice(None)):
        return jnp.concatenate([mod_s[j, :, c]] * (n // 8), axis=0)

    cp_x0.wait()

    @pl.loop(0, X0 // 32)
    def _(i):
        r = pl.ds(pl.multiple_of(i * 32, 32), 32)
        h_s[r, :] = _ln(x_s[r, :].astype(F32))

    mod_vec(1, 1.0)
    mod_vec(0)
    for i in range(X0 // 16):
        r = pl.ds(i * 16, 16)
        h = h_s[r, :] * mod(1, 16) + mod(0, 16)
        h_s[r, :] = h
        if i < LOOK // 16:
            hb_s[pl.ds(i * 8, 8), :] = pltpu.bitcast(h.astype(BF16), U32)

    NC = D // _CH
    cp_k(0).wait()
    _repack(wkv_s, 0, 0, NC)

    @pl.loop(0, HP)
    def _(i):
        second = i >= HP // 2
        pq = jnp.where(second, 2 * (i - HP // 2), HP)
        for u in range(2):
            nxt = 2 * i + u + 1

            @pl.when(nxt < HP)
            def _():
                cp_k(nxt).wait()

            @pl.when((nxt >= HP) & (nxt < 2 * HP))
            def _():
                cp_v(nxt - HP).wait()

        @pl.when(second)
        def _():
            for u in range(2):
                cp_q(pq + u).wait()

        for u in range(2):
            p = 2 * i + u
            for j in range(2):
                w = pltpu.bitcast(_head_words(wkv_s, p, j), BF16)
                y = _dot(pltpu.bitcast(hb_s[...], BF16), w)
                ring_s[p, pl.ds(ROFF, LOOK), pl.ds(j * DH, DH)] = y.astype(BF16)
                if j == 0:
                    _repack(wkv_s, p + 1, 0, NC)
                    _repack(wq_s, pq + u, 0, NC)

    for j in range(2, 6):
        cp_m(j).start()
    for cp in cp_b:
        cp.start()
    cp_m0.wait()
    ql_s[pl.ds(0, M), :] = m0_s[...].astype(F32)
    cp_x1.wait()
    for p in range(HP):
        cp_o(p).wait()

    KP = 128
    row = lax.broadcasted_iota(jnp.int32, (L, KP), 0)
    col = lax.broadcasted_iota(jnp.int32, (L, KP), 1)
    visible = (col < L) & ((row < M) | (col >= SEG) | (row - M >= col))
    fill = jnp.where(col < L, -1e9, -jnp.inf).astype(F32)

    def wpair(w_s, p):
        return pltpu.bitcast(jnp.concatenate(
            [_head_words(w_s, p, 0), _head_words(w_s, p, 1)], axis=1), BF16)

    def prep(g):
        r = pl.ds(pl.multiple_of(g * SEG, SEG), SEG)
        x1 = x_s[r, :].astype(F32) + mod(2, SEG) * h_s[r, :]
        hb = _ln(x1) * mod(4, SEG) + mod(3, SEG)
        r_s[r, :] = hb
        nb_s[pl.ds(pl.multiple_of(g * (SEG // 2), SEG // 2), SEG // 2), :] = (
            pltpu.bitcast(_ln(hb).astype(BF16), U32))

    LAG = 3
    for j in range(2, 5):
        mod_s[j] = jnp.zeros((8, D), F32)

    @pl.loop(0, NSEG)
    def _(s):
        @pl.when(s == LAG)
        def _():
            mod_vec(2)
            mod_vec(3)
            mod_vec(4, 1.0)
            mod_vec(5)

        seg = pl.ds(pl.multiple_of(s * SEG, SEG), SEG)
        ahead = pl.ds(pl.multiple_of(LOOK + s * KVR, 8), KVR)
        nxt = pl.ds(pl.multiple_of(
            jnp.minimum(LOOK + (s + 1) * KVR, S - KVR), 8), KVR)
        wr = pl.ds(pl.multiple_of(lax.rem(s * KVR, RING), 8), KVR)
        rd = pl.ds(pl.multiple_of(lax.rem(s * SEG + ROFF, RING), SEG), SEG)
        kvl_s[...] = pltpu.bitcast(
            jnp.concatenate([ql_s[pl.ds(0, M), :], h_s[ahead, :]], axis=0).astype(BF16),
            U32)
        ql_s[pl.ds(M, SEG), :] = h_s[seg, :]
        prep(jnp.maximum(s - LAG, 0))
        h_s[nxt, :] = _ln(x_s[nxt, :].astype(F32)) * mod(1, KVR) + mod(0, KVR)
        zpad = jnp.zeros((KP - L, 2 * DH), F32)

        def keys(p):
            y = _dot(pltpu.bitcast(kvl_s[...], BF16), wpair(wkv_s, p))
            ring_s[p, wr, :] = y[M:].astype(BF16)
            tail = jnp.concatenate([y[:M], zpad], axis=0).astype(BF16)
            return jnp.concatenate([ring_s[p, rd, :], tail], axis=0)

        def project(p):
            k = keys(p)
            q = _dot(ql_s[...], wpair(wq_s, p))
            return q, k

        def scores(qk):
            q, k = qk
            out = []
            for i in range(2):
                c = slice(i * DH, (i + 1) * DH)
                z = jnp.where(visible, _dot(q[:, c], k[:, c], _NT) * scale, fill)
                e = jnp.exp(z - jnp.max(z, axis=-1, keepdims=True))
                out.append((e, 1.0 / jnp.sum(e, axis=-1, keepdims=True)))
            return out

        def mix(p, es, v):
            for i, (e, inv) in enumerate(es):
                c = slice(i * DH, (i + 1) * DH)
                o_s[p, :, c] = _dot(e, v[:, c]) * inv

        def out_proj(p0, p1, j):
            c = pl.ds(j * 128, 128)
            lhs = jnp.concatenate([o_s[p] for p in range(p0, p1)], axis=1)
            w = jnp.concatenate([wo_s[p, :, c] for p in range(p0, p1)], axis=0)
            return _dot(lhs, pltpu.bitcast(w, BF16))

        qk, es, vs = {}, {}, {}
        CT = D // 128
        for t in range(HP + 2):
            if t < HP:
                qk[t] = project(t)
            else:
                for j in range((t - HP) * CT // 2, (t - HP + 1) * CT // 2):
                    acc_s[:, pl.ds(j * 128, 128)] = out_proj(0, HP // 2, j)
            if 1 <= t <= HP:
                es[t - 1] = scores(qk.pop(t - 1))
                vs[t - 1] = keys(HP + t - 1)
            if t >= 2:
                mix(t - 2, es.pop(t - 2), vs.pop(t - 2))
        for j in range(CT):
            c = pl.ds(j * 128, 128)
            acc = acc_s[:, c] + out_proj(HP // 2, HP, j)
            ql_s[pl.ds(0, M), c] = acc[:M]
            h_s[seg, c] = acc[M:]

    for g in range(NSEG - LAG, NSEG):
        prep(g)
    for cp in cp_b:
        cp.wait()
    NB = S // RB
    CT = D // 128
    G = CT // 4
    FT = w3_s.shape[1] // 128
    SUB = RB // CT
    for j in range(CT):
        hh_s[j, pl.ds(0, 8), :] = jnp.zeros((8, 128), F32)
        hh_s[j, pl.ds(8 + S, 8), :] = jnp.zeros((8, 128), F32)

    def rows(i, off=0, n=RB):
        return pl.ds(pl.multiple_of(i * RB + off, n), n)

    def col(j, n=1):
        return pl.ds(j * 128, n * 128)

    def put_n(j, v):
        n_s[pl.ds(j * SUB // 2, SUB // 2), :] = pltpu.bitcast(v.astype(BF16), U32)

    @pl.loop(0, NB // 2)
    def _(i):
        for j in range(CT):
            g = _gelu(_dot(pltpu.bitcast(nb_s[rows(i), :], BF16),
                           pltpu.bitcast(w1_s[:, col(j)], BF16)))
            hh_s[j, pl.ds(pl.multiple_of(8 + i * 2 * RB, 8), 2 * RB), :] = g

    @pl.loop(0, NB // 2)
    def _(ii):
        for u in range(2):
            i = 2 * ii + u
            for j in range(CT):
                shifted = jnp.concatenate(
                    [hh_s[k, pl.ds(8 + i * RB + (-1, 1, -2, 2)[k // G], RB), :]
                     for k in range(CT)], axis=1)
                r_s[rows(i), col(j)] += _dot(
                    shifted, pltpu.bitcast(w2_s[:, col(j)], BF16))

    def cp_y(i):
        return pltpu.make_async_copy(y_s.at[i % 2], out_hbm.at[rows(i)], sy.at[i % 2])

    for j in range(CT):
        put_n(j, _ln(r_s[rows(0, j * SUB, SUB), :]))

    @pl.loop(0, NB)
    def _(i):
        @pl.when(i >= 2)
        def _():
            cp_y(i - 2).wait()

        for f in range(FT):
            g = _gelu(_dot(pltpu.bitcast(n_s[...], BF16),
                           pltpu.bitcast(w3_s[:, col(f)], BF16)))
            t_s[:, col(f)] = pltpu.bitcast(g.astype(BF16), U32)
        r = rows(i)
        for j in range(CT):
            h2 = _dot(pltpu.bitcast(t_s[...], BF16),
                      pltpu.bitcast(w4_s[:, col(j)], BF16))
            x1 = x_s[r, col(j)].astype(F32) + mod(2, RB, col(j)) * h_s[r, col(j)]
            y = x1 + mod(5, RB, col(j)) * (r_s[r, col(j)] + h2)
            y_s[i % 2, :, col(j)] = y.astype(y_s.dtype)
            if j < CT // 2:
                for jj in (2 * j, 2 * j + 1):
                    put_n(jj, _ln(
                        r_s[rows(jnp.minimum(i + 1, NB - 1), jj * SUB, SUB), :]))
        cp_y(i).start()

    cp_y(NB - 2).wait()
    cp_y(NB - 1).wait()


@functools.partial(jax.jit, static_argnames=("A_seg_len",))
def pallas_adaLN_cond__memory_aug_recurrent_mem_tr__mixer_s_mlp__prompt_kernel(
    A_x, A_mem0, A_Wq, A_Wk, A_Wv, A_Wo, A_seg_len, B_x, B_w1, B_w2, B_w3, B_w4,
    c, w_mod,
):
    del B_x
    _, S, D = A_x.shape
    _, H, DH = A_Wq.shape
    M = A_mem0.shape[1]
    SEG = int(A_seg_len)
    FF = B_w3.shape[1]
    HP = H // 2
    RB = 256
    LOOK = S - (S // SEG) * (SEG - M)
    RING = LOOK + 64
    vm = pltpu.VMEM
    dma = pltpu.SemaphoreType.DMA
    scratch = [
        vm((HP + 2, D, DH), U32), vm((2 * HP + 1, D, DH), U32), vm((HP, DH, D), U32),
        vm((D // 2, D), U32), vm((D // 2, D), U32),
        vm((D // 2, FF), U32), vm((FF // 2, D), U32),
        vm((6, D // 2, D), U32),
        vm((S, D), A_x.dtype), vm((S, D), F32), vm((LOOK // 2, D), U32),
        vm((2 * HP, RING, 2 * DH), BF16),
        vm((1, D), c.dtype), vm((M, D), A_mem0.dtype), vm((M + SEG, D), F32),
        vm((SEG // 2, D), U32), vm((HP, M + SEG, 2 * DH), F32),
        vm((M + SEG, D), F32), vm((6, 8, D), F32),
        vm((D // 128, S + 16, 128), F32), vm((S, D), F32),
        vm((S // 2, D), U32), vm((RB // 2, D), U32),
        vm((RB // 2, FF), U32), vm((2, RB, D), A_x.dtype),
        dma((HP,)), dma((2 * HP,)), dma((HP,)), dma((6,)), dma((4,)),
        dma((4,)), dma((2,)),
    ]
    out = pl.pallas_call(
        functools.partial(_kernel, S=S, D=D, H=H, DH=DH, M=M, SEG=SEG, RB=RB),
        out_shape=jax.ShapeDtypeStruct((S, D), A_x.dtype),
        in_specs=[pl.BlockSpec(memory_space=pl.ANY)] * 12,
        out_specs=pl.BlockSpec(memory_space=pl.ANY),
        scratch_shapes=scratch,
        compiler_params=pltpu.CompilerParams(vmem_limit_bytes=120 * 1024 * 1024),
    )(A_x.reshape(S, D), A_mem0.reshape(M, D), A_Wq, A_Wk, A_Wv,
      A_Wo.reshape(H * DH, D), B_w1, B_w2, B_w3, B_w4, c, w_mod)
    return out.reshape(A_x.shape)
```

```python
import functools

import jax
import jax.numpy as jnp
import numpy as np
from jax import lax
import jax.experimental.pallas as pl
import jax.experimental.pallas.tpu as pltpu

F32 = jnp.float32
BF16 = jnp.bfloat16
U32 = jnp.uint32

_NN = (((1,), (0,)), ((), ()))
_NT = (((1,), (1,)), ((), ()))


def _dot(a, b, dims=_NN):
    return lax.dot_general(a, b, dims, preferred_element_type=F32)


def _ln(x):
    m = jnp.mean(x, axis=-1, keepdims=True)
    d = x - m
    v = jnp.mean(d * d, axis=-1, keepdims=True)
    return d * lax.rsqrt(v + 1e-5)


def _gelu(x):
    k0 = float(np.sqrt(2.0 / np.pi))
    k1 = float(np.sqrt(2.0 / np.pi) * 0.044715)
    hx = 0.5 * x
    return hx + hx * jnp.tanh(x * (k0 + k1 * (x * x)))


_CH = 64


def _repack(ref, p, lo_c, hi_c):
    for c in range(lo_c, hi_c):
        even = ref[p, pl.ds(c * _CH, _CH // 2, stride=2), :]
        odd = ref[p, pl.ds(c * _CH + 1, _CH // 2, stride=2), :]
        ref[p, pl.ds(c * _CH, _CH // 2), :] = (even & np.uint32(0xFFFF)) | (odd << 16)
        ref[p, pl.ds(c * _CH + _CH // 2, _CH // 2), :] = (
            (even >> 16) | (odd & np.uint32(0xFFFF0000)))


def _head_words(ref, p, j):
    return jnp.concatenate(
        [ref[p, pl.ds(c * _CH + j * (_CH // 2), _CH // 2), :]
         for c in range(ref.shape[1] // _CH)], axis=0)


def _words(x):
    return pltpu.bitcast(x.astype(BF16), U32)


def _strassen_lhs(a11, a12, a21, a22):
    return (a11 + a22, a21 + a22, a11, a22, a11 + a12, a21 - a11, a12 - a22)


def _strassen_rhs_sums(b11, b12, b21, b22):
    return (b11 + b22, b12 - b22, b21 - b11, b11 + b12, b21 + b22)


def _strassen(prod):
    m0, m1 = prod(0), prod(1)
    c22 = m0 - m1
    m3 = prod(3)
    c11 = m0 + m3
    c21 = m1 + m3
    m2 = prod(2)
    c22 = c22 + m2
    m4 = prod(4)
    c12 = m2 + m4
    c11 = c11 - m4
    c22 = c22 + prod(5)
    c11 = c11 + prod(6)
    return c11, c12, c21, c22


def _kernel(x_hbm, mem_hbm, wq_hbm, wk_hbm, wv_hbm, wo_hbm, w1_hbm, w2_hbm,
            w3_hbm, w4_hbm, c_hbm, wm_hbm, out_hbm,
            w_s, wo_s, w3_s, w4_s, wm_s,
            x_s, h_s, hb_s, ring_s, c_s, m0_s, ql_s, kvl_s, o_s, acc_s, mod_s,
            hh_s, r_s, nb_s, n_s, t_s, y_s,
            sq, skv, so, sm, sb, sx, sy,
            *, S, D, H, DH, M, SEG, RB):
    HP = H // 2
    NSEG = S // SEG
    L = M + SEG
    KVR = SEG - M
    LOOK = S - NSEG * KVR
    RING = ring_s.shape[1]
    ROFF = RING - LOOK
    D2 = D // 2
    X0 = LOOK + 32
    Q0 = 2 * HP + 1
    T0 = Q0 + HP + 2
    scale = float(DH) ** -0.5

    wq_w = wq_hbm.bitcast(U32)
    wk_w = wk_hbm.bitcast(U32)
    wv_w = wv_hbm.bitcast(U32)
    wo_w = wo_hbm.bitcast(U32)
    wm_w = wm_hbm.bitcast(U32)

    def cp_q(p):
        return pltpu.make_async_copy(wq_w.at[:, p], w_s.at[Q0 + p], sq.at[p])

    def cp_k(p):
        return pltpu.make_async_copy(wk_w.at[:, p], w_s.at[p], skv.at[p])

    def cp_v(p):
        return pltpu.make_async_copy(wv_w.at[:, p], w_s.at[HP + p], skv.at[HP + p])

    def cp_o(p):
        return pltpu.make_async_copy(
            wo_w.at[pl.ds(p * DH, DH)], wo_s.at[p], so.at[p])

    def cp_m(j):
        return pltpu.make_async_copy(
            wm_w.at[:, pl.ds(j * D, D)], wm_s.at[j], sm.at[j])

    cp_c = pltpu.make_async_copy(c_hbm, c_s, sx.at[0])
    cp_m0 = pltpu.make_async_copy(mem_hbm, m0_s, sx.at[1])
    cp_x0 = pltpu.make_async_copy(
        x_hbm.at[pl.ds(0, X0)], x_s.at[pl.ds(0, X0)], sx.at[2])
    cp_x1 = pltpu.make_async_copy(
        x_hbm.at[pl.ds(X0, S - X0)], x_s.at[pl.ds(X0, S - X0)], sx.at[3])
    CT = D // 128

    def mix_tile(k, j):
        return w_s.at[T0 + j, pl.ds(k * D2, D2)]

    cp_b = [(src.bitcast(U32).at[:, pl.ds(j * 128, 128)], mix_tile(k, j))
            for k, src in enumerate((w1_hbm, w2_hbm)) for j in range(CT)]
    cp_b += [(w3_hbm.bitcast(U32), w3_s), (w4_hbm.bitcast(U32), w4_s)]
    cp_b = [pltpu.make_async_copy(src, dst, sb.at[i])
            for i, (src, dst) in enumerate(cp_b)]

    cp_c.start()
    cp_x0.start()
    cp_m(1).start()
    cp_m(0).start()
    cp_m0.start()
    for p in range(HP):
        cp_k(p).start()
    for p in range(HP):
        cp_v(p).start()
        cp_q(p).start()
    cp_x1.start()
    for p in range(HP):
        cp_o(p).start()

    cp_c.wait()
    cf = c_s[...].astype(F32)
    sc = jnp.broadcast_to(cf * jax.nn.sigmoid(cf), (8, D))

    def mod_vec(j, add=0.0):
        cp_m(j).wait()
        mod_s[j] = _dot(sc, pltpu.bitcast(wm_s[j], BF16)) + add

    def mod(j, n, c=slice(None)):
        return jnp.concatenate([mod_s[j, :, c]] * (n // 8), axis=0)

    cp_x0.wait()

    @pl.loop(0, X0 // 32)
    def _(i):
        r = pl.ds(pl.multiple_of(i * 32, 32), 32)
        h_s[r, :] = _ln(x_s[r, :].astype(F32))

    mod_vec(1, 1.0)
    mod_vec(0)
    for i in range(X0 // 16):
        r = pl.ds(i * 16, 16)
        h = h_s[r, :] * mod(1, 16) + mod(0, 16)
        h_s[r, :] = h
        if i < LOOK // 16:
            hb_s[pl.ds(i * 8, 8), :] = pltpu.bitcast(h.astype(BF16), U32)

    NC = D // _CH
    cp_k(0).wait()
    _repack(w_s, 0, 0, NC)

    @pl.loop(0, HP)
    def _(i):
        second = i >= HP // 2
        pq = jnp.where(second, 2 * (i - HP // 2), HP)
        for u in range(2):
            nxt = 2 * i + u + 1

            @pl.when(nxt < HP)
            def _():
                cp_k(nxt).wait()

            @pl.when((nxt >= HP) & (nxt < 2 * HP))
            def _():
                cp_v(nxt - HP).wait()

        @pl.when(second)
        def _():
            for u in range(2):
                cp_q(pq + u).wait()

        for u in range(2):
            p = 2 * i + u
            for j in range(2):
                w = pltpu.bitcast(_head_words(w_s, p, j), BF16)
                y = _dot(pltpu.bitcast(hb_s[...], BF16), w)
                ring_s[p, pl.ds(ROFF, LOOK), pl.ds(j * DH, DH)] = y.astype(BF16)
                if j == 0:
                    _repack(w_s, p + 1, 0, NC)
                    _repack(w_s, Q0 + pq + u, 0, NC)

    for j in range(2, 6):
        cp_m(j).start()
    for cp in cp_b:
        cp.start()
    cp_m0.wait()
    ql_s[pl.ds(0, M), :] = m0_s[...].astype(F32)
    cp_x1.wait()
    for p in range(HP):
        cp_o(p).wait()

    KP = 128
    row = lax.broadcasted_iota(jnp.int32, (L, KP), 0)
    col = lax.broadcasted_iota(jnp.int32, (L, KP), 1)
    visible = (col < L) & ((row < M) | (col >= SEG) | (row - M >= col))
    fill = jnp.where(col < L, -1e9, -jnp.inf).astype(F32)

    def wpair(p):
        return pltpu.bitcast(jnp.concatenate(
            [_head_words(w_s, p, 0), _head_words(w_s, p, 1)], axis=1), BF16)

    def prep(g):
        r = pl.ds(pl.multiple_of(g * SEG, SEG), SEG)
        x1 = x_s[r, :].astype(F32) + mod(2, SEG) * h_s[r, :]
        hb = _ln(x1) * mod(4, SEG) + mod(3, SEG)
        r_s[r, :] = hb
        nb_s[pl.ds(pl.multiple_of(g * (SEG // 2), SEG // 2), SEG // 2), :] = (
            pltpu.bitcast(_ln(hb).astype(BF16), U32))

    LAG = 3
    for j in range(2, 5):
        mod_s[j] = jnp.zeros((8, D), F32)

    @pl.loop(0, NSEG)
    def _(s):
        @pl.when(s == LAG)
        def _():
            mod_vec(2)
            mod_vec(3)
            mod_vec(4, 1.0)
            mod_vec(5)

        seg = pl.ds(pl.multiple_of(s * SEG, SEG), SEG)
        ahead = pl.ds(pl.multiple_of(LOOK + s * KVR, 8), KVR)
        nxt = pl.ds(pl.multiple_of(
            jnp.minimum(LOOK + (s + 1) * KVR, S - KVR), 8), KVR)
        wr = pl.ds(pl.multiple_of(lax.rem(s * KVR, RING), 8), KVR)
        rd = pl.ds(pl.multiple_of(lax.rem(s * SEG + ROFF, RING), SEG), SEG)
        kvl_s[...] = pltpu.bitcast(
            jnp.concatenate([ql_s[pl.ds(0, M), :], h_s[ahead, :]], axis=0).astype(BF16),
            U32)
        ql_s[pl.ds(M, SEG), :] = h_s[seg, :]
        prep(jnp.maximum(s - LAG, 0))
        h_s[nxt, :] = _ln(x_s[nxt, :].astype(F32)) * mod(1, KVR) + mod(0, KVR)
        zpad = jnp.zeros((KP - L, 2 * DH), F32)

        def keys(p):
            y = _dot(pltpu.bitcast(kvl_s[...], BF16), wpair(p))
            ring_s[p, wr, :] = y[M:].astype(BF16)
            tail = jnp.concatenate([y[:M], zpad], axis=0).astype(BF16)
            return jnp.concatenate([ring_s[p, rd, :], tail], axis=0)

        def project(p):
            k = keys(p)
            q = _dot(ql_s[...], wpair(Q0 + p))
            return q, k

        def scores(qk):
            q, k = qk
            out = []
            for i in range(2):
                c = slice(i * DH, (i + 1) * DH)
                z = jnp.where(visible, _dot(q[:, c], k[:, c], _NT) * scale, fill)
                e = jnp.exp(z - jnp.max(z, axis=-1, keepdims=True))
                out.append((e, 1.0 / jnp.sum(e, axis=-1, keepdims=True)))
            return out

        def mix(p, es, v):
            for i, (e, inv) in enumerate(es):
                c = slice(i * DH, (i + 1) * DH)
                o_s[p, :, c] = _dot(e, v[:, c]) * inv

        def out_proj(p0, p1, j):
            c = pl.ds(j * 128, 128)
            lhs = jnp.concatenate([o_s[p] for p in range(p0, p1)], axis=1)
            w = jnp.concatenate([wo_s[p, :, c] for p in range(p0, p1)], axis=0)
            return _dot(lhs, pltpu.bitcast(w, BF16))

        qk, es, vs = {}, {}, {}
        for t in range(HP + 2):
            if t < HP:
                qk[t] = project(t)
            else:
                for j in range((t - HP) * CT // 2, (t - HP + 1) * CT // 2):
                    acc_s[:, pl.ds(j * 128, 128)] = out_proj(0, HP // 2, j)
            if 1 <= t <= HP:
                es[t - 1] = scores(qk.pop(t - 1))
                vs[t - 1] = keys(HP + t - 1)
            if t >= 2:
                mix(t - 2, es.pop(t - 2), vs.pop(t - 2))
        for j in range(CT):
            c = pl.ds(j * 128, 128)
            acc = acc_s[:, c] + out_proj(HP // 2, HP, j)
            ql_s[pl.ds(0, M), c] = acc[:M]
            h_s[seg, c] = acc[M:]

    for g in range(NSEG - LAG, NSEG):
        prep(g)
    for cp in cp_b:
        cp.wait()
    NB = S // RB
    G = CT // 4
    FT = w3_s.shape[1] // 128
    SUB = RB // CT
    for j in range(CT):
        hh_s[j, pl.ds(0, 8), :] = jnp.zeros((8, 128), F32)
        hh_s[j, pl.ds(8 + S, 8), :] = jnp.zeros((8, 128), F32)

    def rows(i, off=0, n=RB):
        return pl.ds(pl.multiple_of(i * RB + off, n), n)

    def col(j, n=1):
        return pl.ds(j * 128, n * 128)

    FH, CH, RH = FT // 2, CT // 2, RB // 2
    NI = NB // 2
    K3, K4 = D // 4, FT * 32

    def sum3(k, f):
        return 2 * f + k // 4, (k % 4) * K3

    def sums(ref, r0, half, c0, c1):
        w = [ref[pl.ds(r0 + dr, 16), c] for dr in (0, half) for c in (c0, c1)]
        lo = _strassen_rhs_sums(*[pltpu.bitcast(v << 16, F32) for v in w])
        hi = _strassen_rhs_sums(
            *[pltpu.bitcast(v & np.uint32(0xFFFF0000), F32) for v in w])
        return [pltpu.bitcast(pltpu.pack_elementwise([a, b], packed_dtype=BF16), U32)
                for a, b in zip(lo, hi)]

    def make3(i, f):
        for u in range(K3 // NI // 16):
            r0 = pl.multiple_of(i * (K3 // NI) + u * 16, 8)
            for k, v in enumerate(sums(w3_s, r0, K3, col(f), col(FH + f))):
                slot, off = sum3(k, f)
                w_s[slot, pl.ds(off + r0, 16), :] = v

    def make4(i, u):
        r0 = pl.multiple_of(i * (K4 // NI) + u * 16, 8)
        for j in range(CH):
            for k, v in enumerate(sums(w4_s, r0, K4, col(j), col(CH + j))):
                w_s[2 * FH + 5 * j + k, pl.ds(r0, 16), :] = v

    def rhs3(m, f):
        if m == 1:
            return w3_s[pl.ds(0, K3), col(f)]
        if m == 4:
            return w3_s[pl.ds(K3, K3), col(FH + f)]
        slot, off = sum3((0, None, 1, 2, None, 3, 4)[m], f)
        return w_s[slot, pl.ds(off, K3), :]

    def rhs4(m, j):
        if m == 1:
            return w4_s[pl.ds(0, K4), col(j)]
        if m == 4:
            return w4_s[pl.ds(K4, K4), col(CH + j)]
        return w_s[2 * FH + 5 * j + (0, None, 1, 2, None, 3, 4)[m], pl.ds(0, K4), :]

    @pl.loop(0, NI)
    def _(i):
        for j in range(CT):
            g = _gelu(_dot(pltpu.bitcast(nb_s[rows(i), :], BF16),
                           pltpu.bitcast(mix_tile(0, j)[...], BF16)))
            hh_s[j, pl.ds(pl.multiple_of(8 + i * 2 * RB, 8), 2 * RB), :] = g

    @pl.loop(0, NI)
    def _(ii):
        for u in range(2):
            i = 2 * ii + u
            for j in range(CT):
                shifted = jnp.concatenate(
                    [hh_s[k, pl.ds(8 + i * RB + (-1, 1, -2, 2)[k // G], RB), :]
                     for k in range(CT)], axis=1)
                r_s[rows(i), col(j)] += _dot(
                    shifted, pltpu.bitcast(mix_tile(1, j)[...], BF16))
                if u * CT + j < K4 // NI // 16:
                    make3(ii, u * CT + j)
                    make4(ii, u * CT + j)

    def cp_y(i):
        return pltpu.make_async_copy(y_s.at[i % 2], out_hbm.at[rows(i)], sy.at[i % 2])

    def norm2(i, j):
        top = _ln(r_s[rows(i, j * 16, 16), :])
        bot = _ln(r_s[rows(i, RH + j * 16, 16), :])
        for m, v in enumerate(_strassen_lhs(
                top[:, :D2], top[:, D2:], bot[:, :D2], bot[:, D2:])):
            n_s[m][pl.ds(j * 8, 8), :] = _words(v)

    for j in range(RH // 16):
        norm2(0, j)

    @pl.loop(0, NB)
    def _(i):
        @pl.when(i >= 2)
        def _():
            cp_y(i - 2).wait()

        for f in range(FH):
            cs = _strassen(lambda m: _dot(pltpu.bitcast(n_s[m][...], BF16),
                                          pltpu.bitcast(rhs3(m, f), BF16)))
            for m, v in enumerate(_strassen_lhs(*map(_gelu, cs))):
                t_s[m][:, col(f)] = _words(v)
        for j in range(CH):
            cs = _strassen(lambda m: _dot(pltpu.bitcast(t_s[m][...], BF16),
                                          pltpu.bitcast(rhs4(m, j), BF16)))
            for q, h2 in enumerate(cs):
                r, c = rows(i, (q // 2) * RH, RH), col(j + (q % 2) * CH)
                x1 = x_s[r, c].astype(F32) + mod(2, RH, c) * h_s[r, c]
                y = x1 + mod(5, RH, c) * (r_s[r, c] + h2)
                y_s[i % 2, pl.ds((q // 2) * RH, RH), c] = y.astype(y_s.dtype)
            if j < 2:
                for jj in range(j * RH // 32, (j + 1) * RH // 32):
                    norm2(jnp.minimum(i + 1, NB - 1), jj)
        cp_y(i).start()

    cp_y(NB - 2).wait()
    cp_y(NB - 1).wait()


@functools.partial(jax.jit, static_argnames=("A_seg_len",))
def pallas_adaLN_cond__memory_aug_recurrent_mem_tr__mixer_s_mlp__prompt_kernel(
    A_x, A_mem0, A_Wq, A_Wk, A_Wv, A_Wo, A_seg_len, B_x, B_w1, B_w2, B_w3, B_w4,
    c, w_mod,
):
    del B_x
    _, S, D = A_x.shape
    _, H, DH = A_Wq.shape
    M = A_mem0.shape[1]
    SEG = int(A_seg_len)
    FF = B_w3.shape[1]
    HP = H // 2
    RB = 256
    LOOK = S - (S // SEG) * (SEG - M)
    RING = LOOK + 64
    vm = pltpu.VMEM
    dma = pltpu.SemaphoreType.DMA
    scratch = [
        vm((3 * HP + 3 + D // 128, D, DH), U32), vm((HP, DH, D), U32),
        vm((D // 2, FF), U32), vm((FF // 2, D), U32),
        vm((6, D // 2, D), U32),
        vm((S, D), A_x.dtype), vm((S, D), F32), vm((LOOK // 2, D), U32),
        vm((2 * HP, RING, 2 * DH), BF16),
        vm((1, D), c.dtype), vm((M, D), A_mem0.dtype), vm((M + SEG, D), F32),
        vm((SEG // 2, D), U32), vm((HP, M + SEG, 2 * DH), F32),
        vm((M + SEG, D), F32), vm((6, 8, D), F32),
        vm((D // 128, S + 16, 128), F32), vm((S, D), F32),
        vm((S // 2, D), U32), [vm((RB // 4, D // 2), U32)] * 7,
        [vm((RB // 4, FF // 2), U32)] * 7, vm((2, RB, D), A_x.dtype),
        dma((HP,)), dma((2 * HP,)), dma((HP,)), dma((6,)), dma((18,)),
        dma((4,)), dma((2,)),
    ]
    out = pl.pallas_call(
        functools.partial(_kernel, S=S, D=D, H=H, DH=DH, M=M, SEG=SEG, RB=RB),
        out_shape=jax.ShapeDtypeStruct((S, D), A_x.dtype),
        in_specs=[pl.BlockSpec(memory_space=pl.ANY)] * 12,
        out_specs=pl.BlockSpec(memory_space=pl.ANY),
        scratch_shapes=scratch,
        compiler_params=pltpu.CompilerParams(vmem_limit_bytes=120 * 1024 * 1024),
    )(A_x.reshape(S, D), A_mem0.reshape(M, D), A_Wq, A_Wk, A_Wv,
      A_Wo.reshape(H * DH, D), B_w1, B_w2, B_w3, B_w4, c, w_mod)
    return out.reshape(A_x.shape)
```

```python
import functools

import jax
import jax.numpy as jnp
import numpy as np
from jax import lax
import jax.experimental.pallas as pl
import jax.experimental.pallas.tpu as pltpu

F32 = jnp.float32
BF16 = jnp.bfloat16
U32 = jnp.uint32

_NN = (((1,), (0,)), ((), ()))
_NT = (((1,), (1,)), ((), ()))


def _dot(a, b, dims=_NN):
    return lax.dot_general(a, b, dims, preferred_element_type=F32)


def _ln(x):
    m = jnp.mean(x, axis=-1, keepdims=True)
    d = x - m
    v = jnp.mean(d * d, axis=-1, keepdims=True)
    return d * lax.rsqrt(v + 1e-5)


def _gelu(x):
    k0 = float(np.sqrt(2.0 / np.pi))
    k1 = float(np.sqrt(2.0 / np.pi) * 0.044715)
    hx = 0.5 * x
    return hx + hx * jnp.tanh(x * (k0 + k1 * (x * x)))


_CH = 64
import os
_KP = int(os.environ.get('KP', 48))
_TP = int(os.environ.get('TP', 0))
_TL = int(os.environ.get('TL', 3))


def _repack(ref, p, lo_c, hi_c):
    for c in range(lo_c, hi_c):
        even = ref[p, pl.ds(c * _CH, _CH // 2, stride=2), :]
        odd = ref[p, pl.ds(c * _CH + 1, _CH // 2, stride=2), :]
        ref[p, pl.ds(c * _CH, _CH // 2), :] = (even & np.uint32(0xFFFF)) | (odd << 16)
        ref[p, pl.ds(c * _CH + _CH // 2, _CH // 2), :] = (
            (even >> 16) | (odd & np.uint32(0xFFFF0000)))


def _head_words(ref, p, j):
    return jnp.concatenate(
        [ref[p, pl.ds(c * _CH + j * (_CH // 2), _CH // 2), :]
         for c in range(ref.shape[1] // _CH)], axis=0)


def _words(x):
    return pltpu.bitcast(x.astype(BF16), U32)


def _strassen_lhs(a11, a12, a21, a22):
    return (a11 + a22, a21 + a22, a11, a22, a11 + a12, a21 - a11, a12 - a22)


def _strassen_rhs_sums(b11, b12, b21, b22):
    return (b11 + b22, b12 - b22, b21 - b11, b11 + b12, b21 + b22)


def _strassen(prod):
    m0, m1 = prod(0), prod(1)
    c22 = m0 - m1
    m3 = prod(3)
    c11 = m0 + m3
    c21 = m1 + m3
    m2 = prod(2)
    c22 = c22 + m2
    m4 = prod(4)
    c12 = m2 + m4
    c11 = c11 - m4
    c22 = c22 + prod(5)
    c11 = c11 + prod(6)
    return c11, c12, c21, c22


def _kernel(x_hbm, mem_hbm, wq_hbm, wk_hbm, wv_hbm, wo_hbm, w1_hbm, w2_hbm,
            w3_hbm, w4_hbm, c_hbm, wm_hbm, out_hbm,
            w_s, w3_s, w4_s, wm_s,
            x_s, h_s, r_s, acc_s, hb_s, ring_s, c_s, m0_s, o_s, ql_s, kvl_s, mod_s,
            hh_s, wo_s, a_s, t_s, y_s,
            sq, skv, so, sm, sb, sx, sy,
            *, S, D, H, DH, M, SEG, RB):
    HP = H // 2
    NSEG = S // SEG
    L = M + SEG
    KVR = SEG - M
    LOOK = S - NSEG * KVR
    RING = ring_s.shape[1]
    ROFF = RING - LOOK
    D2 = D // 2
    X0 = LOOK + 32
    Q0 = 2 * HP + 1
    T0 = Q0 + HP + 2
    scale = float(DH) ** -0.5

    wq_w = wq_hbm.bitcast(U32)
    wk_w = wk_hbm.bitcast(U32)
    wv_w = wv_hbm.bitcast(U32)
    wo_w = wo_hbm.bitcast(U32)
    wm_w = wm_hbm.bitcast(U32)

    def cp_q(p):
        return pltpu.make_async_copy(wq_w.at[:, p], w_s.at[Q0 + p], sq.at[p])

    def cp_k(p):
        return pltpu.make_async_copy(wk_w.at[:, p], w_s.at[p], skv.at[p])

    def cp_v(p):
        return pltpu.make_async_copy(wv_w.at[:, p], w_s.at[HP + p], skv.at[HP + p])

    def cp_o(p):
        return pltpu.make_async_copy(
            wo_w.at[pl.ds(p * DH, DH)], wo_s.at[pl.ds(p * DH, DH)], so.at[p])

    def cp_m(j):
        return pltpu.make_async_copy(
            wm_w.at[:, pl.ds(j * D, D)], wm_s.at[j], sm.at[j])

    cp_c = pltpu.make_async_copy(c_hbm, c_s, sx.at[0])
    cp_m0 = pltpu.make_async_copy(mem_hbm, m0_s, sx.at[1])
    cp_x0 = pltpu.make_async_copy(
        x_hbm.at[pl.ds(0, X0)], x_s.at[pl.ds(0, X0)], sx.at[2])
    cp_x1 = pltpu.make_async_copy(
        x_hbm.at[pl.ds(X0, S - X0)], x_s.at[pl.ds(X0, S - X0)], sx.at[3])
    CT = D // 128

    def mix_tile(k, j):
        return w_s.at[T0 + j, pl.ds(k * D2, D2)]

    cp_b = [(src.bitcast(U32).at[:, pl.ds(j * 128, 128)], mix_tile(k, j))
            for k, src in enumerate((w1_hbm, w2_hbm)) for j in range(CT)]
    cp_b += [(w3_hbm.bitcast(U32), w3_s), (w4_hbm.bitcast(U32), w4_s)]
    cp_b = [pltpu.make_async_copy(src, dst, sb.at[i])
            for i, (src, dst) in enumerate(cp_b)]

    cp_c.start()
    cp_x0.start()
    cp_m(1).start()
    cp_m(0).start()
    cp_m0.start()
    for p in range(HP):
        cp_k(p).start()
    for p in range(HP):
        cp_v(p).start()
        cp_q(p).start()
    cp_x1.start()
    for p in range(HP):
        cp_o(p).start()

    cp_c.wait()
    cf = c_s[...].astype(F32)
    sc = jnp.broadcast_to(cf * jax.nn.sigmoid(cf), (8, D))

    def mod_vec(j, add=0.0):
        cp_m(j).wait()
        mod_s[j] = _dot(sc, pltpu.bitcast(wm_s[j], BF16)) + add

    def mod(j, n, c=slice(None)):
        return jnp.concatenate([mod_s[j, :, c]] * (n // 8), axis=0)

    cp_x0.wait()

    @pl.loop(0, X0 // 32)
    def _(i):
        r = pl.ds(pl.multiple_of(i * 32, 32), 32)
        h_s[r, :] = _ln(x_s[r, :].astype(F32))

    mod_vec(1, 1.0)
    mod_vec(0)
    for i in range(X0 // 16):
        r = pl.ds(i * 16, 16)
        h = h_s[r, :] * mod(1, 16) + mod(0, 16)
        h_s[r, :] = h
        if i < LOOK // 16:
            hb_s[pl.ds(i * 8, 8), :] = pltpu.bitcast(h.astype(BF16), U32)

    NC = D // _CH
    cp_k(0).wait()
    _repack(w_s, 0, 0, NC)

    @pl.loop(0, HP)
    def _(i):
        second = i >= HP // 2
        pq = jnp.where(second, 2 * (i - HP // 2), HP)
        for u in range(2):
            nxt = 2 * i + u + 1

            @pl.when(nxt < HP)
            def _():
                cp_k(nxt).wait()

            @pl.when((nxt >= HP) & (nxt < 2 * HP))
            def _():
                cp_v(nxt - HP).wait()

        @pl.when(second)
        def _():
            for u in range(2):
                cp_q(pq + u).wait()

        for u in range(2):
            p = 2 * i + u
            for j in range(2):
                w = pltpu.bitcast(_head_words(w_s, p, j), BF16)
                y = _dot(pltpu.bitcast(hb_s[...], BF16), w)
                ring_s[p, pl.ds(ROFF, LOOK), pl.ds(j * DH, DH)] = y.astype(BF16)
                if j == 0:
                    _repack(w_s, p + 1, 0, NC)
                    _repack(w_s, Q0 + pq + u, 0, NC // 4)
                elif u == 0:
                    _repack(w_s, Q0 + pq, NC // 4, NC)
                    _repack(w_s, Q0 + pq + 1, NC // 4, NC)

    for j in range(2, 6):
        cp_m(j).start()
    for cp in cp_b:
        cp.start()
    cp_m0.wait()
    ql_s[pl.ds(0, M), :] = m0_s[...].astype(F32)
    cp_x1.wait()
    for p in range(HP):
        cp_o(p).wait()

    KP = _KP
    row = lax.broadcasted_iota(jnp.int32, (L, KP), 0)
    col = lax.broadcasted_iota(jnp.int32, (L, KP), 1)
    visible = (col < L) & ((row < M) | (col >= SEG) | (row - M >= col))
    fill = jnp.where(col < L, -1e9, -jnp.inf).astype(F32)

    def wpair(p):
        return pltpu.bitcast(jnp.concatenate(
            [_head_words(w_s, p, 0), _head_words(w_s, p, 1)], axis=1), BF16)

    @pl.loop(0, NSEG)
    def _(s):
        seg = pl.ds(pl.multiple_of(s * SEG, SEG), SEG)
        ahead = pl.ds(pl.multiple_of(LOOK + s * KVR, 8), KVR)
        nxt = pl.ds(pl.multiple_of(
            jnp.minimum(LOOK + (s + 1) * KVR, S - KVR), 8), KVR)
        wr = pl.ds(pl.multiple_of(lax.rem(s * KVR, RING), 8), KVR)
        rd = pl.ds(pl.multiple_of(lax.rem(s * SEG + ROFF, RING), SEG), SEG)
        kvl_s[...] = pltpu.bitcast(
            jnp.concatenate([ql_s[pl.ds(0, M), :], h_s[ahead, :]], axis=0).astype(BF16),
            U32)
        ql_s[pl.ds(M, SEG), :] = h_s[seg, :]
        zpad = jnp.zeros((KP - L, 2 * DH), F32)

        def keys(p):
            y = _dot(pltpu.bitcast(kvl_s[...], BF16), wpair(p))
            ring_s[p, wr, :] = y[M:].astype(BF16)
            tail = jnp.concatenate([y[:M], zpad], axis=0).astype(BF16)
            return jnp.concatenate([ring_s[p, rd, :], tail], axis=0)

        def project(p):
            k = keys(p)
            q = _dot(ql_s[...], wpair(Q0 + p))
            return q, k

        def scores(qk):
            q, k = qk
            out = []
            for i in range(2):
                c = slice(i * DH, (i + 1) * DH)
                z = jnp.where(visible, _dot(q[:, c], k[:, c], _NT) * scale, fill)
                e = jnp.exp(z - jnp.max(z, axis=-1, keepdims=True))
                out.append((e, 1.0 / jnp.sum(e, axis=-1, keepdims=True)))
            return out

        def mix(p, es, v):
            for i, (e, inv) in enumerate(es):
                c = slice(i * DH, (i + 1) * DH)
                o_s[p, :, c] = _dot(e, v[:, c]) * inv

        def out_proj(p0, p1, j):
            c = pl.ds(j * 128, 128)
            lhs = jnp.concatenate([o_s[p] for p in range(p0, p1)], axis=1)
            w = wo_s[pl.ds(p0 * DH, (p1 - p0) * DH), c]
            return _dot(lhs, pltpu.bitcast(w, BF16))

        qk, es, vs = {}, {}, {}
        for t in range(HP + 2):
            if t < HP:
                qk[t] = project(t)
            else:
                for j in range((t - HP) * CT // 2, (t - HP + 1) * CT // 2):
                    acc_s[:, pl.ds(j * 128, 128)] = out_proj(0, HP // 2, j)
            if 1 <= t <= HP:
                es[t - 1] = scores(qk.pop(t - 1))
                vs[t - 1] = keys(HP + t - 1)
            if t >= 2:
                mix(t - 2, es.pop(t - 2), vs.pop(t - 2))
        h_s[nxt, :] = _ln(x_s[nxt, :].astype(F32)) * mod(1, KVR) + mod(0, KVR)
        for j in range(CT):
            c = pl.ds(j * 128, 128)
            acc = acc_s[:, c] + out_proj(HP // 2, HP, j)
            ql_s[pl.ds(0, M), c] = acc[:M]
            h_s[seg, c] = acc[M:]

    NB = S // RB
    G = CT // 4
    FT = w3_s.shape[1] // 128
    FH, CH, RH = FT // 2, CT // 2, RB // 2
    NI = NB // 2
    K3, K4 = D // 4, FT * 32
    SUM = (0, None, 1, 2, None, 3, 4)

    def rows(i, off, n):
        return pl.ds(pl.multiple_of(i * RB + off, n), n)

    def col(j):
        return pl.ds(j * 128, 128)

    def block12(k, j):
        return lambda q: (mix_tile(k, j + (q % 2) * CH), (q // 2) * K3, slice(None))

    def block3(f):
        return lambda q: (w3_s, (q // 2) * K3, col(f + (q % 2) * FH))

    def block4(j):
        return lambda q: (w4_s, (q // 2) * K4, col(j + (q % 2) * CH))

    def home12(k, j):
        n = 5 * (CH * k + j)
        return lambda e: (2 * ((n + e) // 3) + 1, (1 + (n + e) % 3) * K3)

    def home3(f):
        return lambda e: (2 * f + e // 4, (e % 4) * K3)

    def home4(j):
        return lambda e: (2 * FH + 5 * j + e, 0)

    def make(block, home, r0):
        w = []
        for q in range(4):
            ref, off, c = block(q)
            w.append(ref[pl.ds(off + r0, 16), c])
        lo = _strassen_rhs_sums(*[pltpu.bitcast(v << 16, F32) for v in w])
        hi = _strassen_rhs_sums(
            *[pltpu.bitcast(v & np.uint32(0xFFFF0000), F32) for v in w])
        for e, pair in enumerate(zip(lo, hi)):
            slot, off = home(e)
            w_s[slot, pl.ds(off + r0, 16), :] = pltpu.bitcast(
                pltpu.pack_elementwise(list(pair), packed_dtype=BF16), U32)

    def spread(jobs, slots):
        state = [0, 0]

        def tick():
            state[0] += 1
            while state[1] < min(len(jobs), (state[0] - 1) * len(jobs) // (slots - 1)):
                jobs[state[1]]()
                state[1] += 1
        return tick

    def matmul(lhs, block, home, n, tick=lambda: None):
        def prod(m):
            tick()
            if SUM[m] is None:
                ref, off, c = block(0 if m == 1 else 3)
                w = ref[pl.ds(off, n), c]
            else:
                slot, off = home(SUM[m])
                w = w_s[slot, pl.ds(off, n), :]
            return _dot(pltpu.bitcast(lhs(m), BF16), pltpu.bitcast(w, BF16))
        return _strassen(prod)

    def get_a(i):
        return lambda m: a_s[m][pl.ds(pl.multiple_of(i * (RH // 2), 8), RH // 2), :]

    def put_a(i, g, half):
        top, bot = half(g * 16), half(RH + g * 16)
        for m, v in enumerate(_strassen_lhs(
                top[:, :D2], top[:, D2:], bot[:, :D2], bot[:, D2:])):
            a_s[m][pl.ds(pl.multiple_of(i * (RH // 2) + g * 8, 8), 8), :] = _words(v)

    def norm1(i, g):
        def half(off):
            r = rows(i, off, 16)
            x1 = x_s[r, :].astype(F32) + mod(2, 16) * h_s[r, :]
            hb = _ln(x1) * mod(4, 16) + mod(3, 16)
            r_s[r, :] = hb
            return _ln(hb)
        put_a(i, g, half)

    def shifted(i, g):
        put_a(i, g, lambda off: jnp.concatenate(
            [hh_s[k, pl.ds(8 + i * RB + off + (-1, 1, -2, 2)[k // G], 16), :]
             for k in range(CT)], axis=1))

    def norm2(i, g):
        put_a(i, g, lambda off: _ln(r_s[rows(i, off, 16), :]))

    NG = RH // 16

    for cp in cp_b:
        cp.wait()
    for j in range(2, 6):
        cp_m(j).wait()
    for j in (2, 3, 4, 5):
        mod_s[j] = _dot(sc, pltpu.bitcast(wm_s[j], BF16)) + (1.0 if j == 4 else 0.0)
        for r0 in range(0, K3, 16):
            make(block12(0, j - 2), home12(0, j - 2), r0)
    for j in range(CT):
        hh_s[j, pl.ds(0, 8), :] = jnp.zeros((8, 128), F32)
        hh_s[j, pl.ds(8 + S, 8), :] = jnp.zeros((8, 128), F32)
    for g in range(NG):
        norm1(0, g)

    @pl.loop(0, NI)
    def _(ii):
        for u in range(2):
            i = 2 * ii + u
            jobs = []
            for g in range(NG):
                jobs.append(functools.partial(norm1, jnp.minimum(i + 1, NB - 1), g))
                jobs.append(functools.partial(
                    make, block12(1, g % CH), home12(1, g % CH),
                    pl.multiple_of(i * (K3 // NB) + (g // CH) * 16, 8)))
            tick = spread(jobs, 7 * CH)
            for j in range(CH):
                cs = matmul(get_a(i), block12(0, j), home12(0, j), K3, tick)
                for q, y in enumerate(cs):
                    hh_s[j + (q % 2) * CH,
                         pl.ds(pl.multiple_of(8 + i * RB + (q // 2) * RH, 8), RH), :] = (
                             _gelu(y))

    for g in range(NG):
        shifted(0, g)

    @pl.loop(0, NI)
    def _(ii):
        for u in range(2):
            i = 2 * ii + u
            work = [(block3(f), home3(f), i * (K3 // NB) + v * 16)
                    for f in range(FH) for v in range(K3 // NB // 16)]
            work += [(block4(j), home4(j), i * (K4 // NB) + v * 16)
                     for j in range(CH) for v in range(K4 // NB // 16)]
            jobs = []
            for g in range(NG):
                jobs.append(functools.partial(shifted, jnp.minimum(i + 1, NB - 1), g))
                jobs += [functools.partial(make, b, h, pl.multiple_of(r0, 8))
                         for b, h, r0 in work[g::NG]]
            tick = spread(jobs, 7 * CH)
            for j in range(CH):
                cs = matmul(get_a(i), block12(1, j), home12(1, j), K3, tick)
                for q, y in enumerate(cs):
                    r_s[rows(i, (q // 2) * RH, RH), col(j + (q % 2) * CH)] += y

    def cp_y(i):
        return pltpu.make_async_copy(
            y_s.at[i % 2], out_hbm.at[rows(i, 0, RB)], sy.at[i % 2])

    for g in range(NG):
        norm2(0, g)

    @pl.loop(0, NB)
    def _(i):
        @pl.when(i >= 2)
        def _():
            cp_y(i - 2).wait()

        for f in range(FH):
            cs = matmul(get_a(i), block3(f), home3(f), K3)
            for m, v in enumerate(_strassen_lhs(*map(_gelu, cs))):
                t_s[m][:, col(f)] = _words(v)
        for j in range(CH):
            cs = matmul(lambda m: t_s[m][...], block4(j), home4(j), K4)
            for q, h2 in enumerate(cs):
                r, c = rows(i, (q // 2) * RH, RH), col(j + (q % 2) * CH)
                x1 = x_s[r, c].astype(F32) + mod(2, RH, c) * h_s[r, c]
                y = x1 + mod(5, RH, c) * (r_s[r, c] + h2)
                y_s[i % 2, pl.ds((q // 2) * RH, RH), c] = y.astype(y_s.dtype)
            if j < 2:
                for g in range(j * NG // 2, (j + 1) * NG // 2):
                    norm2(jnp.minimum(i + 1, NB - 1), g)
        cp_y(i).start()

    cp_y(NB - 2).wait()
    cp_y(NB - 1).wait()


@functools.partial(jax.jit, static_argnames=("A_seg_len",))
def pallas_adaLN_cond__memory_aug_recurrent_mem_tr__mixer_s_mlp__prompt_kernel(
    A_x, A_mem0, A_Wq, A_Wk, A_Wv, A_Wo, A_seg_len, B_x, B_w1, B_w2, B_w3, B_w4,
    c, w_mod,
):
    del B_x
    _, S, D = A_x.shape
    _, H, DH = A_Wq.shape
    M = A_mem0.shape[1]
    SEG = int(A_seg_len)
    FF = B_w3.shape[1]
    HP = H // 2
    RB = 256
    LOOK = S - (S // SEG) * (SEG - M)
    RING = LOOK + 64
    vm = pltpu.VMEM
    dma = pltpu.SemaphoreType.DMA
    scratch = [
        vm((3 * HP + 3 + D // 128, D, DH), U32),
        vm((D // 2, FF), U32), vm((FF // 2, D), U32),
        vm((6, D // 2, D), U32),
        vm((S, D), A_x.dtype), vm((S, D), F32), vm((S, D), F32), vm((M + SEG, D), F32),
        vm((LOOK // 2, D), U32),
        vm((2 * HP, RING, 2 * DH), BF16),
        vm((1, D), c.dtype), vm((M, D), A_mem0.dtype),
        vm((HP, M + SEG, 2 * DH), F32),
        vm((M + SEG, D), F32), vm((SEG // 2, D), U32), vm((6, 8, D), F32),
        vm((D // 128, S + 16, 128), F32),
        vm((HP * DH, D), U32), [vm((S // 4, D // 2), U32)] * 7,
        [vm((RB // 4, FF // 2), U32)] * 7, vm((2, RB, D), A_x.dtype),
        dma((HP,)), dma((2 * HP,)), dma((HP,)), dma((6,)), dma((18,)),
        dma((4,)), dma((2,)),
    ]
    out = pl.pallas_call(
        functools.partial(_kernel, S=S, D=D, H=H, DH=DH, M=M, SEG=SEG, RB=RB),
        out_shape=jax.ShapeDtypeStruct((S, D), A_x.dtype),
        in_specs=[pl.BlockSpec(memory_space=pl.ANY)] * 12,
        out_specs=pl.BlockSpec(memory_space=pl.ANY),
        scratch_shapes=scratch,
        compiler_params=pltpu.CompilerParams(vmem_limit_bytes=120 * 1024 * 1024),
    )(A_x.reshape(S, D), A_mem0.reshape(M, D), A_Wq, A_Wk, A_Wv,
      A_Wo.reshape(H * DH, D), B_w1, B_w2, B_w3, B_w4, c, w_mod)
    return out.reshape(A_x.shape)
```

```python
import functools

import jax
import jax.numpy as jnp
import numpy as np
from jax import lax
import jax.experimental.pallas as pl
import jax.experimental.pallas.tpu as pltpu

F32 = jnp.float32
BF16 = jnp.bfloat16
U32 = jnp.uint32

_NN = (((1,), (0,)), ((), ()))
_NT = (((1,), (1,)), ((), ()))


def _dot(a, b, dims=_NN):
    return lax.dot_general(a, b, dims, preferred_element_type=F32)


def _ln(x):
    m = jnp.mean(x, axis=-1, keepdims=True)
    d = x - m
    v = jnp.mean(d * d, axis=-1, keepdims=True)
    return d * lax.rsqrt(v + 1e-5)


def _gelu(x):
    k0 = float(np.sqrt(2.0 / np.pi))
    k1 = float(np.sqrt(2.0 / np.pi) * 0.044715)
    hx = 0.5 * x
    return hx + hx * jnp.tanh(x * (k0 + k1 * (x * x)))


def _words(x):
    return pltpu.bitcast(x.astype(BF16), U32)


def _halves(w):
    return (pltpu.bitcast(w << 16, F32),
            pltpu.bitcast(w & np.uint32(0xFFFF0000), F32))


def _join(lo, hi):
    return pltpu.bitcast(pltpu.pack_elementwise([lo, hi], packed_dtype=BF16), U32)


def _spread(jobs, slots):
    state = [0, 0]

    def tick():
        state[0] += 1
        while state[1] < min(len(jobs), (state[0] - 1) * len(jobs) // (slots - 1)):
            jobs[state[1]]()
            state[1] += 1
    return tick


def _strassen_lhs(a11, a12, a21, a22):
    return (a11 + a22, a21 + a22, a11, a22, a11 + a12, a21 - a11, a12 - a22)


def _strassen_rhs_sums(b11, b12, b21, b22):
    return (b11 + b22, b12 - b22, b21 - b11, b11 + b12, b21 + b22)


_SUM = (0, None, 1, 2, None, 3, 4)


def _strassen(lhs, rhs, tick=lambda: None):
    def prod(m):
        tick()
        return _dot(pltpu.bitcast(lhs(m), BF16), pltpu.bitcast(rhs(m), BF16))

    m0, m1 = prod(0), prod(1)
    c22 = m0 - m1
    m3 = prod(3)
    c11 = m0 + m3
    c21 = m1 + m3
    m2 = prod(2)
    c22 = c22 + m2
    m4 = prod(4)
    c12 = m2 + m4
    c11 = c11 - m4
    c22 = c22 + prod(5)
    c11 = c11 + prod(6)
    return c11, c12, c21, c22


def _kernel(x_hbm, mem_hbm, wq_hbm, wk_hbm, wv_hbm, wo_hbm, w1_hbm, w2_hbm,
            w3_hbm, w4_hbm, c_hbm, wm_hbm, out_hbm,
            w_s, wo_s, w3_s, w4_s, wm_s, x_s, h_s, r_s, hh_s, ring_s,
            c_s, m0_s, in_s, lhs_s, o_s, acc_s, mod_s, a_s, t_s, y_s,
            sw, sx, sy,
            *, S, D, H, DH, M, SEG, RB):
    HP = H // 2
    NP = 3 * HP
    T0 = NP + 1
    NSEG = S // SEG
    L = M + SEG
    RIDE = SEG - M
    LOOK = S - NSEG * RIDE
    RING = ring_s.shape[1]
    ROFF = RING - LOOK
    D2 = D // 2
    K3 = D // 4
    CT = D // 128
    X0 = LOOK + 32
    scale = float(DH) ** -0.5

    def cp_w(p):
        src = (wk_hbm, wv_hbm, wq_hbm)[p // HP % 3].bitcast(U32)
        return pltpu.make_async_copy(
            src.at[:, p % HP], w_s.at[p], sw.at[(p + 1) // 2])

    def mix_tile(k, j):
        return w_s.at[T0 + j, pl.ds(k * D2, D2)]

    def copies(pairs, sem):
        return [pltpu.make_async_copy(src, dst, sem) for src, dst in pairs]

    def mod_pair(j):
        return wm_hbm.bitcast(U32).at[:, pl.ds(j * D, D)], wm_s.at[j]

    cp_first = copies([(c_hbm, c_s),
                       (x_hbm.at[pl.ds(0, X0)], x_s.at[pl.ds(0, X0)])], sx.at[0])
    cp_ca = copies([mod_pair(1)], sx.at[1])
    cp_sa = copies([mod_pair(0)], sx.at[2])
    cp_a = copies([(mem_hbm, m0_s),
                   (x_hbm.at[pl.ds(X0, S - X0)], x_s.at[pl.ds(X0, S - X0)]),
                   (wo_hbm.bitcast(U32), wo_s)], sx.at[3])
    cp_b = copies(
        [mod_pair(j) for j in range(2, 6)]
        + [(src.bitcast(U32).at[:, pl.ds(j * 128, 128)], mix_tile(k, j))
           for k, src in enumerate((w1_hbm, w2_hbm)) for j in range(CT)]
        + [(w3_hbm.bitcast(U32), w3_s), (w4_hbm.bitcast(U32), w4_s)], sx.at[4])

    def wait(cps):
        for cp in cps:
            cp.wait()

    for cp in cp_first + cp_ca + cp_sa + [cp_w(p) for p in range(NP + 1)] + cp_a:
        cp.start()

    wait(cp_first)
    cf = c_s[...].astype(F32)
    sc = jnp.broadcast_to(cf * jax.nn.sigmoid(cf), (8, D))

    def mod_vec(j):
        y = _dot(sc, pltpu.bitcast(wm_s[j], BF16))
        mod_s[j] = 1.0 + y if j in (1, 4) else y

    def mod(j, n, c=slice(None)):
        return jnp.concatenate([mod_s[j, :, c]] * (n // 8), axis=0)

    def put_a(r, top, bot):
        for m, v in enumerate(_strassen_lhs(
                top[:, :D2], top[:, D2:], bot[:, :D2], bot[:, D2:])):
            a_s[m][r, :] = _words(v)

    @pl.loop(0, X0 // 32)
    def _(i):
        r = pl.ds(pl.multiple_of(i * 32, 32), 32)
        h_s[r, :] = _ln(x_s[r, :].astype(F32))

    wait(cp_ca)
    mod_vec(1)
    wait(cp_sa)
    mod_vec(0)
    for i in range(LOOK // 32):
        put_a(pl.ds(i * 8, 8), *[
            h_s[pl.ds(i * 16 + off, 16), :] * mod(1, 16) + mod(0, 16)
            for off in (0, LOOK // 2)])
    in_s[pl.ds(M, RIDE), :] = h_s[pl.ds(LOOK, RIDE), :] * mod(1, RIDE) + mod(0, RIDE)

    def repack(p, u, c):
        par = []
        for odd in range(2):
            top, bot = [_halves(w_s[p, pl.ds(off + c * 32 + odd, 16, stride=2), :])
                        for off in (0, D2)]
            par.append(top + bot + _strassen_rhs_sums(*top, *bot))
        for e, pair in enumerate(zip(*par)):
            if e < 4:
                w_s[p, pl.ds((e // 2) * D2 + c * 32 + (e % 2) * 16, 16), :] = _join(*pair)
            else:
                w_s[T0 + 2 * u + (e - 4) // 4, pl.ds((e % 4) * K3 + c * 16, 16), :] = (
                    _join(*pair))

    def head(p, j, c0=0, c1=D // 32):
        return jnp.concatenate(
            [w_s[p, pl.ds(c * 32 + j * 16, 16), :] for c in range(c0, c1)], axis=0)

    cp_w(0).wait()
    for c in range(D2 // 32):
        repack(0, 0, c)

    @pl.loop(0, NP // 2)
    def _(i):
        two = w_s.at[pl.ds(2 * i + 1, 2)]
        pltpu.make_async_copy(two, two, sw.at[i + 1]).wait()
        for u in range(2):
            p = 2 * i + u

            def rhs(m):
                if _SUM[m] is None:
                    j = m // 4
                    return head(p, j, j * D2 // 32, (j + 1) * D2 // 32)
                return w_s[T0 + 2 * u + _SUM[m] // 4, pl.ds((_SUM[m] % 4) * K3, K3), :]

            jobs = [functools.partial(repack, p + 1, 1 - u, c) for c in range(D2 // 32)]
            cs = _strassen(lambda m: a_s[m][pl.ds(0, LOOK // 4), :], rhs,
                           _spread(jobs, 7))
            for q, y in enumerate(cs):
                ring_s[p, pl.ds(ROFF + (q // 2) * (LOOK // 2), LOOK // 2),
                       pl.ds((q % 2) * DH, DH)] = y.astype(BF16)

    for cp in cp_b:
        cp.start()
    wait(cp_a)
    in_s[pl.ds(0, M), :] = m0_s[...].astype(F32)

    KP = SEG + 2 * M
    row = lax.broadcasted_iota(jnp.int32, (L, KP), 0)
    col = lax.broadcasted_iota(jnp.int32, (L, KP), 1)
    visible = (col < L) & ((row < M) | (col >= SEG) | (row - M >= col))
    fill = jnp.where(col < L, -1e9, -jnp.inf).astype(F32)

    @pl.loop(0, NSEG)
    def _(s):
        seg = pl.ds(pl.multiple_of(s * SEG, SEG), SEG)
        nxt = pl.ds(pl.multiple_of(
            jnp.minimum(LOOK + (s + 1) * RIDE, S - RIDE), 8), RIDE)
        wr = pl.ds(pl.multiple_of(lax.rem(s * RIDE, RING), 8), RIDE)
        rd = pl.ds(pl.multiple_of(lax.rem(s * SEG + ROFF, RING), SEG), SEG)
        lhs_s[...] = _words(in_s[...])
        in_s[pl.ds(M, RIDE), :] = (
            _ln(x_s[nxt, :].astype(F32)) * mod(1, RIDE) + mod(0, RIDE))

        def project(p):
            w = jnp.concatenate([head(p, 0), head(p, 1)], axis=1)
            y = _dot(pltpu.bitcast(lhs_s[...], BF16), pltpu.bitcast(w, BF16))
            ring_s[p, wr, :] = y[M:].astype(BF16)
            return y[:M], ring_s[p, rd, :]

        def keys(p):
            mem, tok = project(p)
            tail = jnp.concatenate([mem, jnp.zeros_like(mem)], axis=0).astype(BF16)
            return jnp.concatenate([tok, tail], axis=0)

        def queries(p):
            mem, tok = project(2 * HP + p)
            return jnp.concatenate([mem, tok.astype(F32)], axis=0)

        def scores(qk):
            q, k = qk
            out = []
            for i in range(2):
                c = slice(i * DH, (i + 1) * DH)
                z = jnp.where(visible, _dot(q[:, c], k[:, c], _NT) * scale, fill)
                e = jnp.exp(z - jnp.max(z, axis=-1, keepdims=True))
                out.append((e, 1.0 / jnp.sum(e, axis=-1, keepdims=True)))
            return out

        def mix(p, es, v):
            for i, (e, inv) in enumerate(es):
                c = slice(i * DH, (i + 1) * DH)
                o_s[p, :, c] = _dot(e, v[:, c]) * inv

        def out_proj(p0, p1, j):
            c = pl.ds(j * 128, 128)
            lhs = jnp.concatenate([o_s[p] for p in range(p0, p1)], axis=1)
            w = wo_s[pl.ds(p0 * DH, (p1 - p0) * DH), c]
            return _dot(lhs, pltpu.bitcast(w, BF16))

        qk, es, vs = {}, {}, {}
        for t in range(HP + 2):
            if t < HP:
                k = keys(t)
                qk[t] = queries(t), k
            else:
                for j in range((t - HP) * CT // 2, (t - HP + 1) * CT // 2):
                    acc_s[:, pl.ds(j * 128, 128)] = out_proj(0, HP // 2, j)
            if 1 <= t <= HP:
                es[t - 1] = scores(qk.pop(t - 1))
                vs[t - 1] = keys(HP + t - 1)
            if t >= 2:
                mix(t - 2, es.pop(t - 2), vs.pop(t - 2))
        for j in range(CT):
            c = pl.ds(j * 128, 128)
            acc = acc_s[:, c] + out_proj(HP // 2, HP, j)
            in_s[pl.ds(0, M), c] = acc[:M]
            h_s[seg, c] = acc[M:]

    NB = S // RB
    G = CT // 4
    FT = w3_s.shape[1] // 128
    FH, CH, RH = FT // 2, CT // 2, RB // 2
    NI = NB // 2
    K4 = FT * 32

    def rows(i, off, n):
        return pl.ds(pl.multiple_of(i * RB + off, n), n)

    def col(j):
        return pl.ds(j * 128, 128)

    def block12(k, j):
        return lambda q: (mix_tile(k, j + (q % 2) * CH), (q // 2) * K3, slice(None))

    def block3(f):
        return lambda q: (w3_s, (q // 2) * K3, col(f + (q % 2) * FH))

    def block4(j):
        return lambda q: (w4_s, (q // 2) * K4, col(j + (q % 2) * CH))

    def home12(k, j):
        n = 5 * (CH * k + j)
        return lambda e: (2 * ((n + e) // 3) + 1, (1 + (n + e) % 3) * K3)

    def home3(f):
        return lambda e: (2 * f + e // 4, (e % 4) * K3)

    def home4(j):
        return lambda e: (2 * FH + 5 * j + e, 0)

    def make(block, home, r0):
        w = []
        for q in range(4):
            ref, off, c = block(q)
            w.append(_halves(ref[pl.ds(off + r0, 16), c]))
        lo, hi = [_strassen_rhs_sums(*v) for v in zip(*w)]
        for e, pair in enumerate(zip(lo, hi)):
            slot, off = home(e)
            w_s[slot, pl.ds(off + r0, 16), :] = _join(*pair)

    def get_w(block, home, n):
        def rhs(m):
            if _SUM[m] is None:
                ref, off, c = block(0 if m == 1 else 3)
                return ref[pl.ds(off, n), c]
            slot, off = home(_SUM[m])
            return w_s[slot, pl.ds(off, n), :]
        return rhs

    def get_a(i):
        return lambda m: a_s[m][pl.ds(pl.multiple_of(i * (RH // 2), 8), RH // 2), :]

    def put(i, g, half):
        put_a(pl.ds(pl.multiple_of(i * (RH // 2) + g * 8, 8), 8),
              half(g * 16), half(RH + g * 16))

    def norm1(i, g):
        def half(off):
            r = rows(i, off, 16)
            x1 = x_s[r, :].astype(F32) + mod(2, 16) * h_s[r, :]
            hb = _ln(x1) * mod(4, 16) + mod(3, 16)
            r_s[r, :] = hb
            return _ln(hb)
        put(i, g, half)

    def shifted(i, g):
        put(i, g, lambda off: jnp.concatenate(
            [hh_s[k, pl.ds(8 + i * RB + off + (-1, 1, -2, 2)[k // G], 16), :]
             for k in range(CT)], axis=1))

    def norm2(i, g):
        put(i, g, lambda off: _ln(r_s[rows(i, off, 16), :]))

    NG = RH // 16

    wait(cp_b)
    for j in (2, 3, 4, 5):
        mod_vec(j)
        for r0 in range(0, K3, 16):
            make(block12(0, j - 2), home12(0, j - 2), r0)
    for j in range(CT):
        hh_s[j, pl.ds(0, 8), :] = jnp.zeros((8, 128), F32)
        hh_s[j, pl.ds(8 + S, 8), :] = jnp.zeros((8, 128), F32)
    for g in range(NG):
        norm1(0, g)

    @pl.loop(0, NI)
    def _(ii):
        for u in range(2):
            i = 2 * ii + u
            jobs = []
            for g in range(NG):
                jobs.append(functools.partial(norm1, jnp.minimum(i + 1, NB - 1), g))
                jobs.append(functools.partial(
                    make, block12(1, g % CH), home12(1, g % CH),
                    pl.multiple_of(i * (K3 // NB) + (g // CH) * 16, 8)))
            tick = _spread(jobs, 7 * CH)
            for j in range(CH):
                cs = _strassen(get_a(i), get_w(block12(0, j), home12(0, j), K3), tick)
                for q, y in enumerate(cs):
                    hh_s[j + (q % 2) * CH,
                         pl.ds(pl.multiple_of(8 + i * RB + (q // 2) * RH, 8), RH), :] = (
                             _gelu(y))

    for g in range(NG):
        shifted(0, g)

    @pl.loop(0, NI)
    def _(ii):
        for u in range(2):
            i = 2 * ii + u
            work = [(block3(f), home3(f), i * (K3 // NB) + v * 16)
                    for f in range(FH) for v in range(K3 // NB // 16)]
            work += [(block4(j), home4(j), i * (K4 // NB) + v * 16)
                     for j in range(CH) for v in range(K4 // NB // 16)]
            jobs = []
            for g in range(NG):
                jobs.append(functools.partial(shifted, jnp.minimum(i + 1, NB - 1), g))
                jobs += [functools.partial(make, b, h, pl.multiple_of(r0, 8))
                         for b, h, r0 in work[g::NG]]
            tick = _spread(jobs, 7 * CH)
            for j in range(CH):
                cs = _strassen(get_a(i), get_w(block12(1, j), home12(1, j), K3), tick)
                for q, y in enumerate(cs):
                    r_s[rows(i, (q // 2) * RH, RH), col(j + (q % 2) * CH)] += y

    def cp_y(i):
        return pltpu.make_async_copy(
            y_s.at[i % 2], out_hbm.at[rows(i, 0, RB)], sy.at[i % 2])

    for g in range(NG):
        norm2(0, g)

    @pl.loop(0, NB)
    def _(i):
        @pl.when(i >= 2)
        def _():
            cp_y(i - 2).wait()

        for f in range(FH):
            cs = _strassen(get_a(i), get_w(block3(f), home3(f), K3))
            for m, v in enumerate(_strassen_lhs(*map(_gelu, cs))):
                t_s[m][:, col(f)] = _words(v)
        for j in range(CH):
            cs = _strassen(lambda m: t_s[m][...], get_w(block4(j), home4(j), K4))
            for q, h2 in enumerate(cs):
                r, c = rows(i, (q // 2) * RH, RH), col(j + (q % 2) * CH)
                x1 = x_s[r, c].astype(F32) + mod(2, RH, c) * h_s[r, c]
                y = x1 + mod(5, RH, c) * (r_s[r, c] + h2)
                y_s[i % 2, pl.ds((q // 2) * RH, RH), c] = y.astype(y_s.dtype)
            if j < 2:
                for g in range(j * NG // 2, (j + 1) * NG // 2):
                    norm2(jnp.minimum(i + 1, NB - 1), g)
        cp_y(i).start()

    cp_y(NB - 2).wait()
    cp_y(NB - 1).wait()


@functools.partial(jax.jit, static_argnames=("A_seg_len",))
def pallas_adaLN_cond__memory_aug_recurrent_mem_tr__mixer_s_mlp__prompt_kernel(
    A_x, A_mem0, A_Wq, A_Wk, A_Wv, A_Wo, A_seg_len, B_x, B_w1, B_w2, B_w3, B_w4,
    c, w_mod,
):
    del B_x
    _, S, D = A_x.shape
    _, H, DH = A_Wq.shape
    M = A_mem0.shape[1]
    SEG = int(A_seg_len)
    FF = B_w3.shape[1]
    HP = H // 2
    RB = 256
    LOOK = S - (S // SEG) * (SEG - M)
    RING = LOOK + 64
    vm = pltpu.VMEM
    dma = pltpu.SemaphoreType.DMA
    scratch = [
        vm((3 * HP + 1 + D // 128, D, DH), U32), vm((HP * DH, D), U32),
        vm((D // 2, FF), U32), vm((FF // 2, D), U32), vm((6, D // 2, D), U32),
        vm((S, D), A_x.dtype), vm((S, D), F32), vm((S, D), F32),
        vm((D // 128, S + 16, 128), F32), vm((3 * HP, RING, 2 * DH), BF16),
        vm((1, D), c.dtype), vm((M, D), A_mem0.dtype),
        vm((SEG, D), F32), vm((SEG // 2, D), U32),
        vm((HP, M + SEG, 2 * DH), F32), vm((M + SEG, D), F32), vm((6, 8, D), F32),
        [vm((S // 4, D // 2), U32)] * 7, [vm((RB // 4, FF // 2), U32)] * 7,
        vm((2, RB, D), A_x.dtype),
        dma((3 * HP // 2 + 1,)), dma((5,)), dma((2,)),
    ]
    out = pl.pallas_call(
        functools.partial(_kernel, S=S, D=D, H=H, DH=DH, M=M, SEG=SEG, RB=RB),
        out_shape=jax.ShapeDtypeStruct((S, D), A_x.dtype),
        in_specs=[pl.BlockSpec(memory_space=pl.ANY)] * 12,
        out_specs=pl.BlockSpec(memory_space=pl.ANY),
        scratch_shapes=scratch,
        compiler_params=pltpu.CompilerParams(vmem_limit_bytes=124 * 1024 * 1024),
    )(A_x.reshape(S, D), A_mem0.reshape(M, D), A_Wq, A_Wk, A_Wv,
      A_Wo.reshape(H * DH, D), B_w1, B_w2, B_w3, B_w4, c, w_mod)
    return out.reshape(A_x.shape)
```

```python
import functools

import jax
import jax.numpy as jnp
import numpy as np
from jax import lax
import jax.experimental.pallas as pl
import jax.experimental.pallas.tpu as pltpu

F32 = jnp.float32
BF16 = jnp.bfloat16
U32 = jnp.uint32

_NN = (((1,), (0,)), ((), ()))
_NT = (((1,), (1,)), ((), ()))


def _dot(a, b, dims=_NN):
    return lax.dot_general(a, b, dims, preferred_element_type=F32)


def _ln(x):
    m = jnp.mean(x, axis=-1, keepdims=True)
    d = x - m
    v = jnp.mean(d * d, axis=-1, keepdims=True)
    return d * lax.rsqrt(v + 1e-5)


def _gelu(x):
    k0 = float(np.sqrt(2.0 / np.pi))
    k1 = float(np.sqrt(2.0 / np.pi) * 0.044715)
    hx = 0.5 * x
    return hx + hx * jnp.tanh(x * (k0 + k1 * (x * x)))


def _words(x):
    return pltpu.bitcast(x.astype(BF16), U32)


def _halves(w):
    return (pltpu.bitcast(w << 16, F32),
            pltpu.bitcast(w & np.uint32(0xFFFF0000), F32))


def _join(lo, hi):
    return pltpu.bitcast(pltpu.pack_elementwise([lo, hi], packed_dtype=BF16), U32)


def _spread(jobs, slots, first=1):
    state = [0, 0]

    def tick():
        state[0] += 1
        while state[1] < min(len(jobs), -(-(state[0] - first) * len(jobs) // (slots - first))):
            jobs[state[1]]()
            state[1] += 1
    return tick


def _strassen_lhs(a11, a12, a21, a22):
    return (a11 + a22, a21 + a22, a11, a22, a11 + a12, a21 - a11, a12 - a22)


def _strassen_rhs_sums(b11, b12, b21, b22):
    return (b11 + b22, b12 - b22, b21 - b11, b11 + b12, b21 + b22)


_SUM = (0, None, 1, 2, None, 3, 4)


def _strassen(lhs, rhs, tick=lambda: None):
    def prod(m):
        tick()
        return _dot(pltpu.bitcast(lhs(m), BF16), pltpu.bitcast(rhs(m), BF16))

    m0, m1 = prod(0), prod(1)
    c22 = m0 - m1
    m3 = prod(3)
    c11 = m0 + m3
    c21 = m1 + m3
    m2 = prod(2)
    c22 = c22 + m2
    m4 = prod(4)
    c12 = m2 + m4
    c11 = c11 - m4
    c22 = c22 + prod(5)
    c11 = c11 + prod(6)
    return c11, c12, c21, c22


def _kernel(x_hbm, mem_hbm, wq_hbm, wk_hbm, wv_hbm, wo_hbm, w1_hbm, w2_hbm,
            w3_hbm, w4_hbm, c_hbm, wm_hbm, out_hbm,
            w_s, wo_s, w3_s, w4_s, wm_s, x_s, h_s, r_s, hh_s, ring_s,
            c_s, m0_s, in_s, lhs_s, o_s, acc_s, mod_s, a_s, t_s, y_s,
            sw, sx, sy,
            *, S, D, H, DH, M, SEG, RB):
    HP = H // 2
    NP = 3 * HP
    T0 = NP + 1
    NSEG = S // SEG
    L = M + SEG
    RIDE = SEG - M
    LOOK = S - NSEG * RIDE
    RING = ring_s.shape[1]
    ROFF = RING - LOOK
    D2 = D // 2
    K3 = D // 4
    CT = D // 128
    X0 = LOOK + 32
    scale = float(DH) ** -0.5

    def cp_w(p):
        src = (wk_hbm, wv_hbm, wq_hbm)[p // HP % 3].bitcast(U32)
        return pltpu.make_async_copy(
            src.at[:, p % HP], w_s.at[p], sw.at[(p + 1) // 2])

    def mix_tile(k, j):
        return w_s.at[T0 + j, pl.ds(k * D2, D2)]

    def copies(pairs, sem):
        return [pltpu.make_async_copy(src, dst, sem) for src, dst in pairs]

    def mod_pair(j):
        return wm_hbm.bitcast(U32).at[:, pl.ds(j * D, D)], wm_s.at[j]

    cp_first = copies([(c_hbm, c_s),
                       (x_hbm.at[pl.ds(0, X0)], x_s.at[pl.ds(0, X0)])], sx.at[0])
    cp_ca = copies([mod_pair(1)], sx.at[1])
    cp_sa = copies([mod_pair(0)], sx.at[2])
    cp_a = copies([(mem_hbm, m0_s),
                   (x_hbm.at[pl.ds(X0, S - X0)], x_s.at[pl.ds(X0, S - X0)]),
                   (wo_hbm.bitcast(U32), wo_s)], sx.at[3])
    cp_b = copies(
        [mod_pair(j) for j in range(2, 6)]
        + [(src.bitcast(U32).at[:, pl.ds(j * 128, 128)], mix_tile(k, j))
           for k, src in enumerate((w1_hbm, w2_hbm)) for j in range(CT)]
        + [(w3_hbm.bitcast(U32), w3_s), (w4_hbm.bitcast(U32), w4_s)], sx.at[4])

    def wait(cps):
        for cp in cps:
            cp.wait()

    for cp in cp_first + cp_ca + cp_sa + [cp_w(p) for p in range(NP + 1)] + cp_a:
        cp.start()

    wait(cp_first)
    cf = c_s[...].astype(F32)
    sc = jnp.broadcast_to(cf * jax.nn.sigmoid(cf), (8, D))

    def mod_vec(j):
        y = _dot(sc, pltpu.bitcast(wm_s[j], BF16))
        mod_s[j] = 1.0 + y if j in (1, 4) else y

    def mod(j, n, c=slice(None)):
        return jnp.concatenate([mod_s[j, :, c]] * (n // 8), axis=0)

    def put_a(r, top, bot):
        for m, v in enumerate(_strassen_lhs(
                top[:, :D2], top[:, D2:], bot[:, :D2], bot[:, D2:])):
            a_s[m][r, :] = _words(v)

    @pl.loop(0, X0 // 32)
    def _(i):
        r = pl.ds(pl.multiple_of(i * 32, 32), 32)
        h_s[r, :] = _ln(x_s[r, :].astype(F32))

    wait(cp_ca)
    mod_vec(1)
    wait(cp_sa)
    mod_vec(0)
    for i in range(LOOK // 32):
        put_a(pl.ds(i * 8, 8), *[
            h_s[pl.ds(i * 16 + off, 16), :] * mod(1, 16) + mod(0, 16)
            for off in (0, LOOK // 2)])
    in_s[pl.ds(M, RIDE), :] = h_s[pl.ds(LOOK, RIDE), :] * mod(1, RIDE) + mod(0, RIDE)

    def repack(p, u, c):
        par = []
        for odd in range(2):
            top, bot = [_halves(w_s[p, pl.ds(off + c * 32 + odd, 16, stride=2), :])
                        for off in (0, D2)]
            par.append(top + bot + _strassen_rhs_sums(*top, *bot))
        for e, pair in enumerate(zip(*par)):
            if e < 4:
                w_s[p, pl.ds((e // 2) * D2 + c * 32 + (e % 2) * 16, 16), :] = _join(*pair)
            else:
                w_s[T0 + 2 * u + (e - 4) // 4, pl.ds((e % 4) * K3 + c * 16, 16), :] = (
                    _join(*pair))

    def head(p, j, c0=0, c1=D // 32):
        return jnp.concatenate(
            [w_s[p, pl.ds(c * 32 + j * 16, 16), :] for c in range(c0, c1)], axis=0)

    cp_w(0).wait()
    for c in range(D2 // 32):
        repack(0, 0, c)

    @pl.loop(0, NP // 2)
    def _(i):
        two = w_s.at[pl.ds(2 * i + 1, 2)]
        pltpu.make_async_copy(two, two, sw.at[i + 1]).wait()
        for u in range(2):
            p = 2 * i + u

            def rhs(m):
                if _SUM[m] is None:
                    j = m // 4
                    return head(p, j, j * D2 // 32, (j + 1) * D2 // 32)
                return w_s[T0 + 2 * u + _SUM[m] // 4, pl.ds((_SUM[m] % 4) * K3, K3), :]

            jobs = [functools.partial(repack, p + 1, 1 - u, c) for c in range(D2 // 32)]
            cs = _strassen(lambda m: a_s[m][pl.ds(0, LOOK // 4), :], rhs,
                           _spread(jobs, 7))
            for q, y in enumerate(cs):
                ring_s[p, pl.ds(ROFF + (q // 2) * (LOOK // 2), LOOK // 2),
                       pl.ds((q % 2) * DH, DH)] = y.astype(BF16)

    for cp in cp_b:
        cp.start()
    wait(cp_a)
    in_s[pl.ds(0, M), :] = m0_s[...].astype(F32)

    KP = SEG + 2 * M
    row = lax.broadcasted_iota(jnp.int32, (L, KP), 0)
    col = lax.broadcasted_iota(jnp.int32, (L, KP), 1)
    visible = (col < L) & ((row < M) | (col >= SEG) | (row - M >= col))
    fill = jnp.where(col < L, -1e9, -jnp.inf).astype(F32)

    @pl.loop(0, NSEG)
    def _(s):
        seg = pl.ds(pl.multiple_of(s * SEG, SEG), SEG)
        nxt = pl.ds(pl.multiple_of(
            jnp.minimum(LOOK + (s + 1) * RIDE, S - RIDE), 8), RIDE)
        wr = pl.ds(pl.multiple_of(lax.rem(s * RIDE, RING), 8), RIDE)
        rd = pl.ds(pl.multiple_of(lax.rem(s * SEG + ROFF, RING), SEG), SEG)
        lhs_s[...] = _words(in_s[...])
        in_s[pl.ds(M, RIDE), :] = (
            _ln(x_s[nxt, :].astype(F32)) * mod(1, RIDE) + mod(0, RIDE))

        def project(p):
            w = jnp.concatenate([head(p, 0), head(p, 1)], axis=1)
            y = _dot(pltpu.bitcast(lhs_s[...], BF16), pltpu.bitcast(w, BF16))
            ring_s[p, wr, :] = y[M:].astype(BF16)
            return y[:M], ring_s[p, rd, :]

        def keys(p):
            mem, tok = project(p)
            tail = jnp.concatenate([mem, jnp.zeros_like(mem)], axis=0).astype(BF16)
            return jnp.concatenate([tok, tail], axis=0)

        def queries(p):
            mem, tok = project(2 * HP + p)
            return jnp.concatenate([mem, tok.astype(F32)], axis=0)

        def scores(qk):
            q, k = qk
            out = []
            for i in range(2):
                c = slice(i * DH, (i + 1) * DH)
                z = jnp.where(visible, _dot(q[:, c], k[:, c], _NT) * scale, fill)
                e = jnp.exp(z - jnp.max(z, axis=-1, keepdims=True))
                out.append((e, 1.0 / jnp.sum(e, axis=-1, keepdims=True)))
            return out

        def mix(p, es, v):
            for i, (e, inv) in enumerate(es):
                c = slice(i * DH, (i + 1) * DH)
                o_s[p, :, c] = _dot(e, v[:, c]) * inv

        def out_proj(p0, p1, j):
            c = pl.ds(j * 128, 128)
            lhs = jnp.concatenate([o_s[p] for p in range(p0, p1)], axis=1)
            w = wo_s[pl.ds(p0 * DH, (p1 - p0) * DH), c]
            return _dot(lhs, pltpu.bitcast(w, BF16))

        qk, es, vs = {}, {}, {}
        for t in range(HP + 2):
            if t < HP:
                k = keys(t)
                qk[t] = queries(t), k
            else:
                for j in range((t - HP) * CT // 2, (t - HP + 1) * CT // 2):
                    acc_s[:, pl.ds(j * 128, 128)] = out_proj(0, HP // 2, j)
            if 1 <= t <= HP:
                es[t - 1] = scores(qk.pop(t - 1))
                vs[t - 1] = keys(HP + t - 1)
            if t >= 2:
                mix(t - 2, es.pop(t - 2), vs.pop(t - 2))
        for j in range(CT):
            c = pl.ds(j * 128, 128)
            acc = acc_s[:, c] + out_proj(HP // 2, HP, j)
            in_s[pl.ds(0, M), c] = acc[:M]
            h_s[seg, c] = acc[M:]

    NB = S // RB
    G = CT // 4
    FT = w3_s.shape[1] // 128
    FH, CH, RH = FT // 2, CT // 2, RB // 2
    NI = NB // 2
    K4 = FT * 32

    def rows(i, off, n):
        return pl.ds(pl.multiple_of(i * RB + off, n), n)

    def col(j):
        return pl.ds(j * 128, 128)

    def block12(k, j):
        return lambda q: (mix_tile(k, j + (q % 2) * CH), (q // 2) * K3, slice(None))

    def block3(f):
        return lambda q: (w3_s, (q // 2) * K3, col(f + (q % 2) * FH))

    def block4(j):
        return lambda q: (w4_s, (q // 2) * K4, col(j + (q % 2) * CH))

    def home12(k, j):
        n = 5 * (CH * k + j)
        return lambda e: (2 * ((n + e) // 3) + 1, (1 + (n + e) % 3) * K3)

    def home3(f):
        return lambda e: (2 * f + e // 4, (e % 4) * K3)

    def home4(j):
        return lambda e: (2 * FH + 5 * j + e, 0)

    def make(block, home, r0):
        w = []
        for q in range(4):
            ref, off, c = block(q)
            w.append(_halves(ref[pl.ds(off + r0, 16), c]))
        lo, hi = [_strassen_rhs_sums(*v) for v in zip(*w)]
        for e, pair in enumerate(zip(lo, hi)):
            slot, off = home(e)
            w_s[slot, pl.ds(off + r0, 16), :] = _join(*pair)

    def get_w(block, home, n):
        def rhs(m):
            if _SUM[m] is None:
                ref, off, c = block(0 if m == 1 else 3)
                return ref[pl.ds(off, n), c]
            slot, off = home(_SUM[m])
            return w_s[slot, pl.ds(off, n), :]
        return rhs

    def get_a(i):
        return lambda m: a_s[m][pl.ds(pl.multiple_of(i * (RH // 2), 8), RH // 2), :]

    def put(i, g, half):
        put_a(pl.ds(pl.multiple_of(i * (RH // 2) + g * 8, 8), 8),
              half(g * 16), half(RH + g * 16))

    def norm1(i, g):
        def half(off):
            r = rows(i, off, 16)
            x1 = x_s[r, :].astype(F32) + mod(2, 16) * h_s[r, :]
            hb = _ln(x1) * mod(4, 16) + mod(3, 16)
            r_s[r, :] = hb
            return _ln(hb)
        put(i, g, half)

    def shifted(i, g):
        put(i, g, lambda off: jnp.concatenate(
            [hh_s[k, pl.ds(8 + i * RB + off + (-1, 1, -2, 2)[k // G], 16), :]
             for k in range(CT)], axis=1))

    def norm2(i, g):
        put(i, g, lambda off: _ln(r_s[rows(i, off, 16), :]))

    NG = RH // 16

    wait(cp_b)
    for j in (2, 3, 4, 5):
        mod_vec(j)
        for r0 in range(0, K3, 16):
            make(block12(0, j - 2), home12(0, j - 2), r0)
    for j in range(CT):
        hh_s[j, pl.ds(0, 8), :] = jnp.zeros((8, 128), F32)
        hh_s[j, pl.ds(8 + S, 8), :] = jnp.zeros((8, 128), F32)
    for g in range(NG):
        norm1(0, g)

    @pl.loop(0, NI)
    def _(ii):
        for u in range(2):
            i = 2 * ii + u
            jobs = []
            for g in range(NG):
                jobs.append(functools.partial(norm1, jnp.minimum(i + 1, NB - 1), g))
                jobs.append(functools.partial(
                    make, block12(1, g % CH), home12(1, g % CH),
                    pl.multiple_of(i * (K3 // NB) + (g // CH) * 16, 8)))
            tick = _spread(jobs, 7 * CH, 8)
            for j in range(CH):
                cs = _strassen(get_a(i), get_w(block12(0, j), home12(0, j), K3), tick)
                for q, y in enumerate(cs):
                    hh_s[j + (q % 2) * CH,
                         pl.ds(pl.multiple_of(8 + i * RB + (q // 2) * RH, 8), RH), :] = (
                             _gelu(y))

    for g in range(NG):
        shifted(0, g)

    @pl.loop(0, NI)
    def _(ii):
        for u in range(2):
            i = 2 * ii + u
            work = [(block3(f), home3(f), i * (K3 // NB) + v * 16)
                    for f in range(FH) for v in range(K3 // NB // 16)]
            work += [(block4(j), home4(j), i * (K4 // NB) + v * 16)
                     for j in range(CH) for v in range(K4 // NB // 16)]
            jobs = []
            for g in range(NG):
                jobs.append(functools.partial(shifted, jnp.minimum(i + 1, NB - 1), g))
                jobs += [functools.partial(make, b, h, pl.multiple_of(r0, 8))
                         for b, h, r0 in work[g::NG]]
            tick = _spread(jobs, 7 * CH)
            for j in range(CH):
                cs = _strassen(get_a(i), get_w(block12(1, j), home12(1, j), K3), tick)
                for q, y in enumerate(cs):
                    r_s[rows(i, (q // 2) * RH, RH), col(j + (q % 2) * CH)] += y

    def cp_y(i):
        return pltpu.make_async_copy(
            y_s.at[i % 2], out_hbm.at[rows(i, 0, RB)], sy.at[i % 2])

    for g in range(NG):
        norm2(0, g)

    @pl.loop(0, NB)
    def _(i):
        @pl.when(i >= 2)
        def _():
            cp_y(i - 2).wait()

        for f in range(FH):
            cs = _strassen(get_a(i), get_w(block3(f), home3(f), K3))
            for m, v in enumerate(_strassen_lhs(*map(_gelu, cs))):
                t_s[m][:, col(f)] = _words(v)
        for j in range(CH):
            cs = _strassen(lambda m: t_s[m][...], get_w(block4(j), home4(j), K4))
            for q, h2 in enumerate(cs):
                r, c = rows(i, (q // 2) * RH, RH), col(j + (q % 2) * CH)
                x1 = x_s[r, c].astype(F32) + mod(2, RH, c) * h_s[r, c]
                y = x1 + mod(5, RH, c) * (r_s[r, c] + h2)
                y_s[i % 2, pl.ds((q // 2) * RH, RH), c] = y.astype(y_s.dtype)
            if j < 2:
                for g in range(j * NG // 2, (j + 1) * NG // 2):
                    norm2(jnp.minimum(i + 1, NB - 1), g)
        cp_y(i).start()

    cp_y(NB - 2).wait()
    cp_y(NB - 1).wait()


@functools.partial(jax.jit, static_argnames=("A_seg_len",))
def pallas_adaLN_cond__memory_aug_recurrent_mem_tr__mixer_s_mlp__prompt_kernel(
    A_x, A_mem0, A_Wq, A_Wk, A_Wv, A_Wo, A_seg_len, B_x, B_w1, B_w2, B_w3, B_w4,
    c, w_mod,
):
    del B_x
    _, S, D = A_x.shape
    _, H, DH = A_Wq.shape
    M = A_mem0.shape[1]
    SEG = int(A_seg_len)
    FF = B_w3.shape[1]
    HP = H // 2
    RB = 256
    LOOK = S - (S // SEG) * (SEG - M)
    RING = LOOK + 64
    vm = pltpu.VMEM
    dma = pltpu.SemaphoreType.DMA
    scratch = [
        vm((3 * HP + 1 + D // 128, D, DH), U32), vm((HP * DH, D), U32),
        vm((D // 2, FF), U32), vm((FF // 2, D), U32), vm((6, D // 2, D), U32),
        vm((S, D), A_x.dtype), vm((S, D), F32), vm((S, D), F32),
        vm((D // 128, S + 16, 128), F32), vm((3 * HP, RING, 2 * DH), BF16),
        vm((1, D), c.dtype), vm((M, D), A_mem0.dtype),
        vm((SEG, D), F32), vm((SEG // 2, D), U32),
        vm((HP, M + SEG, 2 * DH), F32), vm((M + SEG, D), F32), vm((6, 8, D), F32),
        [vm((S // 4, D // 2), U32)] * 7, [vm((RB // 4, FF // 2), U32)] * 7,
        vm((2, RB, D), A_x.dtype),
        dma((3 * HP // 2 + 1,)), dma((5,)), dma((2,)),
    ]
    out = pl.pallas_call(
        functools.partial(_kernel, S=S, D=D, H=H, DH=DH, M=M, SEG=SEG, RB=RB),
        out_shape=jax.ShapeDtypeStruct((S, D), A_x.dtype),
        in_specs=[pl.BlockSpec(memory_space=pl.ANY)] * 12,
        out_specs=pl.BlockSpec(memory_space=pl.ANY),
        scratch_shapes=scratch,
        compiler_params=pltpu.CompilerParams(
            vmem_limit_bytes=124 * 1024 * 1024,
            flags={"XLA_TPU_EVENLY_DISTRIBUTE_CRITICAL_NODES": True}),
    )(A_x.reshape(S, D), A_mem0.reshape(M, D), A_Wq, A_Wk, A_Wv,
      A_Wo.reshape(H * DH, D), B_w1, B_w2, B_w3, B_w4, c, w_mod)
    return out.reshape(A_x.shape)
```

```python
import functools

import jax
import jax.numpy as jnp
import numpy as np
from jax import lax
import jax.experimental.pallas as pl
import jax.experimental.pallas.tpu as pltpu

F32 = jnp.float32
BF16 = jnp.bfloat16
U32 = jnp.uint32

_NN = (((1,), (0,)), ((), ()))
_NT = (((1,), (1,)), ((), ()))


def _dot(a, b, dims=_NN):
    return lax.dot_general(a, b, dims, preferred_element_type=F32)


def _ln(x):
    m = jnp.mean(x, axis=-1, keepdims=True)
    d = x - m
    v = jnp.mean(d * d, axis=-1, keepdims=True)
    return d * lax.rsqrt(v + 1e-5)


def _gelu(x):
    k0 = float(np.sqrt(2.0 / np.pi))
    k1 = float(np.sqrt(2.0 / np.pi) * 0.044715)
    hx = 0.5 * x
    return hx + hx * jnp.tanh(x * (k0 + k1 * (x * x)))


def _words(x):
    return pltpu.bitcast(x.astype(BF16), U32)


def _halves(w):
    return (pltpu.bitcast(w << 16, F32),
            pltpu.bitcast(w & np.uint32(0xFFFF0000), F32))


def _words_each(xs):
    w = _words(jnp.concatenate(xs, axis=1))
    return [w[:, e * 128:(e + 1) * 128] for e in range(len(xs))]


def _spread(jobs, slots, first=1):
    state = [0, 0]

    def tick():
        state[0] += 1
        while state[1] < min(len(jobs), -(-(state[0] - first) * len(jobs) // (slots - first))):
            jobs[state[1]]()
            state[1] += 1
    return tick


def _strassen_lhs(a11, a12, a21, a22):
    return (a11 + a22, a21 + a22, a11, a22, a11 + a12, a21 - a11, a12 - a22)


def _strassen_rhs_sums(b11, b12, b21, b22):
    return (b11 + b22, b12 - b22, b21 - b11, b11 + b12, b21 + b22)


_SUM = (0, None, 1, 2, None, 3, 4)


def _strassen(lhs, rhs, tick=lambda: None):
    def prod(m):
        tick()
        return _dot(pltpu.bitcast(lhs(m), BF16), pltpu.bitcast(rhs(m), BF16))

    m0, m1 = prod(0), prod(1)
    c22 = m0 - m1
    m3 = prod(3)
    c11 = m0 + m3
    c21 = m1 + m3
    m2 = prod(2)
    c22 = c22 + m2
    m4 = prod(4)
    c12 = m2 + m4
    c11 = c11 - m4
    c22 = c22 + prod(5)
    c11 = c11 + prod(6)
    return c11, c12, c21, c22


def _kernel(x_hbm, mem_hbm, wq_hbm, wk_hbm, wv_hbm, wo_hbm, w1_hbm, w2_hbm,
            w3_hbm, w4_hbm, c_hbm, wm_hbm, out_hbm,
            w_s, wo_s, w3_s, w4_s, wm_s, x_s, h_s, r_s, hh_s, ring_s,
            c_s, m0_s, in_s, lhs_s, o_s, acc_s, mod_s, a_s, t_s, y_s,
            sw, sx, sy,
            *, S, D, H, DH, M, SEG, RB):
    HP = H // 2
    NP = 3 * HP
    T0 = NP + 1
    NSEG = S // SEG
    L = M + SEG
    RIDE = SEG - M
    LOOK = S - NSEG * RIDE
    RING = ring_s.shape[1]
    ROFF = RING - LOOK
    D2 = D // 2
    K3 = D // 4
    CT = D // 128
    X0 = LOOK + 32
    scale = float(DH) ** -0.5

    def cp_w(p):
        src = (wk_hbm, wv_hbm, wq_hbm)[p // HP % 3].bitcast(U32)
        return pltpu.make_async_copy(
            src.at[:, p % HP], w_s.at[p], sw.at[(p + 1) // 2])

    def mix_tile(k, j):
        return w_s.at[T0 + j, pl.ds(k * D2, D2)]

    def copies(pairs, sem):
        return [pltpu.make_async_copy(src, dst, sem) for src, dst in pairs]

    def mod_pair(j):
        return wm_hbm.bitcast(U32).at[:, pl.ds(j * D, D)], wm_s.at[j]

    cp_first = copies([(c_hbm, c_s),
                       (x_hbm.at[pl.ds(0, X0)], x_s.at[pl.ds(0, X0)])], sx.at[0])
    cp_ca = copies([mod_pair(1)], sx.at[1])
    cp_sa = copies([mod_pair(0)], sx.at[2])
    cp_a = copies([(mem_hbm, m0_s),
                   (x_hbm.at[pl.ds(X0, S - X0)], x_s.at[pl.ds(X0, S - X0)]),
                   (wo_hbm.bitcast(U32), wo_s)], sx.at[3])
    cp_b = copies(
        [mod_pair(j) for j in range(2, 6)]
        + [(src.bitcast(U32).at[:, pl.ds(j * 128, 128)], mix_tile(k, j))
           for k, src in enumerate((w1_hbm, w2_hbm)) for j in range(CT)]
        + [(w3_hbm.bitcast(U32), w3_s), (w4_hbm.bitcast(U32), w4_s)], sx.at[4])

    def wait(cps):
        for cp in cps:
            cp.wait()

    for cp in cp_first + cp_ca + cp_sa + [cp_w(p) for p in range(NP + 1)] + cp_a:
        cp.start()

    wait(cp_first)
    cf = c_s[...].astype(F32)
    sc = jnp.broadcast_to(cf * jax.nn.sigmoid(cf), (8, D))

    def mod_vec(j):
        y = _dot(sc, pltpu.bitcast(wm_s[j], BF16))
        mod_s[j] = 1.0 + y if j in (1, 4) else y

    def mod(j, n, c=slice(None)):
        return jnp.concatenate([mod_s[j, :, c]] * (n // 8), axis=0)

    def put_a(r, top, bot):
        for m, v in enumerate(_strassen_lhs(
                top[:, :D2], top[:, D2:], bot[:, :D2], bot[:, D2:])):
            a_s[m][r, :] = _words(v)

    @pl.loop(0, X0 // 32)
    def _(i):
        r = pl.ds(pl.multiple_of(i * 32, 32), 32)
        h_s[r, :] = _ln(x_s[r, :].astype(F32))

    wait(cp_ca)
    mod_vec(1)
    wait(cp_sa)
    mod_vec(0)
    for i in range(LOOK // 32):
        put_a(pl.ds(i * 8, 8), *[
            h_s[pl.ds(i * 16 + off, 16), :] * mod(1, 16) + mod(0, 16)
            for off in (0, LOOK // 2)])
    in_s[pl.ds(M, RIDE), :] = h_s[pl.ds(LOOK, RIDE), :] * mod(1, RIDE) + mod(0, RIDE)

    def repack(p, u, c):
        top, bot = [_halves(w_s[p, pl.ds(off + c * 32, 32), :]) for off in (0, D2)]
        for e, v in enumerate(_words_each(
                top + bot + _strassen_rhs_sums(*top, *bot))):
            if e < 4:
                w_s[p, pl.ds((e // 2) * D2 + c * 32 + (e % 2) * 16, 16), :] = v
            else:
                w_s[T0 + 2 * u + (e - 4) // 4, pl.ds((e % 4) * K3 + c * 16, 16), :] = v

    def head(p, j, c0=0, c1=D // 32):
        return jnp.concatenate(
            [w_s[p, pl.ds(c * 32 + j * 16, 16), :] for c in range(c0, c1)], axis=0)

    cp_w(0).wait()
    for c in range(D2 // 32):
        repack(0, 0, c)

    @pl.loop(0, NP // 2)
    def _(i):
        two = w_s.at[pl.ds(2 * i + 1, 2)]
        pltpu.make_async_copy(two, two, sw.at[i + 1]).wait()
        for u in range(2):
            p = 2 * i + u

            def rhs(m):
                if _SUM[m] is None:
                    j = m // 4
                    return head(p, j, j * D2 // 32, (j + 1) * D2 // 32)
                return w_s[T0 + 2 * u + _SUM[m] // 4, pl.ds((_SUM[m] % 4) * K3, K3), :]

            jobs = [functools.partial(repack, p + 1, 1 - u, c) for c in range(D2 // 32)]
            cs = _strassen(lambda m: a_s[m][pl.ds(0, LOOK // 4), :], rhs,
                           _spread(jobs, 7))
            for q, y in enumerate(cs):
                ring_s[p, pl.ds(ROFF + (q // 2) * (LOOK // 2), LOOK // 2),
                       pl.ds((q % 2) * DH, DH)] = y.astype(BF16)

    for cp in cp_b:
        cp.start()
    wait(cp_a)
    in_s[pl.ds(0, M), :] = m0_s[...].astype(F32)

    KP = SEG + 2 * M
    row = lax.broadcasted_iota(jnp.int32, (L, KP), 0)
    col = lax.broadcasted_iota(jnp.int32, (L, KP), 1)
    visible = (col < L) & ((row < M) | (col >= SEG) | (row - M >= col))
    fill = jnp.where(col < L, -1e9, -jnp.inf).astype(F32)

    @pl.loop(0, NSEG)
    def _(s):
        seg = pl.ds(pl.multiple_of(s * SEG, SEG), SEG)
        nxt = pl.ds(pl.multiple_of(
            jnp.minimum(LOOK + (s + 1) * RIDE, S - RIDE), 8), RIDE)
        wr = pl.ds(pl.multiple_of(lax.rem(s * RIDE, RING), 8), RIDE)
        rd = pl.ds(pl.multiple_of(lax.rem(s * SEG + ROFF, RING), SEG), SEG)
        lhs_s[...] = _words(in_s[...])
        in_s[pl.ds(M, RIDE), :] = (
            _ln(x_s[nxt, :].astype(F32)) * mod(1, RIDE) + mod(0, RIDE))

        def project(p):
            w = jnp.concatenate([head(p, 0), head(p, 1)], axis=1)
            y = _dot(pltpu.bitcast(lhs_s[...], BF16), pltpu.bitcast(w, BF16))
            ring_s[p, wr, :] = y[M:].astype(BF16)
            return y[:M], ring_s[p, rd, :]

        def keys(p):
            mem, tok = project(p)
            tail = jnp.concatenate([mem, jnp.zeros_like(mem)], axis=0).astype(BF16)
            return jnp.concatenate([tok, tail], axis=0)

        def queries(p):
            mem, tok = project(2 * HP + p)
            return jnp.concatenate([mem, tok.astype(F32)], axis=0)

        def scores(qk):
            q, k = qk
            out = []
            for i in range(2):
                c = slice(i * DH, (i + 1) * DH)
                z = jnp.where(visible, _dot(q[:, c], k[:, c], _NT) * scale, fill)
                e = jnp.exp(z - jnp.max(z, axis=-1, keepdims=True))
                out.append((e, 1.0 / jnp.sum(e, axis=-1, keepdims=True)))
            return out

        def mix(p, es, v):
            for i, (e, inv) in enumerate(es):
                c = slice(i * DH, (i + 1) * DH)
                o_s[p, :, c] = _dot(e, v[:, c]) * inv

        def out_proj(p0, p1, j):
            c = pl.ds(j * 128, 128)
            lhs = jnp.concatenate([o_s[p] for p in range(p0, p1)], axis=1)
            w = wo_s[pl.ds(p0 * DH, (p1 - p0) * DH), c]
            return _dot(lhs, pltpu.bitcast(w, BF16))

        qk, es, vs = {}, {}, {}
        for t in range(HP + 2):
            if t < HP:
                k = keys(t)
                qk[t] = queries(t), k
            else:
                for j in range((t - HP) * CT // 2, (t - HP + 1) * CT // 2):
                    acc_s[:, pl.ds(j * 128, 128)] = out_proj(0, HP // 2, j)
            if 1 <= t <= HP:
                es[t - 1] = scores(qk.pop(t - 1))
                vs[t - 1] = keys(HP + t - 1)
            if t >= 2:
                mix(t - 2, es.pop(t - 2), vs.pop(t - 2))
        for j in range(CT):
            c = pl.ds(j * 128, 128)
            acc = acc_s[:, c] + out_proj(HP // 2, HP, j)
            in_s[pl.ds(0, M), c] = acc[:M]
            h_s[seg, c] = acc[M:]

    NB = S // RB
    G = CT // 4
    FT = w3_s.shape[1] // 128
    FH, CH, RH = FT // 2, CT // 2, RB // 2
    NI = NB // 2
    K4 = FT * 32

    def rows(i, off, n):
        return pl.ds(pl.multiple_of(i * RB + off, n), n)

    def col(j):
        return pl.ds(j * 128, 128)

    def block12(k, j):
        return lambda q: (mix_tile(k, j + (q % 2) * CH), (q // 2) * K3, slice(None))

    def block3(f):
        return lambda q: (w3_s, (q // 2) * K3, col(f + (q % 2) * FH))

    def block4(j):
        return lambda q: (w4_s, (q // 2) * K4, col(j + (q % 2) * CH))

    def home12(k, j):
        n = 5 * (CH * k + j)
        return lambda e: (2 * ((n + e) // 3) + 1, (1 + (n + e) % 3) * K3)

    def home3(f):
        return lambda e: (2 * f + e // 4, (e % 4) * K3)

    def home4(j):
        return lambda e: (2 * FH + 5 * j + e, 0)

    def make(block, home, r0):
        w = [ref[pl.ds(off + r0, 16), c] for ref, off, c in map(block, range(4))]
        w = pltpu.bitcast(jnp.concatenate(w, axis=1), BF16).astype(F32)
        for e, v in enumerate(_words_each(_strassen_rhs_sums(
                *[w[:, q * 128:(q + 1) * 128] for q in range(4)]))):
            slot, off = home(e)
            w_s[slot, pl.ds(off + r0, 16), :] = v

    def get_w(block, home, n):
        def rhs(m):
            if _SUM[m] is None:
                ref, off, c = block(0 if m == 1 else 3)
                return ref[pl.ds(off, n), c]
            slot, off = home(_SUM[m])
            return w_s[slot, pl.ds(off, n), :]
        return rhs

    def get_a(i):
        return lambda m: a_s[m][pl.ds(pl.multiple_of(i * (RH // 2), 8), RH // 2), :]

    def put(i, g, half):
        put_a(pl.ds(pl.multiple_of(i * (RH // 2) + g * 8, 8), 8),
              half(g * 16), half(RH + g * 16))

    def norm1(i, g):
        def half(off):
            r = rows(i, off, 16)
            x1 = x_s[r, :].astype(F32) + mod(2, 16) * h_s[r, :]
            hb = _ln(x1) * mod(4, 16) + mod(3, 16)
            r_s[r, :] = hb
            return _ln(hb)
        put(i, g, half)

    def shifted(i, g):
        put(i, g, lambda off: jnp.concatenate(
            [hh_s[k, pl.ds(8 + i * RB + off + (-1, 1, -2, 2)[k // G], 16), :]
             for k in range(CT)], axis=1))

    def norm2(i, g):
        put(i, g, lambda off: _ln(r_s[rows(i, off, 16), :]))

    NG = RH // 16

    wait(cp_b)
    for j in (2, 3, 4, 5):
        mod_vec(j)
        for r0 in range(0, K3, 16):
            make(block12(0, j - 2), home12(0, j - 2), r0)
    for j in range(CT):
        hh_s[j, pl.ds(0, 8), :] = jnp.zeros((8, 128), F32)
        hh_s[j, pl.ds(8 + S, 8), :] = jnp.zeros((8, 128), F32)
    for g in range(NG):
        norm1(0, g)

    @pl.loop(0, NI)
    def _(ii):
        for u in range(2):
            i = 2 * ii + u
            jobs = []
            for g in range(NG):
                jobs.append(functools.partial(norm1, jnp.minimum(i + 1, NB - 1), g))
                jobs.append(functools.partial(
                    make, block12(1, g % CH), home12(1, g % CH),
                    pl.multiple_of(i * (K3 // NB) + (g // CH) * 16, 8)))
            tick = _spread(jobs, 7 * CH, 8)
            for j in range(CH):
                cs = _strassen(get_a(i), get_w(block12(0, j), home12(0, j), K3), tick)
                for q, y in enumerate(cs):
                    hh_s[j + (q % 2) * CH,
                         pl.ds(pl.multiple_of(8 + i * RB + (q // 2) * RH, 8), RH), :] = (
                             _gelu(y))

    for g in range(NG):
        shifted(0, g)

    @pl.loop(0, NI)
    def _(ii):
        for u in range(2):
            i = 2 * ii + u
            work = [(block3(f), home3(f), i * (K3 // NB) + v * 16)
                    for f in range(FH) for v in range(K3 // NB // 16)]
            work += [(block4(j), home4(j), i * (K4 // NB) + v * 16)
                     for j in range(CH) for v in range(K4 // NB // 16)]
            jobs = []
            for g in range(NG):
                jobs.append(functools.partial(shifted, jnp.minimum(i + 1, NB - 1), g))
                jobs += [functools.partial(make, b, h, pl.multiple_of(r0, 8))
                         for b, h, r0 in work[g::NG]]
            tick = _spread(jobs, 7 * CH)
            for j in range(CH):
                cs = _strassen(get_a(i), get_w(block12(1, j), home12(1, j), K3), tick)
                for q, y in enumerate(cs):
                    r_s[rows(i, (q // 2) * RH, RH), col(j + (q % 2) * CH)] += y

    def cp_y(i):
        return pltpu.make_async_copy(
            y_s.at[i % 2], out_hbm.at[rows(i, 0, RB)], sy.at[i % 2])

    for g in range(NG):
        norm2(0, g)

    @pl.loop(0, NB)
    def _(i):
        @pl.when(i >= 2)
        def _():
            cp_y(i - 2).wait()

        for f in range(FH):
            cs = _strassen(get_a(i), get_w(block3(f), home3(f), K3))
            for m, v in enumerate(_strassen_lhs(*map(_gelu, cs))):
                t_s[m][:, col(f)] = _words(v)
        for j in range(CH):
            cs = _strassen(lambda m: t_s[m][...], get_w(block4(j), home4(j), K4))
            for q, h2 in enumerate(cs):
                r, c = rows(i, (q // 2) * RH, RH), col(j + (q % 2) * CH)
                x1 = x_s[r, c].astype(F32) + mod(2, RH, c) * h_s[r, c]
                y = x1 + mod(5, RH, c) * (r_s[r, c] + h2)
                y_s[i % 2, pl.ds((q // 2) * RH, RH), c] = y.astype(y_s.dtype)
            if j < 2:
                for g in range(j * NG // 2, (j + 1) * NG // 2):
                    norm2(jnp.minimum(i + 1, NB - 1), g)
        cp_y(i).start()

    cp_y(NB - 2).wait()
    cp_y(NB - 1).wait()


@functools.partial(jax.jit, static_argnames=("A_seg_len",))
def pallas_adaLN_cond__memory_aug_recurrent_mem_tr__mixer_s_mlp__prompt_kernel(
    A_x, A_mem0, A_Wq, A_Wk, A_Wv, A_Wo, A_seg_len, B_x, B_w1, B_w2, B_w3, B_w4,
    c, w_mod,
):
    del B_x
    _, S, D = A_x.shape
    _, H, DH = A_Wq.shape
    M = A_mem0.shape[1]
    SEG = int(A_seg_len)
    FF = B_w3.shape[1]
    HP = H // 2
    RB = 256
    LOOK = S - (S // SEG) * (SEG - M)
    RING = LOOK + 64
    vm = pltpu.VMEM
    dma = pltpu.SemaphoreType.DMA
    scratch = [
        vm((3 * HP + 1 + D // 128, D, DH), U32), vm((HP * DH, D), U32),
        vm((D // 2, FF), U32), vm((FF // 2, D), U32), vm((6, D // 2, D), U32),
        vm((S, D), A_x.dtype), vm((S, D), F32), vm((S, D), F32),
        vm((D // 128, S + 16, 128), F32), vm((3 * HP, RING, 2 * DH), BF16),
        vm((1, D), c.dtype), vm((M, D), A_mem0.dtype),
        vm((SEG, D), F32), vm((SEG // 2, D), U32),
        vm((HP, M + SEG, 2 * DH), F32), vm((M + SEG, D), F32), vm((6, 8, D), F32),
        [vm((S // 4, D // 2), U32)] * 7, [vm((RB // 4, FF // 2), U32)] * 7,
        vm((2, RB, D), A_x.dtype),
        dma((3 * HP // 2 + 1,)), dma((5,)), dma((2,)),
    ]
    out = pl.pallas_call(
        functools.partial(_kernel, S=S, D=D, H=H, DH=DH, M=M, SEG=SEG, RB=RB),
        out_shape=jax.ShapeDtypeStruct((S, D), A_x.dtype),
        in_specs=[pl.BlockSpec(memory_space=pl.ANY)] * 12,
        out_specs=pl.BlockSpec(memory_space=pl.ANY),
        scratch_shapes=scratch,
        compiler_params=pltpu.CompilerParams(
            vmem_limit_bytes=124 * 1024 * 1024,
            flags={"XLA_TPU_EVENLY_DISTRIBUTE_CRITICAL_NODES": True}),
    )(A_x.reshape(S, D), A_mem0.reshape(M, D), A_Wq, A_Wk, A_Wv,
      A_Wo.reshape(H * DH, D), B_w1, B_w2, B_w3, B_w4, c, w_mod)
    return out.reshape(A_x.shape)
```

```python
import functools

import jax
import jax.numpy as jnp
import numpy as np
from jax import lax
import jax.experimental.pallas as pl
import jax.experimental.pallas.tpu as pltpu

F32 = jnp.float32
BF16 = jnp.bfloat16
U32 = jnp.uint32

_NN = (((1,), (0,)), ((), ()))
_NT = (((1,), (1,)), ((), ()))


def _dot(a, b, dims=_NN):
    return lax.dot_general(a, b, dims, preferred_element_type=F32)


def _ln(x):
    m = jnp.mean(x, axis=-1, keepdims=True)
    d = x - m
    v = jnp.mean(d * d, axis=-1, keepdims=True)
    return d * lax.rsqrt(v + 1e-5)


def _gelu(x):
    k0 = float(np.sqrt(2.0 / np.pi))
    k1 = float(np.sqrt(2.0 / np.pi) * 0.044715)
    hx = 0.5 * x
    return hx + hx * jnp.tanh(x * (k0 + k1 * (x * x)))


def _words(x):
    return pltpu.bitcast(x.astype(BF16), U32)


def _halves(w):
    return (pltpu.bitcast(w << 16, F32),
            pltpu.bitcast(w & np.uint32(0xFFFF0000), F32))


def _words_each(xs):
    w = _words(jnp.concatenate(xs, axis=1))
    return [w[:, e * 128:(e + 1) * 128] for e in range(len(xs))]


def _spread(jobs, slots, first=1):
    state = [0, 0]

    def tick():
        state[0] += 1
        while state[1] < min(len(jobs), -(-(state[0] - first) * len(jobs) // (slots - first))):
            jobs[state[1]]()
            state[1] += 1
    return tick


def _strassen_lhs(a11, a12, a21, a22):
    return (a11 + a22, a21 + a22, a11, a22, a11 + a12, a21 - a11, a12 - a22)


def _strassen_rhs_sums(b11, b12, b21, b22):
    return (b11 + b22, b12 - b22, b21 - b11, b11 + b12, b21 + b22)


_SUM = (0, None, 1, 2, None, 3, 4)


def _strassen(lhs, rhs, tick=lambda: None):
    def prod(m):
        tick()
        return _dot(pltpu.bitcast(lhs(m), BF16), pltpu.bitcast(rhs(m), BF16))

    m0, m1 = prod(0), prod(1)
    c22 = m0 - m1
    m3 = prod(3)
    c11 = m0 + m3
    c21 = m1 + m3
    m2 = prod(2)
    c22 = c22 + m2
    m4 = prod(4)
    c12 = m2 + m4
    c11 = c11 - m4
    c22 = c22 + prod(5)
    c11 = c11 + prod(6)
    return c11, c12, c21, c22


def _kernel(x_hbm, mem_hbm, wq_hbm, wk_hbm, wv_hbm, wo_hbm, w1_hbm, w2_hbm,
            w3_hbm, w4_hbm, c_hbm, wm_hbm, out_hbm,
            w_s, wo_s, w3_s, w4_s, wm_s, x_s, h_s, r_s, hh_s, ring_s,
            c_s, m0_s, in_s, lhs_s, o_s, acc_s, mod_s, a_s, t_s, y_s,
            sw, sx, sy,
            *, S, D, H, DH, M, SEG, RB):
    HP = H // 2
    NP = 3 * HP
    T0 = NP + 1
    NSEG = S // SEG
    L = M + SEG
    RIDE = SEG - M
    LOOK = S - NSEG * RIDE
    RING = ring_s.shape[1]
    ROFF = RING - LOOK
    D2 = D // 2
    K3 = D // 4
    CT = D // 128
    X0 = LOOK + 32
    scale = float(DH) ** -0.5

    def cp_w(p):
        src = (wk_hbm, wv_hbm, wq_hbm)[p // HP % 3].bitcast(U32)
        return pltpu.make_async_copy(
            src.at[:, p % HP], w_s.at[p], sw.at[(p + 1) // 2])

    def mix_tile(k, j):
        return w_s.at[T0 + j, pl.ds(k * D2, D2)]

    def copies(pairs, sem):
        return [pltpu.make_async_copy(src, dst, sem) for src, dst in pairs]

    def mod_pair(j):
        return wm_hbm.bitcast(U32).at[:, pl.ds(j * D, D)], wm_s.at[j]

    cp_first = copies([(c_hbm, c_s),
                       (x_hbm.at[pl.ds(0, X0)], x_s.at[pl.ds(0, X0)])], sx.at[0])
    cp_ca = copies([mod_pair(1)], sx.at[1])
    cp_sa = copies([mod_pair(0)], sx.at[2])
    cp_a = copies([(mem_hbm, m0_s),
                   (x_hbm.at[pl.ds(X0, S - X0)], x_s.at[pl.ds(X0, S - X0)]),
                   (wo_hbm.bitcast(U32), wo_s)], sx.at[3])
    cp_b = copies(
        [mod_pair(j) for j in range(2, 6)]
        + [(src.bitcast(U32).at[:, pl.ds(j * 128, 128)], mix_tile(k, j))
           for k, src in enumerate((w1_hbm, w2_hbm)) for j in range(CT)]
        + [(w3_hbm.bitcast(U32), w3_s), (w4_hbm.bitcast(U32), w4_s)], sx.at[4])

    def wait(cps):
        for cp in cps:
            cp.wait()

    for cp in cp_first + cp_ca + cp_sa + [cp_w(p) for p in range(NP + 1)] + cp_a:
        cp.start()

    wait(cp_first)
    cf = c_s[...].astype(F32)
    sc = jnp.broadcast_to(cf * jax.nn.sigmoid(cf), (8, D))

    def mod_vec(j):
        y = _dot(sc, pltpu.bitcast(wm_s[j], BF16))
        mod_s[j] = 1.0 + y if j in (1, 4) else y

    def mod(j, n, c=slice(None)):
        return jnp.concatenate([mod_s[j, :, c]] * (n // 8), axis=0)

    def put_a(u, r, top, bot):
        for m, v in enumerate(_strassen_lhs(
                top[:, :D2], top[:, D2:], bot[:, :D2], bot[:, D2:])):
            a_s[u][m][r, :] = _words(v)

    @pl.loop(0, X0 // 32)
    def _(i):
        r = pl.ds(pl.multiple_of(i * 32, 32), 32)
        h_s[r, :] = _ln(x_s[r, :].astype(F32))

    wait(cp_ca)
    mod_vec(1)
    wait(cp_sa)
    mod_vec(0)
    for i in range(LOOK // 32):
        put_a(0, pl.ds(i * 8, 8), *[
            h_s[pl.ds(i * 16 + off, 16), :] * mod(1, 16) + mod(0, 16)
            for off in (0, LOOK // 2)])
    in_s[pl.ds(M, RIDE), :] = h_s[pl.ds(LOOK, RIDE), :] * mod(1, RIDE) + mod(0, RIDE)

    def repack(p, u, c):
        top, bot = [_halves(w_s[p, pl.ds(off + c * 32, 32), :]) for off in (0, D2)]
        for e, v in enumerate(_words_each(
                top + bot + _strassen_rhs_sums(*top, *bot))):
            if e < 4:
                w_s[p, pl.ds((e // 2) * D2 + c * 32 + (e % 2) * 16, 16), :] = v
            else:
                w_s[T0 + 2 * u + (e - 4) // 4, pl.ds((e % 4) * K3 + c * 16, 16), :] = v

    def head(p, j, c0=0, c1=D // 32):
        return jnp.concatenate(
            [w_s[p, pl.ds(c * 32 + j * 16, 16), :] for c in range(c0, c1)], axis=0)

    cp_w(0).wait()
    for c in range(D2 // 32):
        repack(0, 0, c)

    @pl.loop(0, NP // 2)
    def _(i):
        two = w_s.at[pl.ds(2 * i + 1, 2)]
        pltpu.make_async_copy(two, two, sw.at[i + 1]).wait()
        for u in range(2):
            p = 2 * i + u

            def rhs(m):
                if _SUM[m] is None:
                    j = m // 4
                    return head(p, j, j * D2 // 32, (j + 1) * D2 // 32)
                return w_s[T0 + 2 * u + _SUM[m] // 4, pl.ds((_SUM[m] % 4) * K3, K3), :]

            jobs = [functools.partial(repack, p + 1, 1 - u, c) for c in range(D2 // 32)]
            cs = _strassen(lambda m: a_s[0][m][...], rhs,
                           _spread(jobs, 7))
            for q, y in enumerate(cs):
                ring_s[p, pl.ds(ROFF + (q // 2) * (LOOK // 2), LOOK // 2),
                       pl.ds((q % 2) * DH, DH)] = y.astype(BF16)

    for cp in cp_b:
        cp.start()
    wait(cp_a)
    in_s[pl.ds(0, M), :] = m0_s[...].astype(F32)

    KP = SEG + 2 * M
    row = lax.broadcasted_iota(jnp.int32, (L, KP), 0)
    col = lax.broadcasted_iota(jnp.int32, (L, KP), 1)
    visible = (col < L) & ((row < M) | (col >= SEG) | (row - M >= col))
    fill = jnp.where(col < L, -1e9, -jnp.inf).astype(F32)

    @pl.loop(0, NSEG)
    def _(s):
        seg = pl.ds(pl.multiple_of(s * SEG, SEG), SEG)
        nxt = pl.ds(pl.multiple_of(
            jnp.minimum(LOOK + (s + 1) * RIDE, S - RIDE), 8), RIDE)
        wr = pl.ds(pl.multiple_of(lax.rem(s * RIDE, RING), 8), RIDE)
        rd = pl.ds(pl.multiple_of(lax.rem(s * SEG + ROFF, RING), SEG), SEG)
        lhs_s[...] = _words(in_s[...])
        in_s[pl.ds(M, RIDE), :] = (
            _ln(x_s[nxt, :].astype(F32)) * mod(1, RIDE) + mod(0, RIDE))

        def project(p):
            w = jnp.concatenate([head(p, 0), head(p, 1)], axis=1)
            y = _dot(pltpu.bitcast(lhs_s[...], BF16), pltpu.bitcast(w, BF16))
            ring_s[p, wr, :] = y[M:].astype(BF16)
            return y[:M], ring_s[p, rd, :]

        def keys(p):
            mem, tok = project(p)
            tail = jnp.concatenate([mem, jnp.zeros_like(mem)], axis=0).astype(BF16)
            return jnp.concatenate([tok, tail], axis=0)

        def queries(p):
            mem, tok = project(2 * HP + p)
            return jnp.concatenate([mem, tok.astype(F32)], axis=0)

        def scores(qk):
            q, k = qk
            out = []
            for i in range(2):
                c = slice(i * DH, (i + 1) * DH)
                z = jnp.where(visible, _dot(q[:, c], k[:, c], _NT) * scale, fill)
                e = jnp.exp(z - jnp.max(z, axis=-1, keepdims=True))
                out.append((e, 1.0 / jnp.sum(e, axis=-1, keepdims=True)))
            return out

        def mix(p, es, v):
            for i, (e, inv) in enumerate(es):
                c = slice(i * DH, (i + 1) * DH)
                o_s[p, :, c] = _dot(e, v[:, c]) * inv

        def out_proj(p0, p1, j):
            c = pl.ds(j * 128, 128)
            lhs = jnp.concatenate([o_s[p] for p in range(p0, p1)], axis=1)
            w = wo_s[pl.ds(p0 * DH, (p1 - p0) * DH), c]
            return _dot(lhs, pltpu.bitcast(w, BF16))

        qk, es, vs = {}, {}, {}
        for t in range(HP + 2):
            if t < HP:
                k = keys(t)
                qk[t] = queries(t), k
            else:
                for j in range((t - HP) * CT // 2, (t - HP + 1) * CT // 2):
                    acc_s[:, pl.ds(j * 128, 128)] = out_proj(0, HP // 2, j)
            if 1 <= t <= HP:
                es[t - 1] = scores(qk.pop(t - 1))
                vs[t - 1] = keys(HP + t - 1)
            if t >= 2:
                mix(t - 2, es.pop(t - 2), vs.pop(t - 2))
        for j in range(CT):
            c = pl.ds(j * 128, 128)
            acc = acc_s[:, c] + out_proj(HP // 2, HP, j)
            in_s[pl.ds(0, M), c] = acc[:M]
            h_s[seg, c] = acc[M:]

    NB = S // RB
    G = CT // 4
    FT = w3_s.shape[1] // 128
    FH, CH, RH = FT // 2, CT // 2, RB // 2
    NI = NB // 2
    K4 = FT * 32

    def rows(i, off, n):
        return pl.ds(pl.multiple_of(i * RB + off, n), n)

    def col(j):
        return pl.ds(j * 128, 128)

    def block12(k, j):
        return lambda q: (mix_tile(k, j + (q % 2) * CH), (q // 2) * K3, slice(None))

    def block3(f):
        return lambda q: (w3_s, (q // 2) * K3, col(f + (q % 2) * FH))

    def block4(j):
        return lambda q: (w4_s, (q // 2) * K4, col(j + (q % 2) * CH))

    def home12(k, j):
        n = 5 * (CH * k + j)
        return lambda e: (2 * ((n + e) // 3) + 1, (1 + (n + e) % 3) * K3)

    def home3(f):
        return lambda e: (2 * f + e // 4, (e % 4) * K3)

    def home4(j):
        return lambda e: (2 * FH + 5 * j + e, 0)

    def make(block, home, r0):
        w = [ref[pl.ds(off + r0, 16), c] for ref, off, c in map(block, range(4))]
        w = pltpu.bitcast(jnp.concatenate(w, axis=1), BF16).astype(F32)
        for e, v in enumerate(_words_each(_strassen_rhs_sums(
                *[w[:, q * 128:(q + 1) * 128] for q in range(4)]))):
            slot, off = home(e)
            w_s[slot, pl.ds(off + r0, 16), :] = v

    def get_w(block, home, n):
        def rhs(m):
            if _SUM[m] is None:
                ref, off, c = block(0 if m == 1 else 3)
                return ref[pl.ds(off, n), c]
            slot, off = home(_SUM[m])
            return w_s[slot, pl.ds(off, n), :]
        return rhs

    def get_a(u):
        return lambda m: a_s[u][m][pl.ds(0, RH // 2), :]

    def put(u, g, half):
        put_a(u, pl.ds(g * 8, 8), half(g * 16), half(RH + g * 16))

    def norm1(i, g, u=0):
        def half(off):
            r = rows(i, off, 16)
            x1 = x_s[r, :].astype(F32) + mod(2, 16) * h_s[r, :]
            hb = _ln(x1) * mod(4, 16) + mod(3, 16)
            r_s[r, :] = hb
            return _ln(hb)
        put(u, g, half)

    def shifted(i, g, u=0):
        put(u, g, lambda off: jnp.concatenate(
            [hh_s[k, pl.ds(8 + i * RB + off + (-1, 1, -2, 2)[k // G], 16), :]
             for k in range(CT)], axis=1))

    def norm2(i, g, u=0):
        put(u, g, lambda off: _ln(r_s[rows(i, off, 16), :]))

    NG = RH // 16

    wait(cp_b)
    for j in (2, 3, 4, 5):
        mod_vec(j)
        for r0 in range(0, K3, 16):
            make(block12(0, j - 2), home12(0, j - 2), r0)
    for j in range(CT):
        hh_s[j, pl.ds(0, 8), :] = jnp.zeros((8, 128), F32)
        hh_s[j, pl.ds(8 + S, 8), :] = jnp.zeros((8, 128), F32)
    for g in range(NG):
        norm1(0, g)

    @pl.loop(0, NI)
    def _(ii):
        for u in range(2):
            i = 2 * ii + u
            jobs = []
            for g in range(NG):
                jobs.append(functools.partial(norm1, jnp.minimum(i + 1, NB - 1), g, 1 - u))
                jobs.append(functools.partial(
                    make, block12(1, g % CH), home12(1, g % CH),
                    pl.multiple_of(i * (K3 // NB) + (g // CH) * 16, 8)))
            tick = _spread(jobs, 7 * CH, 8)
            for j in range(CH):
                cs = _strassen(get_a(u), get_w(block12(0, j), home12(0, j), K3), tick)
                for q, y in enumerate(cs):
                    hh_s[j + (q % 2) * CH,
                         pl.ds(pl.multiple_of(8 + i * RB + (q // 2) * RH, 8), RH), :] = (
                             _gelu(y))

    for g in range(NG):
        shifted(0, g)

    @pl.loop(0, NI)
    def _(ii):
        for u in range(2):
            i = 2 * ii + u
            work = [(block3(f), home3(f), i * (K3 // NB) + v * 16)
                    for f in range(FH) for v in range(K3 // NB // 16)]
            work += [(block4(j), home4(j), i * (K4 // NB) + v * 16)
                     for j in range(CH) for v in range(K4 // NB // 16)]
            jobs = []
            for g in range(NG):
                jobs.append(functools.partial(shifted, jnp.minimum(i + 1, NB - 1), g, 1 - u))
                jobs += [functools.partial(make, b, h, pl.multiple_of(r0, 8))
                         for b, h, r0 in work[g::NG]]
            tick = _spread(jobs, 7 * CH)
            for j in range(CH):
                cs = _strassen(get_a(u), get_w(block12(1, j), home12(1, j), K3), tick)
                for q, y in enumerate(cs):
                    r_s[rows(i, (q // 2) * RH, RH), col(j + (q % 2) * CH)] += y

    def cp_y(i):
        return pltpu.make_async_copy(
            y_s.at[i % 2], out_hbm.at[rows(i, 0, RB)], sy.at[i % 2])

    for g in range(NG):
        norm2(0, g)

    @pl.loop(0, NB)
    def _(i):
        @pl.when(i >= 2)
        def _():
            cp_y(i - 2).wait()

        for f in range(FH):
            cs = _strassen(get_a(0), get_w(block3(f), home3(f), K3))
            for m, v in enumerate(_strassen_lhs(*map(_gelu, cs))):
                t_s[m][:, col(f)] = _words(v)
        for j in range(CH):
            cs = _strassen(lambda m: t_s[m][...], get_w(block4(j), home4(j), K4))
            for q, h2 in enumerate(cs):
                r, c = rows(i, (q // 2) * RH, RH), col(j + (q % 2) * CH)
                x1 = x_s[r, c].astype(F32) + mod(2, RH, c) * h_s[r, c]
                y = x1 + mod(5, RH, c) * (r_s[r, c] + h2)
                y_s[i % 2, pl.ds((q // 2) * RH, RH), c] = y.astype(y_s.dtype)
            if j < 2:
                for g in range(j * NG // 2, (j + 1) * NG // 2):
                    norm2(jnp.minimum(i + 1, NB - 1), g)
        cp_y(i).start()

    cp_y(NB - 2).wait()
    cp_y(NB - 1).wait()


@functools.partial(jax.jit, static_argnames=("A_seg_len",))
def pallas_adaLN_cond__memory_aug_recurrent_mem_tr__mixer_s_mlp__prompt_kernel(
    A_x, A_mem0, A_Wq, A_Wk, A_Wv, A_Wo, A_seg_len, B_x, B_w1, B_w2, B_w3, B_w4,
    c, w_mod,
):
    del B_x
    _, S, D = A_x.shape
    _, H, DH = A_Wq.shape
    M = A_mem0.shape[1]
    SEG = int(A_seg_len)
    FF = B_w3.shape[1]
    HP = H // 2
    RB = 256
    LOOK = S - (S // SEG) * (SEG - M)
    RING = LOOK + 64
    vm = pltpu.VMEM
    dma = pltpu.SemaphoreType.DMA
    scratch = [
        vm((3 * HP + 1 + D // 128, D, DH), U32), vm((HP * DH, D), U32),
        vm((D // 2, FF), U32), vm((FF // 2, D), U32), vm((6, D // 2, D), U32),
        vm((S, D), A_x.dtype), vm((S, D), F32), vm((S, D), F32),
        vm((D // 128, S + 16, 128), F32), vm((3 * HP, RING, 2 * DH), BF16),
        vm((1, D), c.dtype), vm((M, D), A_mem0.dtype),
        vm((SEG, D), F32), vm((SEG // 2, D), U32),
        vm((HP, M + SEG, 2 * DH), F32), vm((M + SEG, D), F32), vm((6, 8, D), F32),
        [[vm((LOOK // 4, D // 2), U32)] * 7] * 2, [vm((RB // 4, FF // 2), U32)] * 7,
        vm((2, RB, D), A_x.dtype),
        dma((3 * HP // 2 + 1,)), dma((5,)), dma((2,)),
    ]
    out = pl.pallas_call(
        functools.partial(_kernel, S=S, D=D, H=H, DH=DH, M=M, SEG=SEG, RB=RB),
        out_shape=jax.ShapeDtypeStruct((S, D), A_x.dtype),
        in_specs=[pl.BlockSpec(memory_space=pl.ANY)] * 12,
        out_specs=pl.BlockSpec(memory_space=pl.ANY),
        scratch_shapes=scratch,
        compiler_params=pltpu.CompilerParams(
            vmem_limit_bytes=124 * 1024 * 1024,
            flags={"XLA_TPU_EVENLY_DISTRIBUTE_CRITICAL_NODES": True}),
    )(A_x.reshape(S, D), A_mem0.reshape(M, D), A_Wq, A_Wk, A_Wv,
      A_Wo.reshape(H * DH, D), B_w1, B_w2, B_w3, B_w4, c, w_mod)
    return out.reshape(A_x.shape)
```

```python
import functools

import jax
import jax.numpy as jnp
import numpy as np
from jax import lax
import jax.experimental.pallas as pl
import jax.experimental.pallas.tpu as pltpu

F32 = jnp.float32
BF16 = jnp.bfloat16
U32 = jnp.uint32

_NN = (((1,), (0,)), ((), ()))
_NT = (((1,), (1,)), ((), ()))


def _dot(a, b, dims=_NN):
    return lax.dot_general(a, b, dims, preferred_element_type=F32)


def _ln(x):
    m = jnp.mean(x, axis=-1, keepdims=True)
    d = x - m
    v = jnp.mean(d * d, axis=-1, keepdims=True)
    return d * lax.rsqrt(v + 1e-5)


def _gelu(x):
    k0 = float(np.sqrt(2.0 / np.pi))
    k1 = float(np.sqrt(2.0 / np.pi) * 0.044715)
    hx = 0.5 * x
    return hx + hx * jnp.tanh(x * (k0 + k1 * (x * x)))


def _words(x):
    return pltpu.bitcast(x.astype(BF16), U32)


def _halves(w):
    return (pltpu.bitcast(w << 16, F32),
            pltpu.bitcast(w & np.uint32(0xFFFF0000), F32))


def _words_each(xs):
    w = _words(jnp.concatenate(xs, axis=1))
    return [w[:, e * 128:(e + 1) * 128] for e in range(len(xs))]


def _spread(jobs, last, first=1):
    state = [0, 0]

    def tick():
        state[0] += 1
        due = -(-(state[0] - first) * len(jobs) // (last - first))
        while state[1] < min(len(jobs), due):
            jobs[state[1]]()
            state[1] += 1
    return tick


def _strassen_lhs(a11, a12, a21, a22):
    return (a11 + a22, a21 + a22, a11, a22, a11 + a12, a21 - a11, a12 - a22)


def _strassen_rhs_sums(b11, b12, b21, b22):
    return (b11 + b22, b12 - b22, b21 - b11, b11 + b12, b21 + b22)


_SUM = (0, None, 1, 2, None, 3, 4)


def _strassen(lhs, rhs, tick=lambda: None):
    def prod(m):
        tick()
        return _dot(pltpu.bitcast(lhs(m), BF16), pltpu.bitcast(rhs(m), BF16))

    m0, m1 = prod(0), prod(1)
    c22 = m0 - m1
    m3 = prod(3)
    c11 = m0 + m3
    c21 = m1 + m3
    m2 = prod(2)
    c22 = c22 + m2
    m4 = prod(4)
    c12 = m2 + m4
    c11 = c11 - m4
    c22 = c22 + prod(5)
    c11 = c11 + prod(6)
    return c11, c12, c21, c22


def _kernel(x_hbm, mem_hbm, wq_hbm, wk_hbm, wv_hbm, wo_hbm, w1_hbm, w2_hbm,
            w3_hbm, w4_hbm, c_hbm, wm_hbm, out_hbm,
            w_s, wo_s, w3_s, w4_s, wm_s, x_s, h_s, r_s, hh_s, ring_s,
            c_s, m0_s, in_s, lhs_s, o_s, acc_s, mod_s, a_s, t_s, y_s,
            sw, sx, sy,
            *, S, D, H, DH, M, SEG, RB):
    HP = H // 2
    NP = 3 * HP
    T0 = NP + 1
    NSEG = S // SEG
    L = M + SEG
    RIDE = SEG - M
    LOOK = S - NSEG * RIDE
    RING = ring_s.shape[1]
    ROFF = RING - LOOK
    D2 = D // 2
    K3 = D // 4
    CT = D // 128
    X0 = LOOK + 32
    scale = float(DH) ** -0.5

    def cp_w(p):
        src = (wk_hbm, wv_hbm, wq_hbm)[p // HP % 3].bitcast(U32)
        return pltpu.make_async_copy(
            src.at[:, p % HP], w_s.at[p], sw.at[(p + 1) // 2])

    def mix_tile(k, j):
        return w_s.at[T0 + j, pl.ds(k * D2, D2)]

    def copies(pairs, sem):
        return [pltpu.make_async_copy(src, dst, sem) for src, dst in pairs]

    def mod_pair(j):
        return wm_hbm.bitcast(U32).at[:, pl.ds(j * D, D)], wm_s.at[j]

    cp_first = copies([(c_hbm, c_s),
                       (x_hbm.at[pl.ds(0, X0)], x_s.at[pl.ds(0, X0)])], sx.at[0])
    cp_ca = copies([mod_pair(1)], sx.at[1])
    cp_sa = copies([mod_pair(0)], sx.at[2])
    cp_a = copies([(mem_hbm, m0_s),
                   (x_hbm.at[pl.ds(X0, S - X0)], x_s.at[pl.ds(X0, S - X0)]),
                   (wo_hbm.bitcast(U32), wo_s)], sx.at[3])
    cp_b = copies(
        [mod_pair(j) for j in range(2, 6)]
        + [(src.bitcast(U32).at[:, pl.ds(j * 128, 128)], mix_tile(k, j))
           for k, src in enumerate((w1_hbm, w2_hbm)) for j in range(CT)]
        + [(w3_hbm.bitcast(U32), w3_s), (w4_hbm.bitcast(U32), w4_s)], sx.at[4])

    def wait(cps):
        for cp in cps:
            cp.wait()

    for cp in cp_first + cp_ca + cp_sa + [cp_w(p) for p in range(NP + 1)] + cp_a:
        cp.start()

    wait(cp_first)
    cf = c_s[...].astype(F32)
    sc = jnp.broadcast_to(cf * jax.nn.sigmoid(cf), (8, D))

    def mod_vec(j):
        y = _dot(sc, pltpu.bitcast(wm_s[j], BF16))
        mod_s[j] = 1.0 + y if j in (1, 4) else y

    def mod(j, n, c=slice(None)):
        return jnp.concatenate([mod_s[j, :, c]] * (n // 8), axis=0)

    def put_a(u, r, top, bot):
        for m, v in enumerate(_strassen_lhs(
                top[:, :D2], top[:, D2:], bot[:, :D2], bot[:, D2:])):
            a_s[u][m][r, :] = _words(v)

    @pl.loop(0, X0 // 32)
    def _(i):
        r = pl.ds(pl.multiple_of(i * 32, 32), 32)
        h_s[r, :] = _ln(x_s[r, :].astype(F32))

    wait(cp_ca)
    mod_vec(1)
    wait(cp_sa)
    mod_vec(0)
    for i in range(LOOK // 32):
        put_a(0, pl.ds(i * 8, 8), *[
            h_s[pl.ds(i * 16 + off, 16), :] * mod(1, 16) + mod(0, 16)
            for off in (0, LOOK // 2)])
    in_s[pl.ds(M, RIDE), :] = h_s[pl.ds(LOOK, RIDE), :] * mod(1, RIDE) + mod(0, RIDE)

    def repack(p, u, c):
        top, bot = [_halves(w_s[p, pl.ds(off + c * 32, 32), :]) for off in (0, D2)]
        for e, v in enumerate(_words_each(
                top + bot + _strassen_rhs_sums(*top, *bot))):
            if e < 4:
                w_s[p, pl.ds((e // 2) * D2 + c * 32 + (e % 2) * 16, 16), :] = v
            else:
                w_s[T0 + 2 * u + (e - 4) // 4, pl.ds((e % 4) * K3 + c * 16, 16), :] = v

    def head(p, j, c0=0, c1=D // 32):
        return jnp.concatenate(
            [w_s[p, pl.ds(c * 32 + j * 16, 16), :] for c in range(c0, c1)], axis=0)

    cp_w(0).wait()
    for c in range(D2 // 32):
        repack(0, 0, c)

    @pl.loop(0, NP // 2)
    def _(i):
        two = w_s.at[pl.ds(2 * i + 1, 2)]
        pltpu.make_async_copy(two, two, sw.at[i + 1]).wait()
        for u in range(2):
            p = 2 * i + u

            def rhs(m):
                if _SUM[m] is None:
                    j = m // 4
                    return head(p, j, j * D2 // 32, (j + 1) * D2 // 32)
                return w_s[T0 + 2 * u + _SUM[m] // 4, pl.ds((_SUM[m] % 4) * K3, K3), :]

            jobs = [functools.partial(repack, p + 1, 1 - u, c) for c in range(D2 // 32)]
            cs = _strassen(lambda m: a_s[0][m][...], rhs,
                           _spread(jobs, 7))
            for q, y in enumerate(cs):
                ring_s[p, pl.ds(ROFF + (q // 2) * (LOOK // 2), LOOK // 2),
                       pl.ds((q % 2) * DH, DH)] = y.astype(BF16)

    for cp in cp_b:
        cp.start()
    wait(cp_a)
    in_s[pl.ds(0, M), :] = m0_s[...].astype(F32)

    KP = SEG + 2 * M
    row = lax.broadcasted_iota(jnp.int32, (L, KP), 0)
    col = lax.broadcasted_iota(jnp.int32, (L, KP), 1)
    visible = (col < L) & ((row < M) | (col >= SEG) | (row - M >= col))
    fill = jnp.where(col < L, -1e9, -jnp.inf).astype(F32)

    @pl.loop(0, NSEG)
    def _(s):
        seg = pl.ds(pl.multiple_of(s * SEG, SEG), SEG)
        nxt = pl.ds(pl.multiple_of(
            jnp.minimum(LOOK + (s + 1) * RIDE, S - RIDE), 8), RIDE)
        wr = pl.ds(pl.multiple_of(lax.rem(s * RIDE, RING), 8), RIDE)
        rd = pl.ds(pl.multiple_of(lax.rem(s * SEG + ROFF, RING), SEG), SEG)
        lhs_s[...] = _words(in_s[...])
        in_s[pl.ds(M, RIDE), :] = (
            _ln(x_s[nxt, :].astype(F32)) * mod(1, RIDE) + mod(0, RIDE))

        def project(p):
            w = jnp.concatenate([head(p, 0), head(p, 1)], axis=1)
            y = _dot(pltpu.bitcast(lhs_s[...], BF16), pltpu.bitcast(w, BF16))
            ring_s[p, wr, :] = y[M:].astype(BF16)
            return y[:M], ring_s[p, rd, :]

        def keys(p):
            mem, tok = project(p)
            tail = jnp.concatenate([mem, jnp.zeros_like(mem)], axis=0).astype(BF16)
            return jnp.concatenate([tok, tail], axis=0)

        def queries(p):
            mem, tok = project(2 * HP + p)
            return jnp.concatenate([mem, tok.astype(F32)], axis=0)

        def scores(qk):
            q, k = qk
            out = []
            for i in range(2):
                c = slice(i * DH, (i + 1) * DH)
                z = jnp.where(visible, _dot(q[:, c], k[:, c], _NT) * scale, fill)
                e = jnp.exp(z - jnp.max(z, axis=-1, keepdims=True))
                out.append((e, 1.0 / jnp.sum(e, axis=-1, keepdims=True)))
            return out

        def mix(p, es, v):
            for i, (e, inv) in enumerate(es):
                c = slice(i * DH, (i + 1) * DH)
                o_s[p, :, c] = _dot(e, v[:, c]) * inv

        def out_proj(p0, p1, j):
            c = pl.ds(j * 128, 128)
            lhs = jnp.concatenate([o_s[p] for p in range(p0, p1)], axis=1)
            w = wo_s[pl.ds(p0 * DH, (p1 - p0) * DH), c]
            return _dot(lhs, pltpu.bitcast(w, BF16))

        qk, es, vs = {}, {}, {}
        for t in range(HP + 2):
            if t < HP:
                k = keys(t)
                qk[t] = queries(t), k
            else:
                for j in range((t - HP) * CT // 2, (t - HP + 1) * CT // 2):
                    acc_s[:, pl.ds(j * 128, 128)] = out_proj(0, HP // 2, j)
            if 1 <= t <= HP:
                es[t - 1] = scores(qk.pop(t - 1))
                vs[t - 1] = keys(HP + t - 1)
            if t >= 2:
                mix(t - 2, es.pop(t - 2), vs.pop(t - 2))
        for j in range(CT):
            c = pl.ds(j * 128, 128)
            acc = acc_s[:, c] + out_proj(HP // 2, HP, j)
            in_s[pl.ds(0, M), c] = acc[:M]
            h_s[seg, c] = acc[M:]

    NB = S // RB
    G = CT // 4
    FT = w3_s.shape[1] // 128
    FH, CH, RH = FT // 2, CT // 2, RB // 2
    NI = NB // 2
    K4 = FT * 32

    def rows(i, off, n):
        return pl.ds(pl.multiple_of(i * RB + off, n), n)

    def col(j):
        return pl.ds(j * 128, 128)

    def block12(k, j):
        return lambda q: (mix_tile(k, j + (q % 2) * CH), (q // 2) * K3, slice(None))

    def block3(f):
        return lambda q: (w3_s, (q // 2) * K3, col(f + (q % 2) * FH))

    def block4(j):
        return lambda q: (w4_s, (q // 2) * K4, col(j + (q % 2) * CH))

    def home12(k, j):
        n = 5 * (CH * k + j)
        return lambda e: (2 * ((n + e) // 3) + 1, (1 + (n + e) % 3) * K3)

    def home3(f):
        return lambda e: (2 * f + e // 4, (e % 4) * K3)

    def home4(j):
        return lambda e: (2 * FH + 5 * j + e, 0)

    def make(block, home, r0):
        w = [ref[pl.ds(off + r0, 16), c] for ref, off, c in map(block, range(4))]
        w = pltpu.bitcast(jnp.concatenate(w, axis=1), BF16).astype(F32)
        for e, v in enumerate(_words_each(_strassen_rhs_sums(
                *[w[:, q * 128:(q + 1) * 128] for q in range(4)]))):
            slot, off = home(e)
            w_s[slot, pl.ds(off + r0, 16), :] = v

    def get_w(block, home, n):
        def rhs(m):
            if _SUM[m] is None:
                ref, off, c = block(0 if m == 1 else 3)
                return ref[pl.ds(off, n), c]
            slot, off = home(_SUM[m])
            return w_s[slot, pl.ds(off, n), :]
        return rhs

    def get_a(u):
        return lambda m: a_s[u][m][pl.ds(0, RH // 2), :]

    def put(u, g, half):
        put_a(u, pl.ds(g * 8, 8), half(g * 16), half(RH + g * 16))

    def norm1(i, g, u=0):
        def half(off):
            r = rows(i, off, 16)
            x1 = x_s[r, :].astype(F32) + mod(2, 16) * h_s[r, :]
            hb = _ln(x1) * mod(4, 16) + mod(3, 16)
            r_s[r, :] = hb
            return _ln(hb)
        put(u, g, half)

    def shifted(i, g, u=0):
        put(u, g, lambda off: jnp.concatenate(
            [hh_s[k, pl.ds(8 + i * RB + off + (-1, 1, -2, 2)[k // G], 16), :]
             for k in range(CT)], axis=1))

    def norm2(i, g, u=0):
        put(u, g, lambda off: _ln(r_s[rows(i, off, 16), :]))

    NG = RH // 16

    wait(cp_b)
    for j in (2, 3, 4, 5):
        mod_vec(j)
        for r0 in range(0, K3, 16):
            make(block12(0, j - 2), home12(0, j - 2), r0)
    for j in range(CT):
        hh_s[j, pl.ds(0, 8), :] = jnp.zeros((8, 128), F32)
        hh_s[j, pl.ds(8 + S, 8), :] = jnp.zeros((8, 128), F32)
    for g in range(NG):
        norm1(0, g)

    @pl.loop(0, NI)
    def _(ii):
        for u in range(2):
            i = 2 * ii + u
            nxt, jobs = jnp.minimum(i + 1, NB - 1), []
            for g in range(NG):
                jobs.append(functools.partial(norm1, nxt, g, 1 - u))
                jobs.append(functools.partial(
                    make, block12(1, g % CH), home12(1, g % CH),
                    pl.multiple_of(i * (K3 // NB) + (g // CH) * 16, 8)))
            tick = _spread(jobs, 7 * CH - 4, 4)
            for j in range(CH):
                cs = _strassen(get_a(u), get_w(block12(0, j), home12(0, j), K3), tick)
                for q, y in enumerate(cs):
                    hh_s[j + (q % 2) * CH,
                         pl.ds(pl.multiple_of(8 + i * RB + (q // 2) * RH, 8), RH), :] = (
                             _gelu(y))

    for g in range(NG):
        shifted(0, g)

    @pl.loop(0, NI)
    def _(ii):
        for u in range(2):
            i = 2 * ii + u
            work = [(block3(f), home3(f), i * (K3 // NB) + v * 16)
                    for f in range(FH) for v in range(K3 // NB // 16)]
            work += [(block4(j), home4(j), i * (K4 // NB) + v * 16)
                     for j in range(CH) for v in range(K4 // NB // 16)]
            nxt, jobs = jnp.minimum(i + 1, NB - 1), []
            for g in range(NG):
                jobs.append(functools.partial(shifted, nxt, g, 1 - u))
                jobs += [functools.partial(make, b, h, pl.multiple_of(r0, 8))
                         for b, h, r0 in work[g::NG]]
            tick = _spread(jobs, 7 * CH)
            for j in range(CH):
                cs = _strassen(get_a(u), get_w(block12(1, j), home12(1, j), K3), tick)
                for q, y in enumerate(cs):
                    r_s[rows(i, (q // 2) * RH, RH), col(j + (q % 2) * CH)] += y

    def cp_y(i):
        return pltpu.make_async_copy(
            y_s.at[i % 2], out_hbm.at[rows(i, 0, RB)], sy.at[i % 2])

    for g in range(NG):
        norm2(0, g)

    @pl.loop(0, NB)
    def _(i):
        @pl.when(i >= 2)
        def _():
            cp_y(i - 2).wait()

        for f in range(FH):
            cs = _strassen(get_a(0), get_w(block3(f), home3(f), K3))
            for m, v in enumerate(_strassen_lhs(*map(_gelu, cs))):
                t_s[m][:, col(f)] = _words(v)
        for j in range(CH):
            cs = _strassen(lambda m: t_s[m][...], get_w(block4(j), home4(j), K4))
            for q, h2 in enumerate(cs):
                r, c = rows(i, (q // 2) * RH, RH), col(j + (q % 2) * CH)
                x1 = x_s[r, c].astype(F32) + mod(2, RH, c) * h_s[r, c]
                y = x1 + mod(5, RH, c) * (r_s[r, c] + h2)
                y_s[i % 2, pl.ds((q // 2) * RH, RH), c] = y.astype(y_s.dtype)
            if j < 2:
                for g in range(j * NG // 2, (j + 1) * NG // 2):
                    norm2(jnp.minimum(i + 1, NB - 1), g)
        cp_y(i).start()

    cp_y(NB - 2).wait()
    cp_y(NB - 1).wait()


@functools.partial(jax.jit, static_argnames=("A_seg_len",))
def pallas_adaLN_cond__memory_aug_recurrent_mem_tr__mixer_s_mlp__prompt_kernel(
    A_x, A_mem0, A_Wq, A_Wk, A_Wv, A_Wo, A_seg_len, B_x, B_w1, B_w2, B_w3, B_w4,
    c, w_mod,
):
    del B_x
    _, S, D = A_x.shape
    _, H, DH = A_Wq.shape
    M = A_mem0.shape[1]
    SEG = int(A_seg_len)
    FF = B_w3.shape[1]
    assert (A_x.shape, H, DH, M, SEG, FF) == ((1, 2048, 1024), 32, 128, 8, 32, 3584)
    HP = H // 2
    RB = 256
    LOOK = S - (S // SEG) * (SEG - M)
    RING = LOOK + 64
    vm = pltpu.VMEM
    dma = pltpu.SemaphoreType.DMA
    scratch = [
        vm((3 * HP + 1 + D // 128, D, DH), U32), vm((HP * DH, D), U32),
        vm((D // 2, FF), U32), vm((FF // 2, D), U32), vm((6, D // 2, D), U32),
        vm((S, D), A_x.dtype), vm((S, D), F32), vm((S, D), F32),
        vm((D // 128, S + 16, 128), F32), vm((3 * HP, RING, 2 * DH), BF16),
        vm((1, D), c.dtype), vm((M, D), A_mem0.dtype),
        vm((SEG, D), F32), vm((SEG // 2, D), U32),
        vm((HP, M + SEG, 2 * DH), F32), vm((M + SEG, D), F32), vm((6, 8, D), F32),
        [[vm((LOOK // 4, D // 2), U32)] * 7] * 2, [vm((RB // 4, FF // 2), U32)] * 7,
        vm((2, RB, D), A_x.dtype),
        dma((3 * HP // 2 + 1,)), dma((5,)), dma((2,)),
    ]
    out = pl.pallas_call(
        functools.partial(_kernel, S=S, D=D, H=H, DH=DH, M=M, SEG=SEG, RB=RB),
        out_shape=jax.ShapeDtypeStruct((S, D), A_x.dtype),
        in_specs=[pl.BlockSpec(memory_space=pl.ANY)] * 12,
        out_specs=pl.BlockSpec(memory_space=pl.ANY),
        scratch_shapes=scratch,
        compiler_params=pltpu.CompilerParams(
            vmem_limit_bytes=124 * 1024 * 1024,
            flags={"XLA_TPU_EVENLY_DISTRIBUTE_CRITICAL_NODES": True}),
    )(A_x.reshape(S, D), A_mem0.reshape(M, D), A_Wq, A_Wk, A_Wv,
      A_Wo.reshape(H * DH, D), B_w1, B_w2, B_w3, B_w4, c, w_mod)
    return out.reshape(A_x.shape)
```
